```python
import os as _os
_os.environ.setdefault('JAX_PLATFORMS', 'cpu')
import jax
import jax.numpy as jnp

def _softmax(x, axis=-1):
    return jax.nn.softmax(x, axis=axis)

def _gelu(x):
    return jax.nn.gelu(x, approximate=True)

def _silu(x):
    return jax.nn.silu(x)

def _sigmoid(x):
    return jax.nn.sigmoid(x)

def _layernorm(x, axis=-1, eps=1e-05):
    m = jnp.mean(x, axis=axis, keepdims=True)
    v = jnp.var(x, axis=axis, keepdims=True)
    return (x - m) / jnp.sqrt(v + eps)

def _scatter_add(tgt, idx, src, axis=0):
    return tgt.at[idx].add(src)

def _segment_sum(src, seg, n):
    return jax.ops.segment_sum(src, seg, n)

class _Rng:

    def __init__(self, key):
        self._k = key

    def _next(self):
        self._k, sub = jax.random.split(self._k)
        return sub

    def normal(self, shape):
        return jax.random.normal(self._next(), shape, dtype=jnp.bfloat16)

    def randint(self, lo, hi, shape):
        return jax.random.randint(self._next(), shape, lo, hi, dtype=jnp.int32)

    def uniform(self, shape, lo=0.0, hi=1.0):
        return jax.random.uniform(self._next(), shape, jnp.bfloat16, lo, hi)

    def permutation(self, n):
        return jax.random.permutation(self._next(), n)
kernel_name = 'adaLN_cond__sliding_block__mixer_channel_mlp__prompt'

def setup_inputs():
    _rng = _Rng(jax.random.key(int.from_bytes(__import__("os").urandom(4), "little")))
    _w = lambda a: (lambda t: t.astype(jnp.bfloat16) if jnp.issubdtype(t.dtype, jnp.floating) else t)(jnp.asarray(a))

    def _A_setup():
        B, S, D = (1, 2048, 640)
        return {'x': _w((lambda *s: _rng.normal(s) * 0.05)(B, S, D)), 'wqkv': _w((lambda *s: _rng.normal(s) * 0.05)(D, 3 * D)), 'wo': _w((lambda *s: _rng.normal(s) * 0.05)(D, D))}
    _A_in = _A_setup()

    def _B_setup():
        B, S, D, F = (1, 2048, 640, 1728)
        return {'x': _w((lambda *s: _rng.normal(s) * 0.05)(B, S, D)), 'w1': _w((lambda *s: _rng.normal(s) * 0.8)(D, F) * D ** (-0.5)), 'b1': _w((lambda *s: _rng.normal(s) * 0.8)(F)), 'w2': _w((lambda *s: _rng.normal(s) * 0.8)(F, D) * F ** (-0.5)), 'b2': _w((lambda *s: _rng.normal(s) * 0.4)(D))}
    _B_in = _B_setup()
    return {'A_x': _A_in['x'], 'A_wqkv': _A_in['wqkv'], 'A_wo': _A_in['wo'], 'B_x': _B_in['x'], 'B_w1': _B_in['w1'], 'B_b1': _B_in['b1'], 'B_w2': _B_in['w2'], 'B_b2': _B_in['b2'], 'c': _w((lambda *s: _rng.normal(s) * 0.05)(1, 640) * 8.0), 'w_mod': _w((lambda *s: _rng.normal(s) * 0.05)(640, 6 * 640) * 640 ** (-0.5) * 8.0)}

def reference(A_x, A_wqkv, A_wo, B_x, B_w1, B_b1, B_w2, B_b2, c, w_mod):

    def _A_ref(x, wqkv, wo):
        B, S, D = x.shape
        H = 32
        Dh = D // H
        W = 256
        qkv = (lambda x, *d: x.transpose(*d))((x @ wqkv).reshape(B, S, 3, H, Dh), 2, 0, 3, 1, 4)
        q, k, v = (qkv[0], qkv[1], qkv[2])
        scores = jnp.einsum('bhqd,bhkd->bhqk', q, k) * Dh ** (-0.5)
        idx = jnp.arange(S)
        mask = (idx[:, None] - idx[None, :] >= 0) & (idx[:, None] - idx[None, :] < W)
        scores = jnp.where(mask[None, None], scores, -1000000000.0)
        p = _softmax(scores, axis=-1)
        o = jnp.einsum('bhqk,bhkd->bhqd', p, v)
        return (lambda x, *d: x.transpose(*d))(o, 0, 2, 1, 3).reshape(B, S, D) @ wo

    def _B_ref(x, w1, b1, w2, b2):
        y = _layernorm(x, axis=-1)
        h = _gelu(jnp.einsum('bsd,df->bsf', y, w1) + b1)
        return jnp.einsum('bsf,fd->bsd', h, w2) + b2
    x = A_x
    mod = (_silu(c) @ w_mod).reshape(c.shape[0], 6, 1, -1)
    sa, ca, ga, sb, cb, gb = (mod[:, 0].copy(), mod[:, 1].copy(), mod[:, 2].copy(), mod[:, 3].copy(), mod[:, 4].copy(), mod[:, 5].copy())
    h = _layernorm(x, axis=-1) * (1 + ca) + sa
    x = x + ga * _A_ref(h, A_wqkv, A_wo)
    h = _layernorm(x, axis=-1) * (1 + cb) + sb
    x = x + gb * _B_ref(h, B_w1, B_b1, B_w2, B_b2)
    return x
```

```python
import functools
import jax
import jax.numpy as jnp
from jax import lax
import jax.experimental.pallas as pl
import jax.experimental.pallas.tpu as pltpu

S, D, H, DH, WIN, F = 2048, 640, 32, 20, 256, 1728
T = 256
QB = 128
NB = S // QB
NS = S // T
NG = 8
EPS = 1e-5
LOG2E = 1.4426950408889634
QSCALE = DH ** -0.5 * LOG2E
f32, bf16, u32 = jnp.float32, jnp.bfloat16, jnp.uint32
NT = (((1,), (1,)), ((), ()))


def _ln(x):
    m = jnp.mean(x, axis=-1, keepdims=True)
    xc = x - m
    v = jnp.mean(xc * xc, axis=-1, keepdims=True)
    return xc * lax.rsqrt(v + EPS)


def _pack(x):
    return pltpu.bitcast(x.astype(bf16), u32)


def _packi(a, b):
    return pltpu.bitcast(pltpu.pack_elementwise([a, b], packed_dtype=bf16), u32)


def _unpack(x):
    return pltpu.bitcast(x, bf16)


def _gelu(x):
    c = 0.7978845608028654
    return 0.5 * x * (1.0 + jnp.tanh(x * (c + (c * 0.044715) * (x * x))))


def kernel(x_h, c_h, b1_h, b2_h, wqkv_h, wo_h, w1t_h, w2_h, wmod_h, o_ref,
           x_v, c_v, b1_v, b2_v, wq_v, wk_v, wv_v, wo_v, w1t_v, w2_v, wm1_v, wm2_v, sems,
           mod_s, wqT_s, wvT_s, k_s, vT_s, qT_s, oT_s, s_s, ob_s):
    step = pl.program_id(0)

    pairs = dict(
        c=(c_h, c_v), x0=(x_h.at[0, 0:T], x_v.at[0:T]),
        wq=(wqkv_h.at[:, 0:D], wq_v), wm1=(wmod_h.at[:, 0:2 * D], wm1_v),
        wk=(wqkv_h.at[:, D:2 * D], wk_v), wv=(wqkv_h.at[:, 2 * D:3 * D], wv_v),
        x1=(x_h.at[0, T:2 * T], x_v.at[T:2 * T]),
        wo=(wo_h, wo_v), wm2=(wmod_h.at[:, 2 * D:6 * D], wm2_v),
        b1=(b1_h, b1_v), b2=(b2_h, b2_v), w1=(w1t_h, w1t_v), w2=(w2_h, w2_v),
        xr=(x_h.at[0, 2 * T:S], x_v.at[2 * T:S]),
    )
    names = list(pairs)

    def cp(n):
        s, d = pairs[n]
        return pltpu.make_async_copy(s, d, sems.at[names.index(n)])

    def silu_c():
        c = c_v[...].astype(f32)
        return jnp.broadcast_to((c * jax.nn.sigmoid(c)).astype(bf16), (16, D))

    def modv(i):
        return mod_s[0:1, i * D:(i + 1) * D]

    def body(variant):
        first = variant == "first"
        do_a = variant != "last"
        do_m = variant != "first"
        g0 = step * (T // QB)
        row8 = lax.broadcasted_iota(jnp.int32, (8, QB), 0)
        lo4 = row8 < 4
        st = {}

        def ln1():
            x = x_v[pl.ds(pl.multiple_of(step * T, T), T), :].astype(f32)
            n = _ln(x)
            if first:
                cp("wm1").wait()
                mod_s[:, 0:2 * D] = jnp.dot(silu_c(), wm1_v[...], preferred_element_type=f32)[0:8]
            h = n * (1.0 + modv(1)) + modv(0)
            st["hb"] = h.astype(bf16)
            st["hi"] = _unpack(jnp.concatenate(
                [_packi(h[QB * b:QB * b + 64], h[QB * b + 64:QB * b + 128]) for b in range(T // QB)], axis=0))

        def kproj():
            kf = jnp.dot(st["hb"], wk_v[...], preferred_element_type=f32)
            lane = lax.broadcasted_iota(jnp.int32, (QB, 128), 1)
            for b in range(T // QB):
                kb = kf[QB * b:QB * b + QB]
                tiles = []
                for g in range(NG):
                    t0, t1 = (80 * g) // 128, (80 * g + 79) // 128
                    if t0 == t1:
                        tiles.append(kb[:, 128 * t0:128 * t0 + 128])
                    else:
                        tiles.append(jnp.where(lane >= 64, kb[:, 128 * t0:128 * t0 + 128],
                                               kb[:, 128 * t1:128 * t1 + 128]))
                k_s[g0 + b] = _pack(jnp.concatenate(tiles, axis=1))

        def windows(src, fill):
            fl = jnp.full((8, QB), fill, f32)
            out = []
            for hh in range(H):
                a = (DH * hh) // 16
                off = DH * hh - 16 * a
                v = [src[16 * a + 8 * i:16 * a + 8 * i + 8] for i in range(4)]
                if off == 0:
                    out += [v[0], v[1], jnp.where(lo4, v[2], fl), fl]
                elif off == 4:
                    out += [jnp.where(lo4, fl, v[0]), v[1], v[2], fl]
                elif off == 8:
                    out += [fl, v[1], v[2], jnp.where(lo4, v[3], fl)]
                else:
                    out += [fl, jnp.where(lo4, fl, v[1]), v[2], v[3]]
            return jnp.concatenate(out, axis=0)

        def qproj():
            qf = lax.dot_general(_unpack(wqT_s[...]), st["hb"], NT, preferred_element_type=f32) * QSCALE
            for b in range(T // QB):
                qT_s[b] = _pack(windows(qf[:, QB * b:QB * b + QB], 0.0))

        def vproj():
            vf = lax.dot_general(_unpack(wvT_s[...]), st["hi"], NT, preferred_element_type=f32)
            for b in range(T // QB):
                vT_s[g0 + b] = _pack(windows(vf[:, QB * b:QB * b + QB], 1.0))

        dd = (lax.broadcasted_iota(jnp.int32, (16, 128), 1)
              - lax.broadcasted_iota(jnp.int32, (16, 128), 0))
        r64 = lax.broadcasted_iota(jnp.int32, (64, 128), 0)
        l64 = lax.broadcasted_iota(jnp.int32, (64, 128), 1)
        obits = (jnp.where(r64 > l64, jnp.uint32(0xFFFF), jnp.uint32(0))
                 | jnp.where(r64 + 64 > l64, jnp.uint32(0xFFFF0000), jnp.uint32(0)))
        z8 = jnp.zeros((8, 128), u32)

        def nkeys(b):
            return min(b + 1, 3) if first else 3

        def stage1(u):
            b, g = divmod(u, NG)
            nk = nkeys(b)
            gb_ = g0 + b
            slot = g % 2
            ws = []
            for j in range(4):
                hh = 4 * g + j
                p0 = ((DH * hh) // 16) % 8
                qw = qT_s[b, 16 * hh:16 * hh + 16, :]
                parts = [z8] * 8
                parts[p0] = qw[0:8]
                parts[(p0 + 1) % 8] = qw[8:16]
                ws.append(jnp.concatenate(parts, axis=0))
            w = _unpack(jnp.concatenate(ws, axis=1))
            ln = slice(128 * g, 128 * g + 128)
            rows = []
            for i in range(8):
                if nk == 3:
                    rows.append(k_s[gb_ - 2, 8 * i:8 * i + 8, ln])
                rows.append(k_s[gb_, 8 * i:8 * i + 8, ln])
            if nk >= 2:
                rows.append(k_s[gb_ - 1, :, ln])
            s = jnp.dot(_unpack(jnp.concatenate(rows, axis=0)), w, preferred_element_type=f32)
            mx = None
            rs = 32 if nk == 3 else 16
            for i in range(8):
                old = dd < 16 * i
                old4 = jnp.concatenate([old] * 4, axis=1)
                if nk == 3:
                    sm = jnp.where(old4, s[rs * i:rs * i + 16], s[rs * i + 16:rs * i + 32])
                else:
                    sm = jnp.where(old4, -1e30, s[rs * i:rs * i + 16])
                s_s[slot, 16 * i:16 * i + 16, :] = sm
                mx = sm if mx is None else jnp.maximum(mx, sm)
            if nk >= 2:
                for i in range(8):
                    sm = s[8 * rs + 16 * i:8 * rs + 16 * i + 16]
                    s_s[slot, 128 + 16 * i:128 + 16 * i + 16, :] = sm
                    mx = jnp.maximum(mx, sm)
            st["m", u] = jnp.max(mx, axis=0, keepdims=True)

        def stage2(u):
            b, g = divmod(u, NG)
            m = st.pop(("m", u))
            nk = nkeys(b)
            gb_ = g0 + b
            slot = g % 2
            res = []
            for j in range(4):
                hh = 4 * g + j
                off = DH * hh - 16 * ((DH * hh) // 16)
                ln = slice(128 * j, 128 * j + 128)
                mj = m[:, ln]

                def pp(r0):
                    return _packi(jnp.exp2(s_s[slot, r0:r0 + 64, ln] - mj),
                                  jnp.exp2(s_s[slot, r0 + 64:r0 + 128, ln] - mj))
                pm = pp(0)
                if nk == 3:
                    pold = pm & obits
                    p = jnp.concatenate([pold, pm ^ pold, pp(128)], axis=0)
                    blks = [gb_ - 2, gb_, gb_ - 1]
                elif nk == 2:
                    p = jnp.concatenate([pm, pp(128)], axis=0)
                    blks = [gb_, gb_ - 1]
                else:
                    p = pm
                    blks = [gb_]
                vw = _unpack(jnp.concatenate([vT_s[bb, 16 * hh:16 * hh + 16, :] for bb in blks], axis=1))
                o = jnp.dot(vw, _unpack(p), preferred_element_type=f32)
                if off < 8:
                    l, o3 = o[24:32], o[0:24]
                else:
                    l, o3 = o[0:8], o[8:32]
                r = pl.reciprocal(l, approx=True)
                r = r * (2.0 - l * r)
                res.append([o3[8 * i:8 * i + 8] * r for i in range(3)])
            out = []
            for j in (0, 2):
                a_, b_ = res[j], res[j + 1]
                out += [a_[0], a_[1], jnp.where(lo4, a_[2], b_[0]), b_[1], b_[2]]
            oT_s[b, 80 * g:80 * g + 80, :] = jnp.concatenate(out, axis=0)
            if g == NG - 1:
                ob_s[64 * b:64 * b + 64, :] = _pack(oT_s[b].T)

        def wo_stage(r0, n):
            y = jnp.dot(_unpack(ob_s[r0 // 2:(r0 + n) // 2, :]), wo_v[...], preferred_element_type=f32)
            x = x_v[pl.ds(pl.multiple_of((step - 1) * T + r0, QB), n), :].astype(f32)
            x1 = x + modv(2) * y
            h2 = _ln(x1) * (1.0 + modv(4)) + modv(3)
            st["x1", r0] = x1
            st["y", r0] = _ln(h2).astype(bf16)

        def w1_stage(r0):
            b1 = b1_v[...].astype(f32).reshape(1, F)
            st["hh", r0] = _gelu(lax.dot_general(st["y", r0], w1t_v[...], NT, preferred_element_type=f32)
                                 + b1).astype(bf16)

        def w2_stage(r0, lo, n):
            b2 = b2_v[...].astype(f32).reshape(1, D)
            mo = jnp.dot(st["hh", r0][lo:lo + n], w2_v[...], preferred_element_type=f32) + b2
            o_ref[r0 + lo:r0 + lo + n, :] = (st["x1", r0][lo:lo + n] + modv(5) * mo).astype(o_ref.dtype)

        NU = 2 * NG
        if variant == "first":
            for n in ("c", "x0", "wq", "wm1", "wk", "wv"):
                cp(n).start()
            cp("wq").wait()
            wqT_s[...] = _pack(wq_v[...].astype(f32).T)
            cp("c").wait()
            cp("x0").wait()
            ln1()
            for n in ("x1", "wo", "wm2"):
                cp(n).start()
            qproj()
            cp("wk").wait()
            cp("wv").wait()
            for n in ("b1", "b2", "w1", "w2", "xr"):
                cp(n).start()
            kproj()
            wvT_s[...] = _pack(wv_v[...].astype(f32).T)
            stage1(0)
            vproj()
            for u in range(NU):
                if u + 1 < NU:
                    stage1(u + 1)
                stage2(u)
            cp("x1").wait()
            cp("wo").wait()
            cp("wm2").wait()
            mod_s[:, 2 * D:6 * D] = jnp.dot(silu_c(), wm2_v[...], preferred_element_type=f32)[0:8]
        elif variant in ("second", "mid"):
            ln1()
            wo_stage(0, T)
            kproj()
            qproj()
            vproj()
            stage1(0)
            for u in range(NU):
                if u == NU - 2:
                    if variant == "second":
                        for n in ("b1", "b2", "w1", "w2", "xr"):
                            cp(n).wait()
                    w1_stage(0)
                if u + 1 < NU:
                    stage1(u + 1)
                else:
                    w2_stage(0, 0, QB)
                stage2(u)
            w2_stage(0, QB, QB)
        else:
            wo_stage(0, QB)
            wo_stage(QB, QB)
            w1_stage(0)
            w1_stage(QB)
            w2_stage(0, 0, QB)
            w2_stage(QB, 0, QB)

    @pl.when(step == 0)
    def _():
        body("first")

    @pl.when(step == 1)
    def _():
        body("second")

    @pl.when((step > 1) & (step < NS))
    def _():
        body("mid")

    @pl.when(step == NS)
    def _():
        body("last")


@jax.jit
def pallas_adaLN_cond__sliding_block__mixer_channel_mlp__prompt_kernel(A_x, A_wqkv, A_wo, B_x, B_w1, B_b1, B_w2, B_b2, c, w_mod):
    anyspec = pl.BlockSpec(memory_space=pl.ANY)
    return pl.pallas_call(
        kernel,
        grid=(NS + 1,),
        in_specs=[anyspec] * 9,
        out_specs=pl.BlockSpec((None, T, D), lambda i: (0, jnp.maximum(i - 1, 0), 0)),
        out_shape=jax.ShapeDtypeStruct((1, S, D), bf16),
        scratch_shapes=[
            pltpu.VMEM((S, D), bf16),
            pltpu.VMEM((1, D), bf16),
            pltpu.VMEM((F,), bf16),
            pltpu.VMEM((D,), bf16),
            pltpu.VMEM((D, D), bf16),
            pltpu.VMEM((D, D), bf16),
            pltpu.VMEM((D, D), bf16),
            pltpu.VMEM((D, D), bf16),
            pltpu.VMEM((F, D), bf16),
            pltpu.VMEM((F, D), bf16),
            pltpu.VMEM((D, 2 * D), bf16),
            pltpu.VMEM((D, 4 * D), bf16),
            pltpu.SemaphoreType.DMA((14,)),
            pltpu.VMEM((8, 6 * D), f32),
            pltpu.VMEM((D // 2, D), u32),
            pltpu.VMEM((D // 2, D), u32),
            pltpu.VMEM((NB, QB // 2, 128 * NG), u32),
            pltpu.VMEM((NB, 16 * H, QB), u32),
            pltpu.VMEM((T // QB, 16 * H, QB), u32),
            pltpu.VMEM((T // QB, D, QB), f32),
            pltpu.VMEM((2, 256, 512), f32),
            pltpu.VMEM((T // 2, D), u32),
        ],
        compiler_params=pltpu.CompilerParams(
            dimension_semantics=("arbitrary",),
            vmem_limit_bytes=100 * 1024 * 1024,
        ),
    )(A_x, c, B_b1, B_b2, A_wqkv, A_wo, B_w1.T, B_w2, w_mod)
```

```python
import functools
import jax
import jax.numpy as jnp
from jax import lax
import jax.experimental.pallas as pl
import jax.experimental.pallas.tpu as pltpu

S, D, H, DH, WIN, F = 2048, 640, 32, 20, 256, 1728
T = 256
QB = 128
NB = S // QB
NS = S // T
NG = 8
CH = 16
EPS = 1e-5
LOG2E = 1.4426950408889634
QSCALE = DH ** -0.5 * LOG2E
f32, bf16, u32 = jnp.float32, jnp.bfloat16, jnp.uint32
NT = (((1,), (1,)), ((), ()))


def _ln(x):
    m = jnp.mean(x, axis=-1, keepdims=True)
    xc = x - m
    v = jnp.mean(xc * xc, axis=-1, keepdims=True)
    return xc * lax.rsqrt(v + EPS)


def _pack(x):
    return pltpu.bitcast(x.astype(bf16), u32)


def _packi(a, b):
    return pltpu.bitcast(pltpu.pack_elementwise([a, b], packed_dtype=bf16), u32)


def _unpack(x):
    return pltpu.bitcast(x, bf16)


def _gelu(x):
    c = 0.7978845608028654
    return 0.5 * x * (1.0 + jnp.tanh(x * (c + (c * 0.044715) * (x * x))))


def kernel(x_h, c_h, b1_h, b2_h, wqkv_h, wo_h, w1t_h, w2_h, wmod_h, o_ref,
           x_v, c_v, b1_v, b2_v, wq_v, wk_v, wv_v, wo_v, w1t_v, w2_v, wm1_v, wm2_v, sems,
           mod_s, wqT_s, wvT_s, k_s, vT_s, qT_s, oT_s, s_s, ob_s, hb_s, hi_s, x1_s, y_s, hh_s):
    step = pl.program_id(0)

    pairs = dict(
        c=(c_h, c_v), x0=(x_h.at[0, 0:T], x_v.at[0:T]),
        wq=(wqkv_h.at[:, 0:D], wq_v), wm1=(wmod_h.at[:, 0:2 * D], wm1_v),
        wk=(wqkv_h.at[:, D:2 * D], wk_v), wv=(wqkv_h.at[:, 2 * D:3 * D], wv_v),
        x1=(x_h.at[0, T:2 * T], x_v.at[T:2 * T]),
        wo=(wo_h, wo_v), wm2=(wmod_h.at[:, 2 * D:6 * D], wm2_v),
        b1=(b1_h, b1_v), b2=(b2_h, b2_v), w1=(w1t_h, w1t_v), w2=(w2_h, w2_v),
        xr=(x_h.at[0, 2 * T:S], x_v.at[2 * T:S]),
    )
    names = list(pairs)

    def cp(n):
        s, d = pairs[n]
        return pltpu.make_async_copy(s, d, sems.at[names.index(n)])

    def silu_c():
        c = c_v[...].astype(f32)
        return jnp.broadcast_to((c * jax.nn.sigmoid(c)).astype(bf16), (16, D))

    def modv(i):
        return mod_s[0:1, i * D:(i + 1) * D]

    def body(variant):
        first = variant == "first"
        do_a = variant != "last"
        do_m = variant != "first"
        g0 = step * (T // QB)
        row8 = lax.broadcasted_iota(jnp.int32, (8, QB), 0)
        lo4 = row8 < 4
        st = {}

        def ln1_chunk(c):
            x = x_v[pl.ds(pl.multiple_of(step * T + CH * c, CH), CH), :].astype(f32)
            h = _ln(x) * (1.0 + modv(1)) + modv(0)
            hb_s[CH // 2 * c:CH // 2 * (c + 1), :] = _pack(h)
            hi_s[CH // 2 * c:CH // 2 * (c + 1), :] = jnp.concatenate(
                [_packi(h[16 * i:16 * i + 8], h[16 * i + 8:16 * i + 16]) for i in range(CH // 16)], axis=0)

        def ln1():
            if first:
                cp("wm1").wait()
                mod_s[:, 0:2 * D] = jnp.dot(silu_c(), wm1_v[...], preferred_element_type=f32)[0:8]
            for c in range(T // CH):
                ln1_chunk(c)

        def kproj():
            kf = jnp.dot(_unpack(hb_s[...]), wk_v[...], preferred_element_type=f32)
            lane = lax.broadcasted_iota(jnp.int32, (QB, 128), 1)
            for b in range(T // QB):
                kb = kf[QB * b:QB * b + QB]
                tiles = []
                for g in range(NG):
                    t0, t1 = (80 * g) // 128, (80 * g + 79) // 128
                    if t0 == t1:
                        tiles.append(kb[:, 128 * t0:128 * t0 + 128])
                    else:
                        tiles.append(jnp.where(lane >= 64, kb[:, 128 * t0:128 * t0 + 128],
                                               kb[:, 128 * t1:128 * t1 + 128]))
                k_s[g0 + b] = _pack(jnp.concatenate(tiles, axis=1))

        def windows(src, fill):
            fl = jnp.full((8, QB), fill, f32)
            out = []
            for hh in range(H):
                a = (DH * hh) // 16
                off = DH * hh - 16 * a
                v = [src[16 * a + 8 * i:16 * a + 8 * i + 8] for i in range(4)]
                if off == 0:
                    out += [v[0], v[1], jnp.where(lo4, v[2], fl), fl]
                elif off == 4:
                    out += [jnp.where(lo4, fl, v[0]), v[1], v[2], fl]
                elif off == 8:
                    out += [fl, v[1], v[2], jnp.where(lo4, v[3], fl)]
                else:
                    out += [fl, jnp.where(lo4, fl, v[1]), v[2], v[3]]
            return jnp.concatenate(out, axis=0)

        def qproj():
            qf = lax.dot_general(_unpack(wqT_s[...]), _unpack(hb_s[...]), NT, preferred_element_type=f32) * QSCALE
            for b in range(T // QB):
                qT_s[b] = _pack(qf[:, QB * b:QB * b + QB])

        def vproj():
            vf = lax.dot_general(_unpack(wvT_s[...]), _unpack(hi_s[...]), NT, preferred_element_type=f32)
            for b in range(T // QB):
                vT_s[g0 + b] = _pack(windows(vf[:, QB * b:QB * b + QB], 1.0))

        dd = (lax.broadcasted_iota(jnp.int32, (16, 128), 1)
              - lax.broadcasted_iota(jnp.int32, (16, 128), 0))
        r64 = lax.broadcasted_iota(jnp.int32, (64, 128), 0)
        l64 = lax.broadcasted_iota(jnp.int32, (64, 128), 1)
        r64 = r64 + (r64 & ~7)
        obits = (jnp.where(r64 > l64, jnp.uint32(0xFFFF), jnp.uint32(0))
                 | jnp.where(r64 + 8 > l64, jnp.uint32(0xFFFF0000), jnp.uint32(0)))
        z8 = jnp.zeros((8, 128), u32)

        def nkeys(b):
            return min(b + 1, 3) if first else 3

        lane8 = lax.broadcasted_iota(jnp.int32, (8, 128), 1)
        lane16 = lax.broadcasted_iota(jnp.int32, (16, 128), 1)
        g_lo = (lane16 & 32) != 0
        g_hi = lane16 >= 64
        r40 = lax.broadcasted_iota(jnp.int32, (40, 128), 0)
        hrow = (r40 >= 10).astype(jnp.int32) + (r40 >= 20).astype(jnp.int32) + (r40 >= 30).astype(jnp.int32)
        hx = hrow ^ (lax.broadcasted_iota(jnp.int32, (40, 128), 1) >> 5)

        def place(g, vs):
            parts = [z8] * 8
            for i, v in vs.items():
                parts[(5 * g + i) % 8] = v
            return jnp.concatenate(parts, axis=0)

        def stage1(u):
            b, g = divmod(u, NG)
            nk = nkeys(b)
            gb_ = g0 + b
            slot = g % 2
            q5 = qT_s[b, 40 * g:40 * g + 40, :]
            ws = []
            for j in range(4):
                qm = jnp.where(hrow[8 * j:8 * j + 16] == j, q5[8 * j:8 * j + 16], jnp.uint32(0))
                ws.append(place(g, {j: qm[0:8], j + 1: qm[8:16]}))
            w = _unpack(jnp.concatenate(ws, axis=1))
            ln = slice(128 * g, 128 * g + 128)
            mx = [None]

            def emit(r0, sm):
                s_s[slot, r0:r0 + 16, :] = sm
                mx[0] = sm if mx[0] is None else jnp.maximum(mx[0], sm)

            if nk < 3:
                rows = [k_s[gb_, :, ln]]
                if nk == 2:
                    rows.append(k_s[gb_ - 1, :, ln])
                s = jnp.dot(_unpack(jnp.concatenate(rows, axis=0)), w, preferred_element_type=f32)
                for i in range(8):
                    old4 = jnp.concatenate([dd < 16 * i] * 4, axis=1)
                    emit(16 * i, jnp.where(old4, -1e30, s[16 * i:16 * i + 16]))
                for i in range(8, 8 * nk):
                    emit(16 * i, s[16 * i:16 * i + 16])
            else:
                def kb(B):
                    return k_s[gb_ - 2 + B // 4, 16 * (B % 4):16 * (B % 4) + 16, ln]
                fl = (lane16 - (80 * g) % 128) & 127
                h_hi = fl >= 40
                h_lo = ((fl >= 20) & (fl < 40)) | (fl >= 60)
                x = [kb(0), kb(1), kb(2), kb(11)]
                t = [jnp.where(h_lo, x[v ^ 1], x[v]) for v in range(4)]
                e_l = [jnp.where(h_hi, t[v ^ 2], t[v]) for v in range(4)]
                k9, k10 = kb(9), kb(10)
                j2_l = [jnp.where(h_hi, k10, x[2]), jnp.where(h_hi, x[2], k10)]
                sm = []
                for v in range(4):
                    j1_l = jnp.where((fl >= 20 * v) & (fl < 20 * v + 20), x[1], k9)
                    lhs = jnp.concatenate([e_l[v][0:8], j1_l[0:8], j2_l[v // 2][0:8],
                                           e_l[v][8:16], j1_l[8:16], j2_l[v // 2][8:16]], axis=0)
                    qm = jnp.where(hx == v, q5, jnp.uint32(0))
                    wv = place(g, {i: qm[8 * i:8 * i + 8] for i in range(5)})
                    sm.append(jnp.dot(_unpack(lhs), _unpack(wv), preferred_element_type=f32))
                for c in range(2):
                    for J in (1, 2):
                        msk = (dd < 32 * J + 16 * c) & (lane16 >= 32 * J)
                        uu = [jnp.where(msk, sm[v][48 * c:48 * c + 16], sm[v][48 * c + 16 * J:48 * c + 16 * J + 16])
                              for v in range(4)]
                        t = [jnp.where(g_lo, uu[v ^ 1], uu[v]) for v in range(4)]
                        emit(32 * J + 16 * c,
                             jnp.concatenate([jnp.where(g_hi, t[v ^ 2], t[v]) for v in range(4)], axis=1))
                k8, k3 = kb(8), kb(3)
                lhs = jnp.concatenate([k8[0:8], k3[0:8], k8[8:16], k3[8:16], k_s[gb_ - 1, :, ln]], axis=0)
                s = jnp.dot(_unpack(lhs), w, preferred_element_type=f32)
                for c in range(2):
                    e0 = jnp.concatenate([sm[v][48 * c:48 * c + 16] for v in range(4)], axis=1)
                    e3 = jnp.concatenate([sm[v ^ 3][48 * c:48 * c + 16] for v in range(4)], axis=1)
                    old4 = jnp.concatenate([dd < 16 * c] * 4, axis=1)
                    emit(16 * c, jnp.where(old4, e0, s[32 * c:32 * c + 16]))
                    old4 = jnp.concatenate([dd < 96 + 16 * c] * 4, axis=1)
                    emit(96 + 16 * c, jnp.where(old4, s[32 * c + 16:32 * c + 32], e3))
                for i in range(8):
                    emit(128 + 16 * i, s[64 + 16 * i:64 + 16 * i + 16])
            st["m", u] = jnp.max(mx[0], axis=0, keepdims=True)

        def stage2(u):
            b, g = divmod(u, NG)
            m = st.pop(("m", u))
            nk = nkeys(b)
            gb_ = g0 + b
            slot = g % 2
            res = []
            for j in range(4):
                hh = 4 * g + j
                off = DH * hh - 16 * ((DH * hh) // 16)
                ln = slice(128 * j, 128 * j + 128)
                mj = m[:, ln]

                def pp(r0):
                    e = jnp.exp2(s_s[slot, r0:r0 + 128, ln] - mj)
                    return jnp.concatenate(
                        [_packi(e[16 * i:16 * i + 8], e[16 * i + 8:16 * i + 16]) for i in range(8)], axis=0)
                pm = pp(0)
                if nk == 3:
                    pold = pm & obits
                    p = jnp.concatenate([pold, pm ^ pold, pp(128)], axis=0)
                    blks = [gb_ - 2, gb_, gb_ - 1]
                elif nk == 2:
                    p = jnp.concatenate([pm, pp(128)], axis=0)
                    blks = [gb_, gb_ - 1]
                else:
                    p = pm
                    blks = [gb_]
                vw = _unpack(jnp.concatenate([vT_s[bb, 16 * hh:16 * hh + 16, :] for bb in blks], axis=1))
                o = jnp.dot(vw, _unpack(p), preferred_element_type=f32)
                if off < 8:
                    l, o3 = o[24:32], o[0:24]
                else:
                    l, o3 = o[0:8], o[8:32]
                r = pl.reciprocal(l, approx=True)
                r = r * (2.0 - l * r)
                res.append([o3[8 * i:8 * i + 8] * r for i in range(3)])
            out = []
            for j in (0, 2):
                a_, b_ = res[j], res[j + 1]
                out += [a_[0], a_[1], jnp.where(lo4, a_[2], b_[0]), b_[1], b_[2]]
            oT_s[b, 80 * g:80 * g + 80, :] = jnp.concatenate(out, axis=0)
            if g == NG - 1:
                ob_s[64 * b:64 * b + 64, :] = _pack(oT_s[b].T)

        def wo_stage(r0, n):
            y = jnp.dot(_unpack(ob_s[r0 // 2:(r0 + n) // 2, :]), wo_v[...], preferred_element_type=f32)
            x = x_v[pl.ds(pl.multiple_of((step - 1) * T + r0, QB), n), :].astype(f32)
            x1_s[r0:r0 + n, :] = x + modv(2) * y

        def ln23_chunk(c):
            h2 = _ln(x1_s[CH * c:CH * (c + 1), :]) * (1.0 + modv(4)) + modv(3)
            y_s[CH // 2 * c:CH // 2 * (c + 1), :] = _pack(_ln(h2))

        def w1_stage(r0, n):
            b1 = b1_v[...].astype(f32).reshape(1, F)
            hh_s[r0 // 2:(r0 + n) // 2, :] = _pack(_gelu(
                lax.dot_general(_unpack(y_s[r0 // 2:(r0 + n) // 2, :]), w1t_v[...], NT,
                                preferred_element_type=f32) + b1))

        def w2_stage(r0, n):
            b2 = b2_v[...].astype(f32).reshape(1, D)
            mo = jnp.dot(_unpack(hh_s[r0 // 2:(r0 + n) // 2, :]), w2_v[...], preferred_element_type=f32) + b2
            o_ref[r0:r0 + n, :] = (x1_s[r0:r0 + n, :] + modv(5) * mo).astype(o_ref.dtype)

        NU = 2 * NG
        if variant == "first":
            for n in ("c", "x0", "wq", "wm1", "wk", "wv"):
                cp(n).start()
            cp("wq").wait()
            wqT_s[...] = _pack(wq_v[...].astype(f32).T)
            cp("c").wait()
            cp("x0").wait()
            ln1()
            for n in ("x1", "wo", "wm2"):
                cp(n).start()
            qproj()
            cp("wk").wait()
            cp("wv").wait()
            for n in ("b1", "b2", "w1", "w2", "xr"):
                cp(n).start()
            kproj()
            wvT_s[...] = _pack(wv_v[...].astype(f32).T)
            stage1(0)
            vproj()
            for u in range(NU):
                if u + 1 < NU:
                    stage1(u + 1)
                stage2(u)
            cp("x1").wait()
            cp("wo").wait()
            cp("wm2").wait()
            mod_s[:, 2 * D:6 * D] = jnp.dot(silu_c(), wm2_v[...], preferred_element_type=f32)[0:8]
        elif variant in ("second", "mid"):
            ln1()
            wo_stage(0, T)
            kproj()
            qproj()
            vproj()
            stage1(0)
            for u in range(NU):
                if u < 8:
                    for c in range(T // CH // 8 * u, T // CH // 8 * (u + 1)):
                        ln23_chunk(c)
                if u == NU - 2:
                    if variant == "second":
                        for n in ("b1", "b2", "w1", "w2", "xr"):
                            cp(n).wait()
                    w1_stage(0, T)
                if u + 1 < NU:
                    stage1(u + 1)
                else:
                    w2_stage(0, QB)
                stage2(u)
            w2_stage(QB, QB)
        else:
            wo_stage(0, QB)
            for c in range(QB // CH):
                ln23_chunk(c)
            wo_stage(QB, QB)
            for c in range(QB // CH, T // CH):
                ln23_chunk(c)
            w1_stage(0, QB)
            w1_stage(QB, QB)
            w2_stage(0, QB)
            w2_stage(QB, QB)

    @pl.when(step == 0)
    def _():
        with jax.named_scope("sc_first"):
            body("first")

    @pl.when(step == 1)
    def _():
        with jax.named_scope("sc_second"):
            body("second")

    @pl.when((step > 1) & (step < NS))
    def _():
        with jax.named_scope("sc_mid"):
            body("mid")

    @pl.when(step == NS)
    def _():
        with jax.named_scope("sc_last"):
            body("last")


@jax.jit
def pallas_adaLN_cond__sliding_block__mixer_channel_mlp__prompt_kernel(A_x, A_wqkv, A_wo, B_x, B_w1, B_b1, B_w2, B_b2, c, w_mod):
    anyspec = pl.BlockSpec(memory_space=pl.ANY)
    return pl.pallas_call(
        kernel,
        grid=(NS + 1,),
        in_specs=[anyspec] * 9,
        out_specs=pl.BlockSpec((None, T, D), lambda i: (0, jnp.maximum(i - 1, 0), 0)),
        out_shape=jax.ShapeDtypeStruct((1, S, D), bf16),
        scratch_shapes=[
            pltpu.VMEM((S, D), bf16),
            pltpu.VMEM((1, D), bf16),
            pltpu.VMEM((F,), bf16),
            pltpu.VMEM((D,), bf16),
            pltpu.VMEM((D, D), bf16),
            pltpu.VMEM((D, D), bf16),
            pltpu.VMEM((D, D), bf16),
            pltpu.VMEM((D, D), bf16),
            pltpu.VMEM((F, D), bf16),
            pltpu.VMEM((F, D), bf16),
            pltpu.VMEM((D, 2 * D), bf16),
            pltpu.VMEM((D, 4 * D), bf16),
            pltpu.SemaphoreType.DMA((14,)),
            pltpu.VMEM((8, 6 * D), f32),
            pltpu.VMEM((D // 2, D), u32),
            pltpu.VMEM((D // 2, D), u32),
            pltpu.VMEM((NB, QB // 2, 128 * NG), u32),
            pltpu.VMEM((NB, 16 * H, QB), u32),
            pltpu.VMEM((T // QB, D // 2, QB), u32),
            pltpu.VMEM((T // QB, D, QB), f32),
            pltpu.VMEM((2, 256, 512), f32),
            pltpu.VMEM((T // 2, D), u32),
            pltpu.VMEM((T // 2, D), u32),
            pltpu.VMEM((T // 2, D), u32),
            pltpu.VMEM((T, D), f32),
            pltpu.VMEM((T // 2, D), u32),
            pltpu.VMEM((T // 2, F), u32),
        ],
        compiler_params=pltpu.CompilerParams(
            dimension_semantics=("arbitrary",),
            vmem_limit_bytes=100 * 1024 * 1024,
        ),
    )(A_x, c, B_b1, B_b2, A_wqkv, A_wo, B_w1.T, B_w2, w_mod)
```

```python
import os
import jax
import jax.numpy as jnp
from jax import lax
import jax.experimental.pallas as pl
import jax.experimental.pallas.tpu as pltpu

S, D, H, DH, WIN, F = 2048, 640, 32, 20, 256, 1728
T = 256
QB = 128
NB = S // QB
NS = S // T
NG = 8
NU = 2 * NG
CH = 16
EPS = 1e-5
LOG2E = 1.4426950408889634
QSCALE = DH ** -0.5 * LOG2E
f32, bf16, u32 = jnp.float32, jnp.bfloat16, jnp.uint32
NT = (((1,), (1,)), ((), ()))

LN1_AT = os.environ.get("LN1_AT", "attn")
LN23_AT = os.environ.get("LN23_AT", "proj")
K1 = int(os.environ.get("K1", "3"))
K2 = int(os.environ.get("K2", "3"))
RL1 = os.environ.get("RL1", "0") == "1"
RL2 = os.environ.get("RL2", "0") == "1"
MW = int(os.environ.get("MW", "8"))
SCOPES = os.environ.get("SCOPES", "0") == "1"


def _ln(x):
    m = jnp.sum(x, axis=-1, keepdims=True) * (1.0 / D)
    xc = x - m
    v = jnp.sum(xc * xc, axis=-1, keepdims=True) * (1.0 / D)
    return xc * lax.rsqrt(v + EPS)


def _stats(x):
    m = jnp.sum(x, axis=-1, keepdims=True) * (1.0 / D)
    v = jnp.sum(x * x, axis=-1, keepdims=True) * (1.0 / D) - m * m
    return m, lax.rsqrt(jnp.maximum(v, 0.0) + EPS)


def _pack(x):
    return pltpu.bitcast(x.astype(bf16), u32)


def _packi(x):
    n = x.shape[0] // 16
    return jnp.concatenate(
        [pltpu.bitcast(pltpu.pack_elementwise([x[16 * i:16 * i + 8], x[16 * i + 8:16 * i + 16]],
                                              packed_dtype=bf16), u32) for i in range(n)], axis=0)


def _unpack(x):
    return pltpu.bitcast(x, bf16)


def _gelu(x):
    c = 0.7978845608028654
    return 0.5 * x * (1.0 + jnp.tanh(x * (c + (c * 0.044715) * (x * x))))


class _Null:
    def __enter__(self):
        return None

    def __exit__(self, *a):
        return False


def ns(name):
    return jax.named_scope(name) if SCOPES else _Null()


def kernel(x_h, c_h, b1_h, b2_h, wqkv_h, wo_h, w1t_h, w2_h, wmod_h, o_h,
           x_v, c_v, b1_v, b2_v, wq_v, wk_v, wv_v, wo_v, w1t_v, w2_v, wm1_v, wm2_v, wm3_v, sems,
           mod_s, wqT_s, wvT_s, k_s, vT_s, qT_s, oT_s, s_s, ob_s, hb_s, hi_s, x1_s, y_s, hh_s, h2_s, o_v, osem, col_s):
    step = pl.program_id(0)

    pairs = dict(
        c=(c_h, c_v), x0=(x_h.at[0, 0:T], x_v.at[0:T]),
        wm1=(wmod_h.at[:, 0:2 * D], wm1_v),
        wk=(wqkv_h.at[:, D:2 * D], wk_v), wq=(wqkv_h.at[:, 0:D], wq_v),
        x1=(x_h.at[0, T:2 * T], x_v.at[T:2 * T]),
        wv=(wqkv_h.at[:, 2 * D:3 * D], wv_v),
        wm2=(wmod_h.at[:, 2 * D:5 * D], wm2_v), wo=(wo_h, wo_v),
        x2=(x_h.at[0, 2 * T:3 * T], x_v.at[2 * T:3 * T]),
        wm3=(wmod_h.at[:, 5 * D:6 * D], wm3_v),
        b1=(b1_h, b1_v), b2=(b2_h, b2_v), w1=(w1t_h, w1t_v), w2=(w2_h, w2_v),
        xr=(x_h.at[0, 3 * T:S], x_v.at[3 * T:S]),
    )
    names = list(pairs)

    def cp(n):
        s, d = pairs[n]
        return pltpu.make_async_copy(s, d, sems.at[names.index(n)])

    def wait(*ns_):
        with ns("w_" + ns_[-1]):
            for n in ns_:
                cp(n).wait()

    def silu_c():
        c = c_v[...].astype(f32)
        return c * jax.nn.sigmoid(c)

    def modv(i, n):
        v = mod_s[:, i * D:(i + 1) * D]
        return jnp.concatenate([v] * (n // 8), axis=0)

    def mod_store(r, lo, hi):
        for i in range(lo, hi):
            v = r[:, (i - lo) * D:(i - lo + 1) * D]
            mod_s[:, i * D:(i + 1) * D] = v + 1.0 if i in (1, 4) else v

    def mod_mxu(w_v, lo, hi):
        sc = jnp.broadcast_to(silu_c().astype(bf16), (16, D))
        mod_store(jnp.dot(sc, w_v[...], preferred_element_type=f32)[0:8], lo, hi)

    def mod_vpu(w_v, lo, hi):
        never = (step >> 10) == 1
        outs = []
        acc = jnp.zeros((MW, 128), f32)
        for t in range((hi - lo) * D // 128):
            acc = jnp.where(never, acc, 0.0)
            for r in range(D // MW):
                rows = slice(MW * r, MW * r + MW)
                acc = acc + w_v[rows, 128 * t:128 * t + 128].astype(f32) * col_s[rows, :]
            outs.append(jnp.broadcast_to(jnp.sum(acc, axis=0, keepdims=True), (8, 128)))
        mod_store(jnp.concatenate(outs, axis=1), lo, hi)

    def body(variant):
        first = variant == "first"
        g0 = step * (T // QB)
        row8 = lax.broadcasted_iota(jnp.int32, (8, QB), 0)
        lo4 = row8 < 4
        st = {}
        dyn0 = step >> 10

        def anchor_x1(v):
            x1_s[pl.ds(pl.multiple_of(T + 8 * dyn0, 8), 8), 0:128] = v

        def anchor_x(v):
            x_v[pl.ds(pl.multiple_of(S + 16 * dyn0, 16), 16), 0:128] = jnp.concatenate([v, v], axis=0).astype(bf16)

        def h_store(c, h):
            hb_s[CH // 2 * c:CH // 2 * (c + 1), :] = _pack(h)
            hi_s[CH // 2 * c:CH // 2 * (c + 1), :] = _packi(h)

        def ln1_chunk(c, blk):
            x = x_v[pl.ds(pl.multiple_of(blk * T + CH * c, CH), CH), :].astype(f32)
            m, r = _stats(x)
            if RL1:
                x = x_v[pl.ds(pl.multiple_of((blk + dyn0) * T + CH * c, CH), CH), :].astype(f32)
            h = (x - m) * r * modv(1, CH) + modv(0, CH)
            h_store(c, h)
            return h[0:8, 0:128]

        def chain(chunk_fn, anchor_fn, k, cs):
            outs = []
            for i, c in enumerate(cs):
                if i >= k:
                    anchor_fn(outs[i - k])
                outs.append(chunk_fn(c))

        def kproj():
            kf = jnp.dot(_unpack(hb_s[...]), wk_v[...], preferred_element_type=f32)
            lane = lax.broadcasted_iota(jnp.int32, (QB, 128), 1)
            for b in range(T // QB):
                kb = kf[QB * b:QB * b + QB]
                tiles = []
                for g in range(NG):
                    t0, t1 = (80 * g) // 128, (80 * g + 79) // 128
                    if t0 == t1:
                        tiles.append(kb[:, 128 * t0:128 * t0 + 128])
                    else:
                        tiles.append(jnp.where(lane >= 64, kb[:, 128 * t0:128 * t0 + 128],
                                               kb[:, 128 * t1:128 * t1 + 128]))
                k_s[g0 + b] = _pack(jnp.concatenate(tiles, axis=1))
            return kf

        def windows(src):
            fl = jnp.ones((8, QB), f32)
            out = []
            for hh in range(H):
                a = (DH * hh) // 16
                off = DH * hh - 16 * a
                v = [src[16 * a + 8 * i:16 * a + 8 * i + 8] for i in range(4)]
                if off == 0:
                    out += [v[0], v[1], jnp.where(lo4, v[2], fl), fl]
                elif off == 4:
                    out += [jnp.where(lo4, fl, v[0]), v[1], v[2], fl]
                elif off == 8:
                    out += [fl, v[1], v[2], jnp.where(lo4, v[3], fl)]
                else:
                    out += [fl, jnp.where(lo4, fl, v[1]), v[2], v[3]]
            return jnp.concatenate(out, axis=0)

        def qproj():
            if first:
                qf = (jnp.dot(_unpack(hb_s[...]), wq_v[...], preferred_element_type=f32) * QSCALE).T
            else:
                qf = lax.dot_general(_unpack(wqT_s[...]), _unpack(hb_s[...]), NT,
                                     preferred_element_type=f32) * QSCALE
            for b in range(T // QB):
                qT_s[b] = _pack(qf[:, QB * b:QB * b + QB])
            return qf

        def vproj():
            if first:
                vf = jnp.dot(_unpack(hi_s[...]), wv_v[...], preferred_element_type=f32).T
            else:
                vf = lax.dot_general(_unpack(wvT_s[...]), _unpack(hi_s[...]), NT, preferred_element_type=f32)
            for b in range(T // QB):
                vT_s[g0 + b] = _pack(windows(vf[:, QB * b:QB * b + QB]))
            return vf

        dd = (lax.broadcasted_iota(jnp.int32, (16, 128), 1)
              - lax.broadcasted_iota(jnp.int32, (16, 128), 0))
        r64 = lax.broadcasted_iota(jnp.int32, (64, 128), 0)
        l64 = lax.broadcasted_iota(jnp.int32, (64, 128), 1)
        r64 = r64 + (r64 & ~7)
        obits = (jnp.where(r64 > l64, jnp.uint32(0xFFFF), jnp.uint32(0))
                 | jnp.where(r64 + 8 > l64, jnp.uint32(0xFFFF0000), jnp.uint32(0)))
        z8 = jnp.zeros((8, 128), u32)
        lane16 = lax.broadcasted_iota(jnp.int32, (16, 128), 1)
        g_lo = (lane16 & 32) != 0
        g_hi = lane16 >= 64
        r40 = lax.broadcasted_iota(jnp.int32, (40, 128), 0)
        hrow = (r40 >= 10).astype(jnp.int32) + (r40 >= 20).astype(jnp.int32) + (r40 >= 30).astype(jnp.int32)
        hx = hrow ^ (lax.broadcasted_iota(jnp.int32, (40, 128), 1) >> 5)

        def nkeys(b):
            return min(b + 1, 3) if first else 3

        def place(g, vs):
            parts = [z8] * 8
            for i, v in vs.items():
                parts[(5 * g + i) % 8] = v
            return jnp.concatenate(parts, axis=0)

        def stage1(u, slot):
            b, g = divmod(u, NG)
            nk = nkeys(b)
            gb_ = g0 + b
            q5 = qT_s[b, 40 * g:40 * g + 40, :]
            ws = []
            for j in range(4):
                qm = jnp.where(hrow[8 * j:8 * j + 16] == j, q5[8 * j:8 * j + 16], jnp.uint32(0))
                ws.append(place(g, {j: qm[0:8], j + 1: qm[8:16]}))
            w = _unpack(jnp.concatenate(ws, axis=1))
            ln = slice(128 * g, 128 * g + 128)
            mx = [None]

            def emit(r0, sm):
                s_s[slot, r0:r0 + 16, :] = sm
                mx[0] = sm if mx[0] is None else jnp.maximum(mx[0], sm)

            if nk < 3:
                rows = [k_s[gb_, :, ln]]
                if nk == 2:
                    rows.append(k_s[gb_ - 1, :, ln])
                s = jnp.dot(_unpack(jnp.concatenate(rows, axis=0)), w, preferred_element_type=f32)
                for i in range(8):
                    old4 = jnp.concatenate([dd < 16 * i] * 4, axis=1)
                    emit(16 * i, jnp.where(old4, -1e30, s[16 * i:16 * i + 16]))
                for i in range(8, 8 * nk):
                    emit(16 * i, s[16 * i:16 * i + 16])
            else:
                def kb(B):
                    return k_s[gb_ - 2 + B // 4, 16 * (B % 4):16 * (B % 4) + 16, ln]
                fl = (lane16 - (80 * g) % 128) & 127
                h_hi = fl >= 40
                h_lo = ((fl >= 20) & (fl < 40)) | (fl >= 60)
                x = [kb(0), kb(1), kb(2), kb(11)]
                t = [jnp.where(h_lo, x[v ^ 1], x[v]) for v in range(4)]
                e_l = [jnp.where(h_hi, t[v ^ 2], t[v]) for v in range(4)]
                k9, k10 = kb(9), kb(10)
                j2_l = [jnp.where(h_hi, k10, x[2]), jnp.where(h_hi, x[2], k10)]
                sm = []
                for v in range(4):
                    j1_l = jnp.where((fl >= 20 * v) & (fl < 20 * v + 20), x[1], k9)
                    lhs = jnp.concatenate([e_l[v][0:8], j1_l[0:8], j2_l[v // 2][0:8],
                                           e_l[v][8:16], j1_l[8:16], j2_l[v // 2][8:16]], axis=0)
                    qm = jnp.where(hx == v, q5, jnp.uint32(0))
                    wv = place(g, {i: qm[8 * i:8 * i + 8] for i in range(5)})
                    sm.append(jnp.dot(_unpack(lhs), _unpack(wv), preferred_element_type=f32))
                for c in range(2):
                    for J in (1, 2):
                        msk = (dd < 32 * J + 16 * c) & (lane16 >= 32 * J)
                        uu = [jnp.where(msk, sm[v][48 * c:48 * c + 16], sm[v][48 * c + 16 * J:48 * c + 16 * J + 16])
                              for v in range(4)]
                        t = [jnp.where(g_lo, uu[v ^ 1], uu[v]) for v in range(4)]
                        emit(32 * J + 16 * c,
                             jnp.concatenate([jnp.where(g_hi, t[v ^ 2], t[v]) for v in range(4)], axis=1))
                k8, k3 = kb(8), kb(3)
                lhs = jnp.concatenate([k8[0:8], k3[0:8], k8[8:16], k3[8:16], k_s[gb_ - 1, :, ln]], axis=0)
                s = jnp.dot(_unpack(lhs), w, preferred_element_type=f32)
                for c in range(2):
                    e0 = jnp.concatenate([sm[v][48 * c:48 * c + 16] for v in range(4)], axis=1)
                    e3 = jnp.concatenate([sm[v ^ 3][48 * c:48 * c + 16] for v in range(4)], axis=1)
                    old4 = jnp.concatenate([dd < 16 * c] * 4, axis=1)
                    emit(16 * c, jnp.where(old4, e0, s[32 * c:32 * c + 16]))
                    old4 = jnp.concatenate([dd < 96 + 16 * c] * 4, axis=1)
                    emit(96 + 16 * c, jnp.where(old4, s[32 * c + 16:32 * c + 32], e3))
                for i in range(8):
                    emit(128 + 16 * i, s[64 + 16 * i:64 + 16 * i + 16])
            st["m", u] = (jnp.max(mx[0], axis=0, keepdims=True), slot)
            return mx[0][0:8, 0:128]

        def stage2(u):
            b, g = divmod(u, NG)
            m, slot = st.pop(("m", u))
            nk = nkeys(b)
            gb_ = g0 + b
            res = []
            for j in range(4):
                hh = 4 * g + j
                off = DH * hh - 16 * ((DH * hh) // 16)
                ln = slice(128 * j, 128 * j + 128)
                mj = m[:, ln]

                def pp(r0):
                    return _packi(jnp.exp2(s_s[slot, r0:r0 + 128, ln] - mj))
                pm = pp(0)
                if nk == 3:
                    pold = pm & obits
                    p = jnp.concatenate([pold, pm ^ pold, pp(128)], axis=0)
                    blks = [gb_ - 2, gb_, gb_ - 1]
                elif nk == 2:
                    p = jnp.concatenate([pm, pp(128)], axis=0)
                    blks = [gb_, gb_ - 1]
                else:
                    p = pm
                    blks = [gb_]
                vw = _unpack(jnp.concatenate([vT_s[bb, 16 * hh:16 * hh + 16, :] for bb in blks], axis=1))
                o = jnp.dot(vw, _unpack(p), preferred_element_type=f32)
                if off < 8:
                    l, o3 = o[24:32], o[0:24]
                else:
                    l, o3 = o[0:8], o[8:32]
                r = pl.reciprocal(l, approx=True)
                r = r * (2.0 - l * r)
                res.append([o3[8 * i:8 * i + 8] * r for i in range(3)])
            out = []
            for j in (0, 2):
                a_, b_ = res[j], res[j + 1]
                out += [a_[0], a_[1], jnp.where(lo4, a_[2], b_[0]), b_[1], b_[2]]
            oT_s[b, 80 * g:80 * g + 80, :] = jnp.concatenate(out, axis=0)
            st["done", b] = st.get(("done", b), 0) + 1
            if st["done", b] == NG:
                ob_s[step % 2, 64 * b:64 * b + 64, :] = _pack(oT_s[b].T)
            return out[0]

        def wo_stage(r0, n):
            y = jnp.dot(_unpack(ob_s[(step + 1) % 2, r0 // 2:(r0 + n) // 2, :]), wo_v[...],
                        preferred_element_type=f32)
            x = x_v[pl.ds(pl.multiple_of((step - 1) * T + r0, QB), n), :].astype(f32)
            x1_s[r0:r0 + n, :] = x + modv(2, n) * y

        def ln23_chunk(c):
            x1 = x1_s[CH * c:CH * (c + 1), :]
            m, r = _stats(x1)
            if RL2:
                x1 = x1_s[pl.ds(pl.multiple_of(CH * (c + dyn0), CH), CH), :]
            h2 = (x1 - m) * r * modv(4, CH) + modv(3, CH)
            m, r = _stats(h2)
            if RL2:
                h2_s[c] = h2
                h2 = h2_s[c]
            y = (h2 - m) * r
            y_s[CH // 2 * c:CH // 2 * (c + 1), :] = _pack(y)
            return y[0:8, 0:128]

        def w1_stage(r0, n):
            b1 = b1_v[...].astype(f32).reshape(1, F)
            hh = _gelu(lax.dot_general(_unpack(y_s[r0 // 2:(r0 + n) // 2, :]), w1t_v[...], NT,
                                       preferred_element_type=f32) + b1)
            hh_s[r0 // 2:(r0 + n) // 2, :] = _pack(hh)
            return hh

        def w2_stage(r0, n):
            b2 = b2_v[...].astype(f32).reshape(1, D)
            mo = jnp.dot(_unpack(hh_s[r0 // 2:(r0 + n) // 2, :]), w2_v[...], preferred_element_type=f32) + b2
            rows = pl.ds(pl.multiple_of((step - 1) * T + r0, n), n)
            o_v[rows, :] = (x1_s[r0:r0 + n, :] + modv(5, n) * mo).astype(bf16)
            pltpu.make_async_copy(o_v.at[rows], o_h.at[0, rows], osem.at[0]).start()
            return mo

        nxt = jnp.minimum(step + 1, NS - 1)
        NCH = T // CH

        def spread(anchors, anchor_fn, chunk_fn):
            n = len(anchors)
            for i, a in enumerate(anchors):
                anchor_fn(a)
                for c in range(NCH * i // n, NCH * (i + 1) // n):
                    chunk_fn(c)

        if variant == "first":
            for n in names:
                cp(n).start()
            wait("c", "x0")
            with ns("ln1a"):
                col_s[...] = jnp.broadcast_to(silu_c().astype(bf16).astype(f32), (128, D)).T
                for c in range(NCH):
                    x1_s[CH * c:CH * (c + 1), :] = _ln(x_v[CH * c:CH * (c + 1), :].astype(f32))
            wait("wm1")
            with ns("mod1"):
                mod_mxu(wm1_v, 0, 2)
                for c in range(NCH):
                    h_store(c, x1_s[CH * c:CH * (c + 1), :] * modv(1, CH) + modv(0, CH))
            wait("wk")
            with ns("kproj"):
                kproj()
            wait("wq")
            order = [u for g in range(NG) for u in (NG + g, g)]
            with ns("qproj"):
                qproj()
                stage1(order[0], 0)
                stage1(order[1], 1)
            wait("x1", "wv")
            with ns("attn"):
                vproj()
                wqT_s[...] = _pack(wq_v[...].astype(f32).T)
                wvT_s[...] = _pack(wv_v[...].astype(f32).T)
                for i, u in enumerate(order):
                    if i + 2 < NU:
                        stage1(order[i + 2], (i + 2) % 3)
                    a2 = stage2(u)
                    if i < 8:
                        anchor_x(a2)
                        ln1_chunk(2 * i, 1)
                        ln1_chunk(2 * i + 1, 1)
            wait("wm2")
        elif variant in ("second", "mid"):
            second = variant == "second"
            if not second:
                wo_stage(0, T)
            if LN1_AT == "start" and not second:
                chain(lambda c: ln1_chunk(c, step), anchor_x, K1, range(NCH))
            if LN23_AT == "free" and not second:
                chain(ln23_chunk, anchor_x1, K2, range(NCH))
            if second:
                mod_vpu(wm2_v, 2, 5)
            kf = kproj()
            qf = qproj()
            vf = vproj()
            if LN23_AT == "proj" and not second:
                an = [kf[248:256, 128 * j:128 * j + 128] for j in range(1, 5)]
                an += [z[r:r + 8, 128 * b:128 * b + 128] for z in (qf, vf) for b in range(2) for r in (200, 400, 632)]
                spread(an, anchor_x1, ln23_chunk)
            if second:
                wait("wo", "x2")
                wo_stage(0, T)
            stage1(0, 0)
            u23 = 0
            for u in range(NU):
                if u == NU - 2:
                    if second:
                        wait("wm3", "b1", "b2", "w1", "w2")
                        mod_vpu(wm3_v, 5, 6)
                    hh = w1_stage(0, T)
                    if LN1_AT == "w1" or second:
                        spread([hh[r:r + 8, 128 * j:128 * j + 128] for j in range(8) for r in (0, 128)],
                               anchor_x, lambda c: ln1_chunk(c, nxt))
                if u + 1 < NU:
                    a1 = stage1(u + 1, (u + 1) % 2)
                else:
                    mo = w2_stage(0, QB)
                    if LN1_AT == "w2":
                        spread([mo[r:r + 8, 128 * j:128 * j + 128] for j in range(5) for r in (0, 120)],
                               anchor_x, lambda c: ln1_chunk(c, nxt))
                a2 = stage2(u)
                if (LN23_AT == "attn" or second) and u23 <= u < u23 + 8:
                    anchor_x1(a1)
                    ln23_chunk(2 * (u - u23))
                    anchor_x1(a2)
                    ln23_chunk(2 * (u - u23) + 1)
                if LN1_AT == "attn" and 4 <= u < 12 and not second:
                    anchor_x(a1)
                    ln1_chunk(2 * (u - 4), nxt)
                    anchor_x(a2)
                    ln1_chunk(2 * (u - 4) + 1, nxt)
            w2_stage(QB, QB)
            if second:
                wait("xr")
        else:
            wo_stage(0, QB)
            for c in range(QB // CH):
                ln23_chunk(c)
            wo_stage(QB, QB)
            for c in range(QB // CH, T // CH):
                ln23_chunk(c)
            w1_stage(0, QB)
            w1_stage(QB, QB)
            w2_stage(0, QB)
            w2_stage(QB, QB)
            pltpu.make_async_copy(o_v, o_h.at[0], osem.at[0]).wait()

    @pl.when(step == 0)
    def _():
        with jax.named_scope("sc_first"):
            body("first")

    @pl.when(step == 1)
    def _():
        with jax.named_scope("sc_second"):
            body("second")

    @pl.when((step > 1) & (step < NS))
    def _():
        with jax.named_scope("sc_mid"):
            body("mid")

    @pl.when(step == NS)
    def _():
        with jax.named_scope("sc_last"):
            body("last")


@jax.jit
def pallas_adaLN_cond__sliding_block__mixer_channel_mlp__prompt_kernel(A_x, A_wqkv, A_wo, B_x, B_w1, B_b1, B_w2, B_b2, c, w_mod):
    anyspec = pl.BlockSpec(memory_space=pl.ANY)
    return pl.pallas_call(
        kernel,
        grid=(NS + 1,),
        in_specs=[anyspec] * 9,
        out_specs=anyspec,
        out_shape=jax.ShapeDtypeStruct((1, S, D), bf16),
        scratch_shapes=[
            pltpu.VMEM((S + 16, D), bf16),
            pltpu.VMEM((1, D), bf16),
            pltpu.VMEM((F,), bf16),
            pltpu.VMEM((D,), bf16),
            pltpu.VMEM((D, D), bf16),
            pltpu.VMEM((D, D), bf16),
            pltpu.VMEM((D, D), bf16),
            pltpu.VMEM((D, D), bf16),
            pltpu.VMEM((F, D), bf16),
            pltpu.VMEM((F, D), bf16),
            pltpu.VMEM((D, 2 * D), bf16),
            pltpu.VMEM((D, 3 * D), bf16),
            pltpu.VMEM((D, D), bf16),
            pltpu.SemaphoreType.DMA((16,)),
            pltpu.VMEM((8, 6 * D), f32),
            pltpu.VMEM((D // 2, D), u32),
            pltpu.VMEM((D // 2, D), u32),
            pltpu.VMEM((NB, QB // 2, 128 * NG), u32),
            pltpu.VMEM((NB, 16 * H, QB), u32),
            pltpu.VMEM((T // QB, D // 2, QB), u32),
            pltpu.VMEM((T // QB, D, QB), f32),
            pltpu.VMEM((3, 256, 512), f32),
            pltpu.VMEM((2, T // 2, D), u32),
            pltpu.VMEM((T // 2, D), u32),
            pltpu.VMEM((T // 2, D), u32),
            pltpu.VMEM((T + 8, D), f32),
            pltpu.VMEM((T // 2, D), u32),
            pltpu.VMEM((T // 2, F), u32),
            pltpu.VMEM((T // CH, CH, D), f32),
            pltpu.VMEM((S, D), bf16),
            pltpu.SemaphoreType.DMA((1,)),
            pltpu.VMEM((D, 128), f32),
        ],
        compiler_params=pltpu.CompilerParams(
            dimension_semantics=("arbitrary",),
            vmem_limit_bytes=100 * 1024 * 1024,
        ),
    )(A_x, c, B_b1, B_b2, A_wqkv, A_wo, B_w1.T, B_w2, w_mod)
```

```python
import os
import jax
import jax.numpy as jnp
from jax import lax
import jax.experimental.pallas as pl
import jax.experimental.pallas.tpu as pltpu

S, D, H, DH, F = 2048, 640, 32, 20, 1728
T = 256
QB = 128
NB = S // QB
NS = S // T
NG = 8
NU = 2 * NG
CH = 16
NCH = T // CH
FM = 1664
EPS = 1e-5
QSCALE = DH ** -0.5 * 1.4426950408889634
f32, bf16, u32 = jnp.float32, jnp.bfloat16, jnp.uint32
NT = (((1,), (1,)), ((), ()))

PR = [int(v) for v in os.environ.get("PR", "0,160,320,480").split(",")]
N1 = int(os.environ.get("N1", "13"))
U23 = int(os.environ.get("U23", "7"))
S23 = int(os.environ.get("S23", "5"))
UWO = int(os.environ.get("UWO", "3"))
MW = int(os.environ.get("MW", "8"))
SCOPES = os.environ.get("SCOPES", "0") == "1"


def _stats(x):
    m = jnp.sum(x, axis=-1, keepdims=True) * (1.0 / D)
    v = jnp.sum(x * x, axis=-1, keepdims=True) * (1.0 / D) - m * m
    return m, lax.rsqrt(jnp.maximum(v, 0.0) + EPS)


def _ln(x):
    m, r = _stats(x)
    return (x - m) * r


def _pack(x):
    return pltpu.bitcast(x.astype(bf16), u32)


def _packi(x):
    n = x.shape[0] // 16
    return jnp.concatenate(
        [pltpu.bitcast(pltpu.pack_elementwise([x[16 * i:16 * i + 8], x[16 * i + 8:16 * i + 16]],
                                              packed_dtype=bf16), u32) for i in range(n)], axis=0)


def _unpack(x):
    return pltpu.bitcast(x, bf16)


def _rep(v, n):
    return jnp.concatenate([v] * (n // 8), axis=0)


def _gelu(x):
    c = 0.7978845608028654
    return 0.5 * x * (1.0 + jnp.tanh(x * (c + (c * 0.044715) * (x * x))))


class _Null:
    def __enter__(self):
        return None

    def __exit__(self, *a):
        return False


def ns(name):
    return jax.named_scope(name) if SCOPES else _Null()


def kernel(x_h, c_h, b1_h, b2_h, wqkv_h, wo_h, w1t_h, w2_h, wmod_h, o_h,
           x_v, c_v, b1_v, b2_v, wqkv_v, wo_v, w1t_v, w2_v, wmod_v, o_v, sems, osem,
           mod_s, col_s, wqT_s, wvT_s, wk_p, wo_p, w1_p, w2_p,
           k_s, vT_s, qT_s, s_s, oT_s, oa_s, ob_s, hb_s, hi_s, x1_s, y_s, hh_s, hr_s,
           n_s, acc_s, pb_s, pi_s):
    step = pl.program_id(0)
    dyn0 = step >> 10

    def xrows(lo, hi):
        return x_h.at[0, lo:hi], x_v.at[lo:hi]

    def wmcols(lo, hi):
        return wmod_h.at[:, lo:hi], wmod_v.at[:, lo:hi]

    def wrows(lo, hi):
        return wqkv_h.at[lo:hi], wqkv_v.at[lo:hi]

    pairs = dict(
        c=(c_h, c_v), x01=xrows(0, 2 * T),
        sa01=wmcols(0, 256), ca01=wmcols(D, D + 256), w0=wrows(0, 128),
        sa2=wmcols(256, 384), ca2=wmcols(D + 256, D + 384), w1r=wrows(128, 256),
        sa34=wmcols(384, D), ca34=wmcols(D + 384, 2 * D), w2r=wrows(256, 384), w34=wrows(384, D),
        wm2=wmcols(2 * D, 5 * D), wo=(wo_h, wo_v), x2=xrows(2 * T, 3 * T),
        b1=(b1_h, b1_v), b2=(b2_h, b2_v), w1=(w1t_h, w1t_v),
        wm3=wmcols(5 * D, 6 * D), w2=(w2_h, w2_v), xr=xrows(3 * T, S),
    )
    names = list(pairs)

    def cp(n):
        s, d = pairs[n]
        return pltpu.make_async_copy(s, d, sems.at[names.index(n)])

    def wait(*ns_):
        with ns("w_" + ns_[-1]):
            for n in ns_:
                cp(n).wait()

    def silu_c():
        c = c_v[...].astype(f32)
        return c * jax.nn.sigmoid(c)

    def modv(i, n):
        return _rep(mod_s[:, i * D:(i + 1) * D], n)

    def mod_put(t, v):
        mod_s[:, 128 * t:128 * t + 128] = v + 1.0 if t // 5 in (1, 4) else v

    def mod_mxu(tiles):
        sc = jnp.broadcast_to(silu_c().astype(bf16), (16, D))
        w = jnp.concatenate([wmod_v[:, 128 * t:128 * t + 128] for t in tiles], axis=1)
        r = jnp.dot(sc, w, preferred_element_type=f32)[0:8]
        for i, t in enumerate(tiles):
            mod_put(t, r[:, 128 * i:128 * i + 128])

    def mod_vpu(tiles):
        acc = jnp.zeros((MW, 128), f32)
        for t in tiles:
            acc = jnp.where(dyn0 == 1, acc, 0.0)
            for r in range(D // MW):
                rows = slice(MW * r, MW * r + MW)
                acc = acc + wmod_v[rows, 128 * t:128 * t + 128].astype(f32) * col_s[rows, :]
            mod_put(t, jnp.broadcast_to(jnp.sum(acc, axis=0, keepdims=True), (8, 128)))

    def token(v):
        return jnp.where(dyn0 == 1, v[0:8, 0:128], jnp.where(dyn0 == 2, v[8:16, 0:128], 0.0))

    def body(variant):
        first = variant == "first"
        second = variant == "second"
        g0 = step * (T // QB)
        q0 = 2 if second else 0
        lo4 = lax.broadcasted_iota(jnp.int32, (8, QB), 0) < 4
        st = {}

        def weight(w_v, w_p, fresh, lo=0, hi=None):
            hi = w_v.shape[0] if hi is None else hi
            if fresh:
                w = w_v[lo:hi, :]
                w_p[lo // 2:hi // 2, :] = pltpu.bitcast(w, u32)
                return w
            return _unpack(w_p[lo // 2:hi // 2, :])

        def anchor_x1(v):
            x1_s[pl.ds(pl.multiple_of(T + 8 * dyn0, 8), 8), 0:128] = v

        def ln1_chunk(c, blk):
            x = x_v[pl.ds(pl.multiple_of(blk * T + CH * c, CH), CH), :].astype(f32)
            h = _ln(x) * modv(1, CH) + modv(0, CH)
            hb_s[CH // 2 * c:CH // 2 * (c + 1), :] = _pack(h)
            hi_s[CH // 2 * c:CH // 2 * (c + 1), :] = _packi(h)
            return token(h)

        def kstore(kb, blk):
            lane = lax.broadcasted_iota(jnp.int32, (QB, 128), 1)
            tiles = []
            for g in range(NG):
                t0, t1 = (80 * g) // 128, (80 * g + 79) // 128
                if t0 == t1:
                    tiles.append(kb[:, 128 * t0:128 * t0 + 128])
                else:
                    tiles.append(jnp.where(lane >= 64, kb[:, 128 * t0:128 * t0 + 128],
                                           kb[:, 128 * t1:128 * t1 + 128]))
            k_s[blk] = _pack(jnp.concatenate(tiles, axis=1))

        def vstore(src, blk):
            fl = jnp.ones((8, QB), f32)
            out = []
            for hh in range(H):
                a = (DH * hh) // 16
                off = DH * hh - 16 * a
                v = [src[16 * a + 8 * i:16 * a + 8 * i + 8] for i in range(4)]
                if off == 0:
                    out += [v[0], v[1], jnp.where(lo4, v[2], fl), fl]
                elif off == 4:
                    out += [jnp.where(lo4, fl, v[0]), v[1], v[2], fl]
                elif off == 8:
                    out += [fl, v[1], v[2], jnp.where(lo4, v[3], fl)]
                else:
                    out += [fl, jnp.where(lo4, fl, v[1]), v[2], v[3]]
            vT_s[blk] = _pack(jnp.concatenate(out, axis=0))

        dd = (lax.broadcasted_iota(jnp.int32, (16, 128), 1)
              - lax.broadcasted_iota(jnp.int32, (16, 128), 0))
        r64 = lax.broadcasted_iota(jnp.int32, (64, 128), 0)
        l64 = lax.broadcasted_iota(jnp.int32, (64, 128), 1)
        r64 = r64 + (r64 & ~7)
        obits = (jnp.where(r64 > l64, jnp.uint32(0xFFFF), jnp.uint32(0))
                 | jnp.where(r64 + 8 > l64, jnp.uint32(0xFFFF0000), jnp.uint32(0)))
        z8 = jnp.zeros((8, 128), u32)
        lane16 = lax.broadcasted_iota(jnp.int32, (16, 128), 1)
        g_lo = (lane16 & 32) != 0
        g_hi = lane16 >= 64
        r40 = lax.broadcasted_iota(jnp.int32, (40, 128), 0)
        hrow = (r40 >= 10).astype(jnp.int32) + (r40 >= 20).astype(jnp.int32) + (r40 >= 30).astype(jnp.int32)
        hx = hrow ^ (lax.broadcasted_iota(jnp.int32, (40, 128), 1) >> 5)

        def nkeys(b):
            return min(b + 1, 3) if first else 3

        def place(g, vs, tok=None):
            parts = [z8] * 8
            if tok is not None:
                parts[(5 * g + 6) % 8] = pltpu.bitcast(tok, u32)
            for i, v in vs.items():
                parts[(5 * g + i) % 8] = v
            return jnp.concatenate(parts, axis=0)

        def stage1(u, slot, toks=()):
            b, g = divmod(u, NG)
            nk = nkeys(b)
            gb_ = g0 + b
            q5 = qT_s[q0 + b, 40 * g:40 * g + 40, :]
            ws = []
            for j in range(4):
                qm = jnp.where(hrow[8 * j:8 * j + 16] == j, q5[8 * j:8 * j + 16], jnp.uint32(0))
                ws.append(place(g, {j: qm[0:8], j + 1: qm[8:16]}))
            w = _unpack(jnp.concatenate(ws, axis=1))
            ln = slice(128 * g, 128 * g + 128)
            mx = [None]

            def emit(r0, sm):
                s_s[slot, r0:r0 + 16, :] = sm
                mx[0] = sm if mx[0] is None else jnp.maximum(mx[0], sm)

            if nk < 3:
                rows = [k_s[gb_, :, ln]]
                if nk == 2:
                    rows.append(k_s[gb_ - 1, :, ln])
                s = jnp.dot(_unpack(jnp.concatenate(rows, axis=0)), w, preferred_element_type=f32)
                for i in range(8):
                    old4 = jnp.concatenate([dd < 16 * i] * 4, axis=1)
                    emit(16 * i, jnp.where(old4, -1e30, s[16 * i:16 * i + 16]))
                for i in range(8, 8 * nk):
                    emit(16 * i, s[16 * i:16 * i + 16])
            else:
                def kb(B):
                    return k_s[gb_ - 2 + B // 4, 16 * (B % 4):16 * (B % 4) + 16, ln]
                fl = (lane16 - (80 * g) % 128) & 127
                h_hi = fl >= 40
                h_lo = ((fl >= 20) & (fl < 40)) | (fl >= 60)
                x = [kb(0), kb(1), kb(2), kb(11)]
                t = [jnp.where(h_lo, x[v ^ 1], x[v]) for v in range(4)]
                e_l = [jnp.where(h_hi, t[v ^ 2], t[v]) for v in range(4)]
                k9, k10 = kb(9), kb(10)
                j2_l = [jnp.where(h_hi, k10, x[2]), jnp.where(h_hi, x[2], k10)]
                sm = []
                for v in range(4):
                    j1_l = jnp.where((fl >= 20 * v) & (fl < 20 * v + 20), x[1], k9)
                    lhs = jnp.concatenate([e_l[v][0:8], j1_l[0:8], j2_l[v // 2][0:8],
                                           e_l[v][8:16], j1_l[8:16], j2_l[v // 2][8:16]], axis=0)
                    qm = jnp.where(hx == v, q5, jnp.uint32(0))
                    wv = place(g, {i: qm[8 * i:8 * i + 8] for i in range(5)}, toks[v] if v < len(toks) else None)
                    sm.append(jnp.dot(_unpack(lhs), _unpack(wv), preferred_element_type=f32))
                for c in range(2):
                    for J in (1, 2):
                        msk = (dd < 32 * J + 16 * c) & (lane16 >= 32 * J)
                        uu = [jnp.where(msk, sm[v][48 * c:48 * c + 16], sm[v][48 * c + 16 * J:48 * c + 16 * J + 16])
                              for v in range(4)]
                        t = [jnp.where(g_lo, uu[v ^ 1], uu[v]) for v in range(4)]
                        emit(32 * J + 16 * c,
                             jnp.concatenate([jnp.where(g_hi, t[v ^ 2], t[v]) for v in range(4)], axis=1))
                k8, k3 = kb(8), kb(3)
                lhs = jnp.concatenate([k8[0:8], k3[0:8], k8[8:16], k3[8:16], k_s[gb_ - 1, :, ln]], axis=0)
                s = jnp.dot(_unpack(lhs), w, preferred_element_type=f32)
                for c in range(2):
                    e0 = jnp.concatenate([sm[v][48 * c:48 * c + 16] for v in range(4)], axis=1)
                    e3 = jnp.concatenate([sm[v ^ 3][48 * c:48 * c + 16] for v in range(4)], axis=1)
                    old4 = jnp.concatenate([dd < 16 * c] * 4, axis=1)
                    emit(16 * c, jnp.where(old4, e0, s[32 * c:32 * c + 16]))
                    old4 = jnp.concatenate([dd < 96 + 16 * c] * 4, axis=1)
                    emit(96 + 16 * c, jnp.where(old4, s[32 * c + 16:32 * c + 32], e3))
                for i in range(8):
                    emit(128 + 16 * i, s[64 + 16 * i:64 + 16 * i + 16])
            st["m", u] = (jnp.max(mx[0], axis=0, keepdims=True), slot)
            return mx[0][0:8, 0:128]

        def stage2(u):
            b, g = divmod(u, NG)
            m, slot = st.pop(("m", u))
            nk = nkeys(b)
            gb_ = g0 + b
            res = []
            for j in range(4):
                hh = 4 * g + j
                off = DH * hh - 16 * ((DH * hh) // 16)
                ln = slice(128 * j, 128 * j + 128)
                mj = m[:, ln]

                def pp(r0):
                    return _packi(jnp.exp2(s_s[slot, r0:r0 + 128, ln] - mj))
                pm = pp(0)
                if nk == 3:
                    pold = pm & obits
                    p = jnp.concatenate([pold, pm ^ pold, pp(128)], axis=0)
                    blks = [gb_ - 2, gb_, gb_ - 1]
                elif nk == 2:
                    p = jnp.concatenate([pm, pp(128)], axis=0)
                    blks = [gb_, gb_ - 1]
                else:
                    p = pm
                    blks = [gb_]
                vw = _unpack(jnp.concatenate([vT_s[bb, 16 * hh:16 * hh + 16, :] for bb in blks], axis=1))
                o = jnp.dot(vw, _unpack(p), preferred_element_type=f32)
                if off < 8:
                    l, o3 = o[24:32], o[0:24]
                else:
                    l, o3 = o[0:8], o[8:32]
                r = pl.reciprocal(l, approx=True)
                r = r * (2.0 - l * r)
                res.append([o3[8 * i:8 * i + 8] * r for i in range(3)])
            out = []
            for j in (0, 2):
                a_, b_ = res[j], res[j + 1]
                out += [a_[0], a_[1], jnp.where(lo4, a_[2], b_[0]), b_[1], b_[2]]
            ot = 2 * b if first else b
            oT_s[ot, 80 * g:80 * g + 80, :] = jnp.concatenate(out, axis=0)
            if u == NG - 1:
                oa_s[q0 // 2 if not first else 2] = _pack(oT_s[0].T)
            return out[0]

        def wo_stage(r0, n):
            if r0 + n > QB:
                ob_s[...] = _pack(oT_s[2 if second else 1].T)
            oa = oa_s[2] if second else oa_s[st["oa"]]
            ob = jnp.concatenate([oa, ob_s[...]][r0 // QB:(r0 + n) // QB], axis=0)
            y = jnp.dot(_unpack(ob), weight(wo_v, wo_p, second), preferred_element_type=f32)
            x = x_v[pl.ds(pl.multiple_of((step - 1) * T + r0, QB), n), :].astype(f32)
            x1_s[r0:r0 + n, :] = x + modv(2, n) * y

        def ln23_chunk(c):
            y = _ln(_ln(x1_s[CH * c:CH * (c + 1), :]) * modv(4, CH) + modv(3, CH))
            y_s[CH // 2 * c:CH // 2 * (c + 1), :] = _pack(y)
            return token(y)

        def bias(b, n, toks):
            nt = b.shape[1] // 128
            b8 = jnp.broadcast_to(b, (8, b.shape[1]))
            tiles = [b8[:, 128 * j:128 * j + 128] for j in range(nt)]
            for i, t in enumerate(toks):
                tiles[i * nt // len(toks)] = tiles[i * nt // len(toks)] + t
            return _rep(jnp.concatenate(tiles, axis=1), n)

        def w1_stage(r0, n, toks=()):
            b1 = b1_v[...].astype(f32).reshape(1, F)
            hh = _gelu(lax.dot_general(_unpack(y_s[r0 // 2:(r0 + n) // 2, :]), weight(w1t_v, w1_p, second, 0, FM),
                                       NT, preferred_element_type=f32) + bias(b1[:, 0:FM], n, toks))
            hh_s[r0 // 2:(r0 + n) // 2, :] = _pack(hh)

        def w1_rem():
            b1 = b1_v[...].astype(f32).reshape(1, F)[:, FM:F]
            rt = lax.dot_general(weight(w1t_v, w1_p, second, FM, F), _unpack(y_s[...]), NT,
                                 preferred_element_type=f32)
            r = jnp.concatenate([rt[:, 0:QB], rt[:, QB:T]], axis=0).T
            hr_s[...] = _pack(_gelu(r + jnp.concatenate([b1, b1], axis=1)))

        def w2_stage(r0, n, toks=()):
            b = r0 // QB
            b2 = bias(b2_v[...].astype(f32).reshape(1, D), n, toks)
            if second and r0 == 0:
                wr = pltpu.bitcast(w2_v[FM:F, :], u32)
                zz = jnp.zeros_like(wr)
                w2_p[FM // 2:FM // 2 + 128, :] = jnp.concatenate([wr, zz, zz, wr], axis=0)
            wm = weight(w2_v, w2_p, second and r0 == 0, 0, FM)
            wr = _unpack(w2_p[FM // 2 + 64 * b:FM // 2 + 64 * b + 64, :])
            rr = r0 - QB * b
            lhs = jnp.concatenate([hh_s[r0 // 2:(r0 + n) // 2, :], hr_s[rr // 2:(rr + n) // 2, :]], axis=1)
            mo = jnp.dot(_unpack(lhs), jnp.concatenate([wm, wr], axis=0), preferred_element_type=f32) + b2
            rows = pl.ds(pl.multiple_of((step - 1) * T + r0, n), n)
            o_v[rows, :] = (x1_s[r0:r0 + n, :] + modv(5, n) * mo).astype(bf16)
            pltpu.make_async_copy(o_v.at[rows], o_h.at[0, rows], osem.at[0]).start()

        def wt_cols(dst, c0, t):
            w = wqkv_v[128 * t:128 * t + 128, c0:c0 + D].astype(f32).T
            dst[:, 128 * t:128 * t + 128] = _pack(w)
            return token(w[D - 16:D])

        nxt = jnp.minimum(step + 1, NS - 1)
        st["oa"] = jnp.where(step == 2, 1, 0)

        if first:
            def hpiece(t):
                cols = slice(128 * t, 128 * t + 128)
                h = (n_s[:, cols] * _rep(mod_s[:, D + 128 * t:D + 128 * t + 128], 2 * T)
                     + _rep(mod_s[:, cols], 2 * T))
                pb_s[:, cols] = _pack(h)
                pi_s[:, cols] = _packi(h)

            def seg(lo, hi, cols, src):
                w = wqkv_v[lo:hi, cols]
                if cols.start == D:
                    wk_p[lo // 2:hi // 2, :] = pltpu.bitcast(w, u32)
                r = jnp.dot(_unpack(src[:, lo:hi]), w, preferred_element_type=f32)
                return r if lo == 0 else r + acc_s[:, cols]

            parts = ((slice(D, 2 * D), pb_s), (slice(0, D), pb_s), (slice(2 * D, 3 * D), pi_s))

            def segment(lo, hi):
                for cols, src in parts:
                    acc_s[:, cols] = seg(lo, hi, cols, src)

            for n in names:
                cp(n).start()
            wait("c", "x01")
            with ns("ln1a"):
                for c in range(2 * NCH):
                    n_s[CH * c:CH * (c + 1), :] = _ln(x_v[CH * c:CH * (c + 1), :].astype(f32))
            wait("sa01", "ca01")
            with ns("mod1"):
                col_s[...] = jnp.broadcast_to(silu_c().astype(bf16).astype(f32), (128, D)).T
                mod_mxu([0, 5, 1, 6])
                hpiece(0)
            wait("w0")
            with ns("seg0"):
                segment(0, 128)
                hpiece(1)
            wait("sa2", "ca2", "w1r")
            with ns("seg1"):
                segment(128, 256)
                mod_vpu([2, 7])
                hpiece(2)
            wait("sa34", "ca34", "w2r")
            with ns("seg2"):
                segment(256, 384)
                mod_vpu([3, 8, 4, 9])
                hpiece(3)
                hpiece(4)
            wait("w34")
            with ns("attn"):
                kf = seg(384, D, *parts[0])
                for b in range(4):
                    kstore(kf[QB * b:QB * b + QB], b)
                qf = seg(384, D, *parts[1]) * QSCALE
                for b in range(4):
                    qT_s[b] = _pack(qf[QB * b:QB * b + QB].T)
                vf = seg(384, D, *parts[2])
                for b in range(4):
                    vstore(vf[QB * b:QB * b + QB].T, b)
                order = [u for g in range(NG) for u in (NG + g, g)]
                stage1(order[0], 0)
                stage1(order[1], 1)
                for i, u in enumerate(order):
                    if i + 2 < NU:
                        stage1(order[i + 2], (i + 2) % 3)
                    stage2(u)
            wait("wm2", "wo", "x2")
        elif variant in ("second", "mid"):
            if second:
                mod_vpu(range(10, 25))
            else:
                kf = jnp.dot(_unpack(hb_s[...]), _unpack(wk_p[...]), preferred_element_type=f32)
                for b in range(2):
                    kstore(kf[QB * b:QB * b + QB], g0 + b)
                wo_stage(0, T)
                qf = lax.dot_general(_unpack(wqT_s[...]), _unpack(hb_s[...]), NT, preferred_element_type=f32)
                for b in range(2):
                    qT_s[b] = _pack(qf[:, QB * b:QB * b + QB] * QSCALE)
                vf = lax.dot_general(_unpack(wvT_s[...]), _unpack(hi_s[...]), NT, preferred_element_type=f32)
                for b in range(2):
                    vstore(vf[:, QB * b:QB * b + QB], g0 + b)
                an = [z[r:r + 8, 128 * b:128 * b + 128] for z in (qf, vf) for b in range(2) for r in PR]
                for i, a in enumerate(an):
                    anchor_x1(a)
                    for c in range(NCH * i // len(an), NCH * (i + 1) // len(an)):
                        ln23_chunk(c)
            a1 = stage1(0, 0)
            pend = {}
            done23 = 0 if second else NCH
            for u in range(NU):
                if second and u == UWO:
                    wo_stage(0, T)
                if u == NU - 2:
                    if second:
                        wait("b1", "b2", "w1")
                    t1 = [ln1_chunk(c, nxt) for c in range(NCH)]
                    w1_rem()
                    w1_stage(0, T, t1 if second else t1[0:N1])
                if done23 < NCH and u >= S23:
                    anchor_x1(a1)
                    hi23 = min(NCH, -(-NCH * (u + 1 - S23) // U23))
                    pend[u + 3] = [ln23_chunk(c) for c in range(done23, hi23)]
                    done23 = hi23
                if u + 1 < NU:
                    a1 = stage1(u + 1, (u + 1) % 2, pend.pop(u + 1, ()))
                elif second:
                    wait("wm3", "w2")
                    mod_vpu(range(25, 30))
                    w2_stage(0, QB, [wt_cols(wqT_s, 0, t) for t in range(5)])
                else:
                    w2_stage(0, QB, t1[N1:])
                stage2(u)
            w2_stage(QB, QB, [wt_cols(wvT_s, 2 * D, t) for t in range(5)] if second else ())
            if second:
                wait("xr")
        else:
            wo_stage(0, QB)
            for c in range(QB // CH):
                ln23_chunk(c)
            wo_stage(QB, QB)
            for c in range(QB // CH, T // CH):
                ln23_chunk(c)
            w1_stage(0, QB)
            w1_rem()
            w1_stage(QB, QB)
            w2_stage(0, QB)
            w2_stage(QB, QB)
            pltpu.make_async_copy(o_v, o_h.at[0], osem.at[0]).wait()

    @pl.when(step == 0)
    def _():
        with jax.named_scope("sc_first"):
            body("first")

    @pl.when(step == 1)
    def _():
        with jax.named_scope("sc_second"):
            body("second")

    @pl.when((step > 1) & (step < NS))
    def _():
        with jax.named_scope("sc_mid"):
            body("mid")

    @pl.when(step == NS)
    def _():
        with jax.named_scope("sc_last"):
            body("last")


@jax.jit
def pallas_adaLN_cond__sliding_block__mixer_channel_mlp__prompt_kernel(A_x, A_wqkv, A_wo, B_x, B_w1, B_b1, B_w2, B_b2, c, w_mod):
    anyspec = pl.BlockSpec(memory_space=pl.ANY)
    V = pltpu.VMEM
    return pl.pallas_call(
        kernel,
        grid=(NS + 1,),
        in_specs=[anyspec] * 9,
        out_specs=anyspec,
        out_shape=jax.ShapeDtypeStruct((1, S, D), bf16),
        scratch_shapes=[
            V((S, D), bf16), V((1, D), bf16), V((F,), bf16), V((D,), bf16),
            V((D, 3 * D), bf16), V((D, D), bf16), V((F, D), bf16), V((F, D), bf16),
            V((D, 6 * D), bf16), V((S, D), bf16),
            pltpu.SemaphoreType.DMA((21,)), pltpu.SemaphoreType.DMA((1,)),
            V((8, 6 * D), f32), V((D, 128), f32),
            V((D // 2, D), u32), V((D // 2, D), u32), V((D // 2, D), u32), V((D // 2, D), u32),
            V((F // 2, D), u32), V((FM // 2 + 128, D), u32),
            V((NB, QB // 2, 128 * NG), u32), V((NB, 16 * H, QB), u32), V((4, D // 2, QB), u32),
            V((3, 256, 512), f32), V((3, D, QB), f32), V((3, QB // 2, D), u32), V((QB // 2, D), u32),
            V((T // 2, D), u32), V((T // 2, D), u32), V((T + 8, D), f32), V((T // 2, D), u32),
            V((T // 2, FM), u32), V((QB // 2, 128), u32),
            V((2 * T, D), f32), V((2 * T, 3 * D), f32), V((T, D), u32), V((T, D), u32),
        ],
        compiler_params=pltpu.CompilerParams(
            dimension_semantics=("arbitrary",),
            vmem_limit_bytes=100 * 1024 * 1024,
        ),
    )(A_x, c, B_b1, B_b2, A_wqkv, A_wo, B_w1.T, B_w2, w_mod)
```

```python
import os
import jax
import jax.numpy as jnp
from jax import lax
import jax.experimental.pallas as pl
import jax.experimental.pallas.tpu as pltpu

S, D, H, DH, F = 2048, 640, 32, 20, 1728
T = 256
QB = 128
NB = S // QB
NS = S // T
NG = 8
NU = 2 * NG
CH = 16
NCH = T // CH
FM = 1664
EPS = 1e-5
QSCALE = DH ** -0.5 * 1.4426950408889634
f32, bf16, u32 = jnp.float32, jnp.bfloat16, jnp.uint32
NT = (((1,), (1,)), ((), ()))

PR = [int(v) for v in os.environ.get("PR", "0,160,320,480").split(",")]
N1 = int(os.environ.get("N1", "13"))
U23 = int(os.environ.get("U23", "10"))
S23 = int(os.environ.get("S23", "3"))
UWO = int(os.environ.get("UWO", "1"))
MW = int(os.environ.get("MW", "16"))
SEGM = int(os.environ.get("SEGM", "128"))
FQ = int(os.environ.get("FQ", "6"))
SCOPES = os.environ.get("SCOPES", "0") == "1"


def _stats(x):
    m = jnp.sum(x, axis=-1, keepdims=True) * (1.0 / D)
    v = jnp.sum(x * x, axis=-1, keepdims=True) * (1.0 / D) - m * m
    return m, lax.rsqrt(jnp.maximum(v, 0.0) + EPS)


def _ln(x):
    m, r = _stats(x)
    return (x - m) * r


def _pack(x):
    return pltpu.bitcast(x.astype(bf16), u32)


def _packi(x):
    n = x.shape[0] // 16
    return jnp.concatenate(
        [pltpu.bitcast(pltpu.pack_elementwise([x[16 * i:16 * i + 8], x[16 * i + 8:16 * i + 16]],
                                              packed_dtype=bf16), u32) for i in range(n)], axis=0)


def _unpack(x):
    return pltpu.bitcast(x, bf16)


def _rep(v, n):
    return jnp.concatenate([v] * (n // 8), axis=0)


def _gelu(x):
    c = 0.7978845608028654
    return 0.5 * x * (1.0 + jnp.tanh(x * (c + (c * 0.044715) * (x * x))))


class _Null:
    def __enter__(self):
        return None

    def __exit__(self, *a):
        return False


def ns(name):
    return jax.named_scope(name) if SCOPES else _Null()


def kernel(x_h, c_h, b1_h, b2_h, wqkv_h, wo_h, w1t_h, w2_h, wmod_h, o_h,
           x_v, c_v, b1_v, b2_v, wqkv_v, wo_v, w1t_v, w2_v, wmod_v, o_v, sems, osem,
           mod_s, col_s, wqT_s, wvT_s, wk_p, wo_p, w1_p, w2_p,
           k_s, vT_s, qT_s, s_s, oT_s, oa_s, ob_s, hb_s, hi_s, x1_s, y_s, hh_s, hr_s,
           n_s, acc_s):
    step = pl.program_id(0)
    dyn0 = step >> 10

    def xrows(lo, hi):
        return x_h.at[0, lo:hi], x_v.at[lo:hi]

    def wmcols(lo, hi):
        return wmod_h.at[:, lo:hi], wmod_v.at[:, lo:hi]

    def wrows(lo, hi):
        return wqkv_h.at[lo:hi], wqkv_v.at[lo:hi]

    pairs = dict(
        c=(c_h, c_v), x01=xrows(0, 2 * T),
        sa01=wmcols(0, 256), ca01=wmcols(D, D + 256), w0=wrows(0, 128),
        sa2=wmcols(256, 384), ca2=wmcols(D + 256, D + 384), w1r=wrows(128, 256),
        sa34=wmcols(384, D), ca34=wmcols(D + 384, 2 * D), w2r=wrows(256, 384), w34=wrows(384, D),
        wm2=wmcols(2 * D, 5 * D), wo=(wo_h, wo_v), x2=xrows(2 * T, 3 * T),
        b1=(b1_h, b1_v), b2=(b2_h, b2_v), w1=(w1t_h, w1t_v),
        wm3=wmcols(5 * D, 6 * D), w2=(w2_h, w2_v), xr=xrows(3 * T, S),
    )
    names = list(pairs)

    def cp(n):
        s, d = pairs[n]
        return pltpu.make_async_copy(s, d, sems.at[names.index(n)])

    def wait(*ns_):
        with ns("w_" + ns_[-1]):
            for n in ns_:
                cp(n).wait()

    def silu_c():
        c = c_v[...].astype(f32)
        return c * jax.nn.sigmoid(c)

    def modv(i, n):
        return _rep(mod_s[:, i * D:(i + 1) * D], n)

    def mod_put(t, v):
        mod_s[:, 128 * t:128 * t + 128] = v + 1.0 if t // 5 in (1, 4) else v

    def mod_mxu(tiles):
        sc = jnp.broadcast_to(silu_c().astype(bf16), (16, D))
        w = jnp.concatenate([wmod_v[:, 128 * t:128 * t + 128] for t in tiles], axis=1)
        r = jnp.dot(sc, w, preferred_element_type=f32)[0:8]
        for i, t in enumerate(tiles):
            mod_put(t, r[:, 128 * i:128 * i + 128])

    def mod_vpu(tiles, MW=8):
        acc = jnp.zeros((MW, 128), f32)
        for t in tiles:
            acc = jnp.where(dyn0 == 1, acc, 0.0)
            for r in range(D // MW):
                rows = slice(MW * r, MW * r + MW)
                acc = acc + wmod_v[rows, 128 * t:128 * t + 128].astype(f32) * col_s[rows, :]
            mod_put(t, jnp.broadcast_to(jnp.sum(acc, axis=0, keepdims=True), (8, 128)))

    def token(v):
        return jnp.where(dyn0 == 1, v[0:8, 0:128], jnp.where(dyn0 == 2, v[8:16, 0:128], 0.0))

    def body(variant):
        first = variant == "first"
        second = variant == "second"
        g0 = step * (T // QB)
        q0 = 2 if second else 0
        lo4 = lax.broadcasted_iota(jnp.int32, (8, QB), 0) < 4
        st = {}

        def weight(w_v, w_p, fresh, lo=0, hi=None):
            hi = w_v.shape[0] if hi is None else hi
            if fresh:
                w = w_v[lo:hi, :]
                w_p[lo // 2:hi // 2, :] = pltpu.bitcast(w, u32)
                return w
            return _unpack(w_p[lo // 2:hi // 2, :])

        def anchor_x1(v):
            x1_s[pl.ds(pl.multiple_of(T + 8 * dyn0, 8), 8), 0:128] = v

        def ln1_chunk(c, blk):
            x = x_v[pl.ds(pl.multiple_of(blk * T + CH * c, CH), CH), :].astype(f32)
            h = _ln(x) * modv(1, CH) + modv(0, CH)
            hb_s[CH // 2 * c:CH // 2 * (c + 1), :] = _pack(h)
            hi_s[CH // 2 * c:CH // 2 * (c + 1), :] = _packi(h)
            return token(h)

        def kstore(kb, blk):
            lane = lax.broadcasted_iota(jnp.int32, (QB, 128), 1)
            tiles = []
            for g in range(NG):
                t0, t1 = (80 * g) // 128, (80 * g + 79) // 128
                if t0 == t1:
                    tiles.append(kb[:, 128 * t0:128 * t0 + 128])
                else:
                    tiles.append(jnp.where(lane >= 64, kb[:, 128 * t0:128 * t0 + 128],
                                           kb[:, 128 * t1:128 * t1 + 128]))
            k_s[blk] = _pack(jnp.concatenate(tiles, axis=1))

        def vstore(src, blk):
            fl = jnp.ones((8, QB), f32)
            out = []
            for hh in range(H):
                a = (DH * hh) // 16
                off = DH * hh - 16 * a
                v = [src[16 * a + 8 * i:16 * a + 8 * i + 8] for i in range(4)]
                if off == 0:
                    out += [v[0], v[1], jnp.where(lo4, v[2], fl), fl]
                elif off == 4:
                    out += [jnp.where(lo4, fl, v[0]), v[1], v[2], fl]
                elif off == 8:
                    out += [fl, v[1], v[2], jnp.where(lo4, v[3], fl)]
                else:
                    out += [fl, jnp.where(lo4, fl, v[1]), v[2], v[3]]
            vT_s[blk] = _pack(jnp.concatenate(out, axis=0))

        dd = (lax.broadcasted_iota(jnp.int32, (16, 128), 1)
              - lax.broadcasted_iota(jnp.int32, (16, 128), 0))
        r64 = lax.broadcasted_iota(jnp.int32, (64, 128), 0)
        l64 = lax.broadcasted_iota(jnp.int32, (64, 128), 1)
        r64 = r64 + (r64 & ~7)
        obits = (jnp.where(r64 > l64, jnp.uint32(0xFFFF), jnp.uint32(0))
                 | jnp.where(r64 + 8 > l64, jnp.uint32(0xFFFF0000), jnp.uint32(0)))
        z8 = jnp.zeros((8, 128), u32)
        lane16 = lax.broadcasted_iota(jnp.int32, (16, 128), 1)
        g_lo = (lane16 & 32) != 0
        g_hi = lane16 >= 64
        r40 = lax.broadcasted_iota(jnp.int32, (40, 128), 0)
        hrow = (r40 >= 10).astype(jnp.int32) + (r40 >= 20).astype(jnp.int32) + (r40 >= 30).astype(jnp.int32)
        hx = hrow ^ (lax.broadcasted_iota(jnp.int32, (40, 128), 1) >> 5)

        def nkeys(b):
            return min(b + 1, 3) if first else 3

        def place(g, vs, tok=None):
            parts = [z8] * 8
            if tok is not None:
                parts[(5 * g + 6) % 8] = pltpu.bitcast(tok, u32)
            for i, v in vs.items():
                parts[(5 * g + i) % 8] = v
            return jnp.concatenate(parts, axis=0)

        def stage1(u, slot, toks=()):
            b, g = divmod(u, NG)
            nk = nkeys(b)
            gb_ = g0 + b
            q5 = qT_s[q0 + b, 40 * g:40 * g + 40, :]
            ws = []
            for j in range(4):
                qm = jnp.where(hrow[8 * j:8 * j + 16] == j, q5[8 * j:8 * j + 16], jnp.uint32(0))
                ws.append(place(g, {j: qm[0:8], j + 1: qm[8:16]}))
            w = _unpack(jnp.concatenate(ws, axis=1))
            ln = slice(128 * g, 128 * g + 128)
            mx = [None]

            def emit(r0, sm):
                s_s[slot, r0:r0 + 16, :] = sm
                mx[0] = sm if mx[0] is None else jnp.maximum(mx[0], sm)

            if nk < 3:
                rows = [k_s[gb_, :, ln]]
                if nk == 2:
                    rows.append(k_s[gb_ - 1, :, ln])
                s = jnp.dot(_unpack(jnp.concatenate(rows, axis=0)), w, preferred_element_type=f32)
                for i in range(8):
                    old4 = jnp.concatenate([dd < 16 * i] * 4, axis=1)
                    emit(16 * i, jnp.where(old4, -1e30, s[16 * i:16 * i + 16]))
                for i in range(8, 8 * nk):
                    emit(16 * i, s[16 * i:16 * i + 16])
            else:
                def kb(B):
                    return k_s[gb_ - 2 + B // 4, 16 * (B % 4):16 * (B % 4) + 16, ln]
                fl = (lane16 - (80 * g) % 128) & 127
                h_hi = fl >= 40
                h_lo = ((fl >= 20) & (fl < 40)) | (fl >= 60)
                x = [kb(0), kb(1), kb(2), kb(11)]
                t = [jnp.where(h_lo, x[v ^ 1], x[v]) for v in range(4)]
                e_l = [jnp.where(h_hi, t[v ^ 2], t[v]) for v in range(4)]
                k9, k10 = kb(9), kb(10)
                j2_l = [jnp.where(h_hi, k10, x[2]), jnp.where(h_hi, x[2], k10)]
                sm = []
                for v in range(4):
                    j1_l = jnp.where((fl >= 20 * v) & (fl < 20 * v + 20), x[1], k9)
                    lhs = jnp.concatenate([e_l[v][0:8], j1_l[0:8], j2_l[v // 2][0:8],
                                           e_l[v][8:16], j1_l[8:16], j2_l[v // 2][8:16]], axis=0)
                    qm = jnp.where(hx == v, q5, jnp.uint32(0))
                    wv = place(g, {i: qm[8 * i:8 * i + 8] for i in range(5)}, toks[v] if v < len(toks) else None)
                    sm.append(jnp.dot(_unpack(lhs), _unpack(wv), preferred_element_type=f32))
                for c in range(2):
                    for J in (1, 2):
                        msk = (dd < 32 * J + 16 * c) & (lane16 >= 32 * J)
                        uu = [jnp.where(msk, sm[v][48 * c:48 * c + 16], sm[v][48 * c + 16 * J:48 * c + 16 * J + 16])
                              for v in range(4)]
                        t = [jnp.where(g_lo, uu[v ^ 1], uu[v]) for v in range(4)]
                        emit(32 * J + 16 * c,
                             jnp.concatenate([jnp.where(g_hi, t[v ^ 2], t[v]) for v in range(4)], axis=1))
                k8, k3 = kb(8), kb(3)
                lhs = jnp.concatenate([k8[0:8], k3[0:8], k8[8:16], k3[8:16], k_s[gb_ - 1, :, ln]], axis=0)
                s = jnp.dot(_unpack(lhs), w, preferred_element_type=f32)
                for c in range(2):
                    e0 = jnp.concatenate([sm[v][48 * c:48 * c + 16] for v in range(4)], axis=1)
                    e3 = jnp.concatenate([sm[v ^ 3][48 * c:48 * c + 16] for v in range(4)], axis=1)
                    old4 = jnp.concatenate([dd < 16 * c] * 4, axis=1)
                    emit(16 * c, jnp.where(old4, e0, s[32 * c:32 * c + 16]))
                    old4 = jnp.concatenate([dd < 96 + 16 * c] * 4, axis=1)
                    emit(96 + 16 * c, jnp.where(old4, s[32 * c + 16:32 * c + 32], e3))
                for i in range(8):
                    emit(128 + 16 * i, s[64 + 16 * i:64 + 16 * i + 16])
            st["m", u] = (jnp.max(mx[0], axis=0, keepdims=True), slot)
            return mx[0][0:8, 0:128]

        def stage2(u):
            b, g = divmod(u, NG)
            m, slot = st.pop(("m", u))
            nk = nkeys(b)
            gb_ = g0 + b
            res = []
            for j in range(4):
                hh = 4 * g + j
                off = DH * hh - 16 * ((DH * hh) // 16)
                ln = slice(128 * j, 128 * j + 128)
                mj = m[:, ln]

                def pp(r0):
                    return _packi(jnp.exp2(s_s[slot, r0:r0 + 128, ln] - mj))
                pm = pp(0)
                if nk == 3:
                    pold = pm & obits
                    p = jnp.concatenate([pold, pm ^ pold, pp(128)], axis=0)
                    blks = [gb_ - 2, gb_, gb_ - 1]
                elif nk == 2:
                    p = jnp.concatenate([pm, pp(128)], axis=0)
                    blks = [gb_, gb_ - 1]
                else:
                    p = pm
                    blks = [gb_]
                vw = _unpack(jnp.concatenate([vT_s[bb, 16 * hh:16 * hh + 16, :] for bb in blks], axis=1))
                o = jnp.dot(vw, _unpack(p), preferred_element_type=f32)
                if off < 8:
                    l, o3 = o[24:32], o[0:24]
                else:
                    l, o3 = o[0:8], o[8:32]
                r = pl.reciprocal(l, approx=True)
                r = r * (2.0 - l * r)
                res.append([o3[8 * i:8 * i + 8] * r for i in range(3)])
            out = []
            for j in (0, 2):
                a_, b_ = res[j], res[j + 1]
                out += [a_[0], a_[1], jnp.where(lo4, a_[2], b_[0]), b_[1], b_[2]]
            ot = 2 if (first and b == 0) else b
            oT_s[ot, 80 * g:80 * g + 80, :] = jnp.concatenate(out, axis=0)
            if u == NG - 1 and not first:
                oa_s[...] = _pack(oT_s[0].T)

        def wo_stage(r0, n):
            if second:
                oa_s[...] = _pack(oT_s[2].T)
            if r0 + n > QB:
                ob_s[...] = _pack(oT_s[1].T)
            ob = jnp.concatenate([r[...] for r in (oa_s, ob_s)[r0 // QB:(r0 + n) // QB]], axis=0)
            y = jnp.dot(_unpack(ob), weight(wo_v, wo_p, second), preferred_element_type=f32)
            x = x_v[pl.ds(pl.multiple_of((step - 1) * T + r0, QB), n), :].astype(f32)
            x1_s[r0:r0 + n, :] = x + modv(2, n) * y

        def ln23_chunk(c):
            y = _ln(_ln(x1_s[CH * c:CH * (c + 1), :]) * modv(4, CH) + modv(3, CH))
            y_s[CH // 2 * c:CH // 2 * (c + 1), :] = _pack(y)
            return token(y)

        def bias(b, n, toks):
            nt = b.shape[1] // 128
            b8 = jnp.broadcast_to(b, (8, b.shape[1]))
            tiles = [b8[:, 128 * j:128 * j + 128] for j in range(nt)]
            for i, t in enumerate(toks):
                tiles[i * nt // len(toks)] = tiles[i * nt // len(toks)] + t
            return _rep(jnp.concatenate(tiles, axis=1), n)

        def w1_stage(r0, n, toks=()):
            b1 = b1_v[...].astype(f32).reshape(1, F)
            hh = _gelu(lax.dot_general(_unpack(y_s[r0 // 2:(r0 + n) // 2, :]), weight(w1t_v, w1_p, second, 0, FM),
                                       NT, preferred_element_type=f32) + bias(b1[:, 0:FM], n, toks))
            hh_s[r0 // 2:(r0 + n) // 2, :] = _pack(hh)

        def w1_rem():
            b1 = b1_v[...].astype(f32).reshape(1, F)[:, FM:F]
            rt = lax.dot_general(weight(w1t_v, w1_p, second, FM, F), _unpack(y_s[...]), NT,
                                 preferred_element_type=f32)
            r = jnp.concatenate([rt[:, 0:QB], rt[:, QB:T]], axis=0).T
            hr_s[...] = _pack(_gelu(r + jnp.concatenate([b1, b1], axis=1)))

        def w2_stage(r0, n, toks=()):
            b = r0 // QB
            b2 = bias(b2_v[...].astype(f32).reshape(1, D), n, toks)
            if second and r0 == 0:
                wr = pltpu.bitcast(w2_v[FM:F, :], u32)
                zz = jnp.zeros_like(wr)
                w2_p[FM // 2:FM // 2 + 128, :] = jnp.concatenate([wr, zz, zz, wr], axis=0)
            wm = weight(w2_v, w2_p, second and r0 == 0, 0, FM)
            wr = _unpack(w2_p[FM // 2 + 64 * b:FM // 2 + 64 * b + 64, :])
            rr = r0 - QB * b
            lhs = jnp.concatenate([hh_s[r0 // 2:(r0 + n) // 2, :], hr_s[rr // 2:(rr + n) // 2, :]], axis=1)
            mo = jnp.dot(_unpack(lhs), jnp.concatenate([wm, wr], axis=0), preferred_element_type=f32) + b2
            rows = pl.ds(pl.multiple_of((step - 1) * T + r0, n), n)
            o_v[rows, :] = (x1_s[r0:r0 + n, :] + modv(5, n) * mo).astype(bf16)
            pltpu.make_async_copy(o_v.at[rows], o_h.at[0, rows], osem.at[0]).start()

        def wt_cols(dst, c0, t):
            w = wqkv_v[128 * t:128 * t + 128, c0:c0 + D].astype(f32).T
            dst[:, 128 * t:128 * t + 128] = _pack(w)
            return token(w[D - 16:D])

        nxt = jnp.minimum(step + 1, NS - 1)

        if first:
            def seg(lo, hi, c0, c1, r0, r1):
                h = (n_s[r0:r1, lo:hi] * _rep(mod_s[:, D + lo:D + hi], r1 - r0) + _rep(mod_s[:, lo:hi], r1 - r0))
                lhs = _unpack(_packi(h)) if c0 == 2 * D else h.astype(bf16)
                w = wqkv_v[lo:hi, c0:c1]
                if r0 == 0 and c1 == 2 * D:
                    wk_p[lo // 2:hi // 2, :] = pltpu.bitcast(w[:, c1 - c0 - D:], u32)
                r = jnp.dot(lhs, w, preferred_element_type=f32)
                return r if lo == 0 else r + acc_s[r0:r1, c0:c1]

            def segment(lo, hi):
                for r0 in range(0, 2 * T, SEGM):
                    acc_s[r0:r0 + SEGM, 0:2 * D] = seg(lo, hi, 0, 2 * D, r0, r0 + SEGM)
                    acc_s[r0:r0 + SEGM, 2 * D:3 * D] = seg(lo, hi, 2 * D, 3 * D, r0, r0 + SEGM)

            def fin(which, b0, b1):
                r = seg(384, D, which * D, (which + 1) * D, QB * b0, QB * b1)
                for b in range(b0, b1):
                    rb = r[QB * (b - b0):QB * (b - b0 + 1)]
                    if which == 0:
                        qT_s[b] = _pack((rb * QSCALE).T)
                    elif which == 1:
                        kstore(rb, b)
                    else:
                        vstore(rb.T, b)

            for n in names:
                cp(n).start()
            wait("c", "x01")
            with ns("ln1a"):
                for c in range(2 * NCH):
                    n_s[CH * c:CH * (c + 1), :] = _ln(x_v[CH * c:CH * (c + 1), :].astype(f32))
            wait("sa01", "ca01")
            with ns("mod1"):
                col_s[...] = jnp.broadcast_to(silu_c().astype(bf16).astype(f32), (128, D)).T
                mod_mxu([0, 5, 1, 6])
            wait("w0")
            with ns("seg0"):
                segment(0, 128)
            wait("sa2", "ca2", "w1r")
            with ns("seg1"):
                segment(128, 256)
                mod_vpu([2, 7])
            wait("sa34", "ca34", "w2r")
            with ns("seg2"):
                segment(256, 384)
                mod_vpu([3, 8, 4, 9])
            wait("w34")
            with ns("attn"):
                fin(2, 0, 2)
                fin(0, 0, 2)
                fin(1, 0, 2)
                fin(2, 2, 4)
                order = [u for g in range(NG) for u in (NG + g, g)]
                stage1(order[0], 0)
                stage1(order[1], 1)
                for i, u in enumerate(order):
                    if i + 2 < NU:
                        stage1(order[i + 2], (i + 2) % 3)
                    if i == FQ:
                        fin(0, 2, 4)
                    if i == NU - 2:
                        fin(1, 2, 3)
                    stage2(u)
                fin(1, 3, 4)
            wait("wm2", "wo", "x2")
        elif variant in ("second", "mid"):
            if second:
                mod_vpu([t + j for j in range(5) for t in (15, 20, 10)], MW)
            else:
                kf = jnp.dot(_unpack(hb_s[...]), _unpack(wk_p[...]), preferred_element_type=f32)
                for b in range(2):
                    kstore(kf[QB * b:QB * b + QB], g0 + b)
                wo_stage(0, T)
                qf = lax.dot_general(_unpack(wqT_s[...]), _unpack(hb_s[...]), NT, preferred_element_type=f32)
                for b in range(2):
                    qT_s[b] = _pack(qf[:, QB * b:QB * b + QB] * QSCALE)
                vf = lax.dot_general(_unpack(wvT_s[...]), _unpack(hi_s[...]), NT, preferred_element_type=f32)
                for b in range(2):
                    vstore(vf[:, QB * b:QB * b + QB], g0 + b)
                an = [z[r:r + 8, 128 * b:128 * b + 128] for z in (qf, vf) for b in range(2) for r in PR]
                for i, a in enumerate(an):
                    anchor_x1(a)
                    for c in range(NCH * i // len(an), NCH * (i + 1) // len(an)):
                        ln23_chunk(c)
            a1 = stage1(0, 0)
            pend = {}
            done23 = 0 if second else NCH
            for u in range(NU):
                if second and u == UWO:
                    wo_stage(0, T)
                if u == NU - 2:
                    if second:
                        wait("b1", "b2", "w1")
                    t1 = [ln1_chunk(c, nxt) for c in range(NCH)]
                    w1_rem()
                    w1_stage(0, T, t1 if second else t1[0:N1])
                if done23 < NCH and u >= S23:
                    anchor_x1(a1)
                    hi23 = min(NCH, -(-NCH * (u + 1 - S23) // U23))
                    pend[u + 3] = [ln23_chunk(c) for c in range(done23, hi23)]
                    done23 = hi23
                if u + 1 < NU:
                    a1 = stage1(u + 1, (u + 1) % 2, pend.pop(u + 1, ()))
                elif second:
                    wait("wm3", "w2")
                    mod_vpu(range(25, 30))
                    w2_stage(0, QB, [wt_cols(wqT_s, 0, t) for t in range(5)])
                else:
                    w2_stage(0, QB, t1[N1:])
                stage2(u)
            w2_stage(QB, QB, [wt_cols(wvT_s, 2 * D, t) for t in range(5)] if second else ())
            if second:
                wait("xr")
        else:
            wo_stage(0, QB)
            for c in range(QB // CH):
                ln23_chunk(c)
            wo_stage(QB, QB)
            for c in range(QB // CH, T // CH):
                ln23_chunk(c)
            w1_stage(0, QB)
            w1_rem()
            w1_stage(QB, QB)
            w2_stage(0, QB)
            w2_stage(QB, QB)
            pltpu.make_async_copy(o_v, o_h.at[0], osem.at[0]).wait()

    @pl.when(step == 0)
    def _():
        with jax.named_scope("sc_first"):
            body("first")

    @pl.when(step == 1)
    def _():
        with jax.named_scope("sc_second"):
            body("second")

    @pl.when((step > 1) & (step < NS))
    def _():
        with jax.named_scope("sc_mid"):
            body("mid")

    @pl.when(step == NS)
    def _():
        with jax.named_scope("sc_last"):
            body("last")


@jax.jit
def pallas_adaLN_cond__sliding_block__mixer_channel_mlp__prompt_kernel(A_x, A_wqkv, A_wo, B_x, B_w1, B_b1, B_w2, B_b2, c, w_mod):
    anyspec = pl.BlockSpec(memory_space=pl.ANY)
    V = pltpu.VMEM
    return pl.pallas_call(
        kernel,
        grid=(NS + 1,),
        in_specs=[anyspec] * 9,
        out_specs=anyspec,
        out_shape=jax.ShapeDtypeStruct((1, S, D), bf16),
        scratch_shapes=[
            V((S, D), bf16), V((1, D), bf16), V((F,), bf16), V((D,), bf16),
            V((D, 3 * D), bf16), V((D, D), bf16), V((F, D), bf16), V((F, D), bf16),
            V((D, 6 * D), bf16), V((S, D), bf16),
            pltpu.SemaphoreType.DMA((21,)), pltpu.SemaphoreType.DMA((1,)),
            V((8, 6 * D), f32), V((D, 128), f32),
            V((D // 2, D), u32), V((D // 2, D), u32), V((D // 2, D), u32), V((D // 2, D), u32),
            V((F // 2, D), u32), V((FM // 2 + 128, D), u32),
            V((NB, QB // 2, 128 * NG), u32), V((NB, 16 * H, QB), u32), V((4, D // 2, QB), u32),
            V((3, 256, 512), f32), V((3, D, QB), f32), V((QB // 2, D), u32), V((QB // 2, D), u32),
            V((T // 2, D), u32), V((T // 2, D), u32), V((T + 8, D), f32), V((T // 2, D), u32),
            V((T // 2, FM), u32), V((QB // 2, 128), u32),
            V((2 * T, D), f32), V((2 * T, 3 * D), f32),
        ],
        compiler_params=pltpu.CompilerParams(
            dimension_semantics=("arbitrary",),
            vmem_limit_bytes=100 * 1024 * 1024,
        ),
    )(A_x, c, B_b1, B_b2, A_wqkv, A_wo, B_w1.T, B_w2, w_mod)
```

```python
import jax
import jax.numpy as jnp
from jax import lax
import jax.experimental.pallas as pl
import jax.experimental.pallas.tpu as pltpu

S, D, H, DH, F = 2048, 640, 32, 20, 1728
T = 256
QB = 128
NB = S // QB
NS = S // T
NG = 8
NU = 2 * NG
CH = 16
NCH = T // CH
FM = 1664
EPS = 1e-5
QSCALE = DH ** -0.5 * 1.4426950408889634
f32, bf16, u32 = jnp.float32, jnp.bfloat16, jnp.uint32
NT = (((1,), (1,)), ((), ()))


def _ln(x):
    m = jnp.sum(x, axis=-1, keepdims=True) * (1.0 / D)
    v = jnp.sum(x * x, axis=-1, keepdims=True) * (1.0 / D) - m * m
    return (x - m) * lax.rsqrt(jnp.maximum(v, 0.0) + EPS)


def _pack(x):
    return pltpu.bitcast(x.astype(bf16), u32)


def _packi(x):
    n = x.shape[0] // 16
    return jnp.concatenate(
        [pltpu.bitcast(pltpu.pack_elementwise([x[16 * i:16 * i + 8], x[16 * i + 8:16 * i + 16]],
                                              packed_dtype=bf16), u32) for i in range(n)], axis=0)


def _unpack(x):
    return pltpu.bitcast(x, bf16)


def _rep(v, n):
    return jnp.concatenate([v] * (n // 8), axis=0)


def _gelu(x):
    c = 0.7978845608028654
    return 0.5 * x * (1.0 + jnp.tanh(x * (c + (c * 0.044715) * (x * x))))


def _kernel(x_h, c_h, b1_h, b2_h, wqkv_h, wo_h, w1t_h, w2_h, wmod_h, o_h,
            x_v, c_v, b1_v, b2_v, wqkv_v, wo_v, w1t_v, w2_v, wmod_v, o_v, sems, osem,
            mod_s, col_s, wqT_s, wvT_s, wk_p, wo_p, w1_p, w2_p,
            k_s, vT_s, qT_s, s_s, oT_s, oa_s, ob_s, hb_s, hi_s, x1_s, y_s, hh_s, hr_s,
            n_s, acc_s):
    step = pl.program_id(0)
    dyn0 = step >> 10

    def xrows(lo, hi):
        return x_h.at[0, lo:hi], x_v.at[lo:hi]

    def wmcols(lo, hi):
        return wmod_h.at[:, lo:hi], wmod_v.at[:, lo:hi]

    def wrows(lo, hi):
        return wqkv_h.at[lo:hi], wqkv_v.at[lo:hi]

    pairs = dict(c=(c_h, c_v), x0=xrows(0, T))
    for k in range(5):
        pairs["sa%d" % k] = wmcols(128 * k, 128 * k + 128)
        pairs["ca%d" % k] = wmcols(D + 128 * k, D + 128 * k + 128)
        pairs["r%d" % k] = wrows(128 * k, 128 * k + 128)
        if k == 0:
            pairs["x1"] = xrows(T, 2 * T)
    pairs.update(
        wm2=wmcols(2 * D, 5 * D), wo=(wo_h, wo_v), x2=xrows(2 * T, 3 * T),
        b1=(b1_h, b1_v), b2=(b2_h, b2_v), w1=(w1t_h, w1t_v),
        wm3=wmcols(5 * D, 6 * D), w2=(w2_h, w2_v), xr=xrows(3 * T, S),
    )
    names = list(pairs)

    def cp(n):
        s, d = pairs[n]
        return pltpu.make_async_copy(s, d, sems.at[names.index(n)])

    def wait(*ns):
        for n in ns:
            cp(n).wait()

    def silu_c():
        c = c_v[...].astype(f32)
        return (c * jax.nn.sigmoid(c)).astype(bf16)

    def modv(i, n):
        return _rep(mod_s[:, i * D:(i + 1) * D], n)

    def mod_put(t, v):
        mod_s[:, 128 * t:128 * t + 128] = v + 1.0 if t // 5 in (1, 4) else v

    def mod_mxu(tiles):
        w = jnp.concatenate([wmod_v[:, 128 * t:128 * t + 128] for t in tiles], axis=1)
        r = jnp.dot(jnp.broadcast_to(silu_c(), (16, D)), w, preferred_element_type=f32)[0:8]
        for i, t in enumerate(tiles):
            mod_put(t, r[:, 128 * i:128 * i + 128])

    def mod_vpu(tiles, mw):
        acc = jnp.zeros((mw, 128), f32)
        for t in tiles:
            acc = jnp.where(dyn0 == 1, acc, 0.0)
            for r in range(D // mw):
                rows = slice(mw * r, mw * r + mw)
                acc = acc + wmod_v[rows, 128 * t:128 * t + 128].astype(f32) * col_s[rows, :]
            mod_put(t, jnp.broadcast_to(jnp.sum(acc, axis=0, keepdims=True), (8, 128)))

    def token(v):
        return jnp.where(dyn0 == 1, v[0:8, 0:128], jnp.where(dyn0 == 2, v[8:16, 0:128], 0.0))

    def body(variant):
        first = variant == "first"
        second = variant == "second"
        g0 = step * (T // QB)
        q0 = 2 if second else 0
        lo4 = lax.broadcasted_iota(jnp.int32, (8, QB), 0) < 4
        st = {}

        def weight(w_v, w_p, fresh, lo=0, hi=None):
            hi = w_v.shape[0] if hi is None else hi
            if fresh:
                w = w_v[lo:hi, :]
                w_p[lo // 2:hi // 2, :] = pltpu.bitcast(w, u32)
                return w
            return _unpack(w_p[lo // 2:hi // 2, :])

        def anchor_x1(v):
            x1_s[pl.ds(pl.multiple_of(T + 8 * dyn0, 8), 8), 0:128] = v

        def ln1_chunk(c, blk):
            x = x_v[pl.ds(pl.multiple_of(blk * T + CH * c, CH), CH), :].astype(f32)
            h = _ln(x) * modv(1, CH) + modv(0, CH)
            hb_s[CH // 2 * c:CH // 2 * (c + 1), :] = _pack(h)
            hi_s[CH // 2 * c:CH // 2 * (c + 1), :] = _packi(h)
            return token(h)

        def kstore(kb, blk):
            lane = lax.broadcasted_iota(jnp.int32, (QB, 128), 1)
            tiles = []
            for g in range(NG):
                t0, t1 = (80 * g) // 128, (80 * g + 79) // 128
                if t0 == t1:
                    tiles.append(kb[:, 128 * t0:128 * t0 + 128])
                else:
                    tiles.append(jnp.where(lane >= 64, kb[:, 128 * t0:128 * t0 + 128],
                                           kb[:, 128 * t1:128 * t1 + 128]))
            k_s[blk] = _pack(jnp.concatenate(tiles, axis=1))

        def vstore(src, blk):
            fl = jnp.ones((8, QB), f32)
            out = []
            for hh in range(H):
                a = (DH * hh) // 16
                off = DH * hh - 16 * a
                v = [src[16 * a + 8 * i:16 * a + 8 * i + 8] for i in range(4)]
                if off == 0:
                    out += [v[0], v[1], jnp.where(lo4, v[2], fl), fl]
                elif off == 4:
                    out += [jnp.where(lo4, fl, v[0]), v[1], v[2], fl]
                elif off == 8:
                    out += [fl, v[1], v[2], jnp.where(lo4, v[3], fl)]
                else:
                    out += [fl, jnp.where(lo4, fl, v[1]), v[2], v[3]]
            vT_s[blk] = _pack(jnp.concatenate(out, axis=0))

        dd = (lax.broadcasted_iota(jnp.int32, (16, 128), 1)
              - lax.broadcasted_iota(jnp.int32, (16, 128), 0))
        r64 = lax.broadcasted_iota(jnp.int32, (64, 128), 0)
        l64 = lax.broadcasted_iota(jnp.int32, (64, 128), 1)
        r64 = r64 + (r64 & ~7)
        obits = (jnp.where(r64 > l64, jnp.uint32(0xFFFF), jnp.uint32(0))
                 | jnp.where(r64 + 8 > l64, jnp.uint32(0xFFFF0000), jnp.uint32(0)))
        z8 = jnp.zeros((8, 128), u32)
        lane16 = lax.broadcasted_iota(jnp.int32, (16, 128), 1)
        g_lo = (lane16 & 32) != 0
        g_hi = lane16 >= 64
        r40 = lax.broadcasted_iota(jnp.int32, (40, 128), 0)
        hrow = (r40 >= 10).astype(jnp.int32) + (r40 >= 20).astype(jnp.int32) + (r40 >= 30).astype(jnp.int32)
        hx = hrow ^ (lax.broadcasted_iota(jnp.int32, (40, 128), 1) >> 5)

        def nkeys(b):
            return min(b + 1, 3) if first else 3

        def place(g, vs, tok=None):
            parts = [z8] * 8
            if tok is not None:
                parts[(5 * g + 6) % 8] = pltpu.bitcast(tok, u32)
            for i, v in vs.items():
                parts[(5 * g + i) % 8] = v
            return jnp.concatenate(parts, axis=0)

        def stage1(u, slot, toks=()):
            b, g = divmod(u, NG)
            nk = nkeys(b)
            gb_ = g0 + b
            q5 = qT_s[q0 + b, 40 * g:40 * g + 40, :]
            ws = []
            for j in range(4):
                qm = jnp.where(hrow[8 * j:8 * j + 16] == j, q5[8 * j:8 * j + 16], jnp.uint32(0))
                ws.append(place(g, {j: qm[0:8], j + 1: qm[8:16]}))
            w = _unpack(jnp.concatenate(ws, axis=1))
            ln = slice(128 * g, 128 * g + 128)
            mx = [None]

            def emit(r0, sm):
                s_s[slot, r0:r0 + 16, :] = sm
                mx[0] = sm if mx[0] is None else jnp.maximum(mx[0], sm)

            if nk < 3:
                rows = [k_s[gb_, :, ln]]
                if nk == 2:
                    rows.append(k_s[gb_ - 1, :, ln])
                s = jnp.dot(_unpack(jnp.concatenate(rows, axis=0)), w, preferred_element_type=f32)
                for i in range(8):
                    old4 = jnp.concatenate([dd < 16 * i] * 4, axis=1)
                    emit(16 * i, jnp.where(old4, -1e30, s[16 * i:16 * i + 16]))
                for i in range(8, 8 * nk):
                    emit(16 * i, s[16 * i:16 * i + 16])
            else:
                def kb(B):
                    return k_s[gb_ - 2 + B // 4, 16 * (B % 4):16 * (B % 4) + 16, ln]
                fl = (lane16 - (80 * g) % 128) & 127
                h_hi = fl >= 40
                h_lo = ((fl >= 20) & (fl < 40)) | (fl >= 60)
                x = [kb(0), kb(1), kb(2), kb(11)]
                t = [jnp.where(h_lo, x[v ^ 1], x[v]) for v in range(4)]
                e_l = [jnp.where(h_hi, t[v ^ 2], t[v]) for v in range(4)]
                k9, k10 = kb(9), kb(10)
                j2_l = [jnp.where(h_hi, k10, x[2]), jnp.where(h_hi, x[2], k10)]
                sm = []
                for v in range(4):
                    j1_l = jnp.where((fl >= 20 * v) & (fl < 20 * v + 20), x[1], k9)
                    lhs = jnp.concatenate([e_l[v][0:8], j1_l[0:8], j2_l[v // 2][0:8],
                                           e_l[v][8:16], j1_l[8:16], j2_l[v // 2][8:16]], axis=0)
                    qm = jnp.where(hx == v, q5, jnp.uint32(0))
                    wv = place(g, {i: qm[8 * i:8 * i + 8] for i in range(5)}, toks[v] if v < len(toks) else None)
                    sm.append(jnp.dot(_unpack(lhs), _unpack(wv), preferred_element_type=f32))
                for c in range(2):
                    for J in (1, 2):
                        msk = (dd < 32 * J + 16 * c) & (lane16 >= 32 * J)
                        uu = [jnp.where(msk, sm[v][48 * c:48 * c + 16], sm[v][48 * c + 16 * J:48 * c + 16 * J + 16])
                              for v in range(4)]
                        t = [jnp.where(g_lo, uu[v ^ 1], uu[v]) for v in range(4)]
                        emit(32 * J + 16 * c,
                             jnp.concatenate([jnp.where(g_hi, t[v ^ 2], t[v]) for v in range(4)], axis=1))
                k8, k3 = kb(8), kb(3)
                lhs = jnp.concatenate([k8[0:8], k3[0:8], k8[8:16], k3[8:16], k_s[gb_ - 1, :, ln]], axis=0)
                s = jnp.dot(_unpack(lhs), w, preferred_element_type=f32)
                for c in range(2):
                    e0 = jnp.concatenate([sm[v][48 * c:48 * c + 16] for v in range(4)], axis=1)
                    e3 = jnp.concatenate([sm[v ^ 3][48 * c:48 * c + 16] for v in range(4)], axis=1)
                    old4 = jnp.concatenate([dd < 16 * c] * 4, axis=1)
                    emit(16 * c, jnp.where(old4, e0, s[32 * c:32 * c + 16]))
                    old4 = jnp.concatenate([dd < 96 + 16 * c] * 4, axis=1)
                    emit(96 + 16 * c, jnp.where(old4, s[32 * c + 16:32 * c + 32], e3))
                for i in range(8):
                    emit(128 + 16 * i, s[64 + 16 * i:64 + 16 * i + 16])
            st["m", u] = (jnp.max(mx[0], axis=0, keepdims=True), slot)
            return mx[0][0:8, 0:128]

        def stage2(u):
            b, g = divmod(u, NG)
            m, slot = st.pop(("m", u))
            nk = nkeys(b)
            gb_ = g0 + b
            res = []
            for j in range(4):
                hh = 4 * g + j
                off = DH * hh - 16 * ((DH * hh) // 16)
                ln = slice(128 * j, 128 * j + 128)
                mj = m[:, ln]

                def pp(r0):
                    return _packi(jnp.exp2(s_s[slot, r0:r0 + 128, ln] - mj))
                pm = pp(0)
                if nk == 3:
                    pold = pm & obits
                    p = jnp.concatenate([pold, pm ^ pold, pp(128)], axis=0)
                    blks = [gb_ - 2, gb_, gb_ - 1]
                elif nk == 2:
                    p = jnp.concatenate([pm, pp(128)], axis=0)
                    blks = [gb_, gb_ - 1]
                else:
                    p = pm
                    blks = [gb_]
                vw = _unpack(jnp.concatenate([vT_s[bb, 16 * hh:16 * hh + 16, :] for bb in blks], axis=1))
                o = jnp.dot(vw, _unpack(p), preferred_element_type=f32)
                if off < 8:
                    l, o3 = o[24:32], o[0:24]
                else:
                    l, o3 = o[0:8], o[8:32]
                r = pl.reciprocal(l, approx=True)
                r = r * (2.0 - l * r)
                res.append([o3[8 * i:8 * i + 8] * r for i in range(3)])
            out = []
            for j in (0, 2):
                a_, b_ = res[j], res[j + 1]
                out += [a_[0], a_[1], jnp.where(lo4, a_[2], b_[0]), b_[1], b_[2]]
            ot = 2 if (first and b == 0) else b
            oT_s[ot, 80 * g:80 * g + 80, :] = jnp.concatenate(out, axis=0)
            if u == NG - 1 and not first:
                oa_s[...] = _pack(oT_s[0].T)

        def wo_stage(r0, n):
            if second:
                oa_s[...] = _pack(oT_s[2].T)
            if r0 + n > QB:
                ob_s[...] = _pack(oT_s[1].T)
            ob = jnp.concatenate([r[...] for r in (oa_s, ob_s)[r0 // QB:(r0 + n) // QB]], axis=0)
            y = jnp.dot(_unpack(ob), weight(wo_v, wo_p, second), preferred_element_type=f32)
            x = x_v[pl.ds(pl.multiple_of((step - 1) * T + r0, QB), n), :].astype(f32)
            x1_s[r0:r0 + n, :] = x + modv(2, n) * y

        def ln23_chunk(c):
            y = _ln(_ln(x1_s[CH * c:CH * (c + 1), :]) * modv(4, CH) + modv(3, CH))
            y_s[CH // 2 * c:CH // 2 * (c + 1), :] = _pack(y)
            return token(y)

        def bias(b, n, toks):
            nt = b.shape[1] // 128
            b8 = jnp.broadcast_to(b, (8, b.shape[1]))
            tiles = [b8[:, 128 * j:128 * j + 128] for j in range(nt)]
            if isinstance(toks, dict):
                toks = list(toks.items())
            else:
                toks = [(i * nt // len(toks), t) for i, t in enumerate(toks)]
            for j, t in toks:
                tiles[j] = tiles[j] + t
            return _rep(jnp.concatenate(tiles, axis=1), n)

        def w1_stage(r0, n, toks=()):
            b1 = b1_v[...].astype(f32).reshape(1, F)
            raw = lax.dot_general(_unpack(y_s[r0 // 2:(r0 + n) // 2, :]), weight(w1t_v, w1_p, second, 0, FM),
                                  NT, preferred_element_type=f32)
            if callable(toks):
                toks = toks(raw)
            hh_s[r0 // 2:(r0 + n) // 2, :] = _pack(_gelu(raw + bias(b1[:, 0:FM], n, toks)))

        def w1_rem():
            b1 = b1_v[...].astype(f32).reshape(1, F)[:, FM:F]
            rt = lax.dot_general(weight(w1t_v, w1_p, second, FM, F), _unpack(y_s[...]), NT,
                                 preferred_element_type=f32)
            r = jnp.concatenate([rt[:, 0:QB], rt[:, QB:T]], axis=0).T
            hr_s[...] = _pack(_gelu(r + jnp.concatenate([b1, b1], axis=1)))

        def w2_stage(b, toks=(), strips=((0, D),)):
            r0 = QB * b
            b2 = bias(b2_v[...].astype(f32).reshape(1, D), QB, toks)
            if second and b == 0:
                wr = pltpu.bitcast(w2_v[FM:F, :], u32)
                zz = jnp.zeros_like(wr)
                w2_p[FM // 2:FM // 2 + 128, :] = jnp.concatenate([wr, zz, zz, wr], axis=0)
            wm = weight(w2_v, w2_p, second and b == 0, 0, FM)
            wr = _unpack(w2_p[FM // 2 + 64 * b:FM // 2 + 64 * b + 64, :])
            lhs = jnp.concatenate([hh_s[r0 // 2:(r0 + QB) // 2, :], hr_s[...]], axis=1)
            mo = jnp.dot(_unpack(lhs), jnp.concatenate([wm, wr], axis=0), preferred_element_type=f32) + b2
            rows = pl.ds(pl.multiple_of((step - 1) * T + r0, QB), QB)
            res = (x1_s[r0:r0 + QB, :] + modv(5, QB) * mo).astype(bf16)
            for c0, c1 in strips:
                o_v[rows, c0:c1] = res[:, c0:c1]
                pltpu.make_async_copy(o_v.at[rows, c0:c1], o_h.at[0, rows, c0:c1], osem.at[0]).start()

        def wt_cols(dst, c0, t):
            w = wqkv_v[128 * t:128 * t + 128, c0:c0 + D].astype(f32).T
            dst[:, 128 * t:128 * t + 128] = _pack(w)
            return token(w[D - 16:D])

        if first:
            def seg(k, c0, c1, r0, r1):
                lo, hi = 128 * k, 128 * k + 128
                h = n_s[r0:r1, lo:hi] * _rep(mod_s[:, D + lo:D + hi], r1 - r0) + _rep(mod_s[:, lo:hi], r1 - r0)
                lhs = _unpack(_packi(h)) if c0 == 2 * D else h.astype(bf16)
                w = wqkv_v[lo:hi, c0:c1]
                if r0 == 0 and c1 == 2 * D:
                    wk_p[lo // 2:hi // 2, :] = pltpu.bitcast(w[:, c1 - c0 - D:], u32)
                r = jnp.dot(lhs, w, preferred_element_type=f32)
                return r if k == 0 else r + acc_s[r0:r1, c0:c1]

            def segment(k, blocks):
                for b in blocks:
                    r0, r1 = QB * b, QB * b + QB
                    acc_s[r0:r1, 0:2 * D] = seg(k, 0, 2 * D, r0, r1)
                    acc_s[r0:r1, 2 * D:3 * D] = seg(k, 2 * D, 3 * D, r0, r1)

            def norm(c0, c1):
                for c in range(c0, c1):
                    n_s[CH * c:CH * (c + 1), :] = _ln(x_v[CH * c:CH * (c + 1), :].astype(f32))

            def fin(which, b0, b1):
                r = seg(4, which * D, (which + 1) * D, QB * b0, QB * b1)
                for b in range(b0, b1):
                    rb = r[QB * (b - b0):QB * (b - b0 + 1)]
                    if which == 0:
                        qT_s[b] = _pack((rb * QSCALE).T)
                    elif which == 1:
                        kstore(rb, b)
                    else:
                        vstore(rb.T, b)

            for n in names:
                cp(n).start()
            wait("c", "x0")
            norm(0, NCH)
            wait("sa0", "ca0")
            col_s[...] = jnp.broadcast_to(silu_c().astype(f32), (128, D)).T
            mod_mxu([0, 5])
            wait("r0")
            segment(0, [0])
            wait("x1")
            norm(NCH, 2 * NCH)
            segment(0, [1, 2])
            wait("sa1", "ca1")
            mod_vpu([1, 6], 16)
            segment(0, [3])
            wait("r1")
            segment(1, [0, 1, 2])
            for k in (2, 3):
                wait("sa%d" % k, "ca%d" % k, "r%d" % k)
                mod_vpu([k, k + 5], 16)
                segment(k - 1, [3])
                segment(k, [0, 1, 2])
            wait("sa4", "ca4", "r4")
            mod_vpu([4, 9], 16)
            segment(3, [3])
            fin(2, 0, 2)
            fin(0, 0, 2)
            fin(1, 0, 2)
            fin(2, 2, 4)
            order = [u for g in range(NG) for u in (NG + g, g)]
            stage1(order[0], 0)
            stage1(order[1], 1)
            for i, u in enumerate(order):
                if i + 2 < NU:
                    stage1(order[i + 2], (i + 2) % 3)
                if i == 6:
                    fin(0, 2, 4)
                if i == NU - 2:
                    fin(1, 2, 3)
                stage2(u)
            fin(1, 3, 4)
            wait("wm2", "wo")
        elif variant in ("second", "mid"):
            if second:
                mod_vpu([15, 20, 10, 16, 21, 17, 11, 22, 18, 23, 12, 19, 24, 14, 13], 16)
            else:
                kf = jnp.dot(_unpack(hb_s[...]), _unpack(wk_p[...]), preferred_element_type=f32)
                for b in range(2):
                    kstore(kf[QB * b:QB * b + QB], g0 + b)
                wo_stage(0, T)
                qf = lax.dot_general(_unpack(wqT_s[...]), _unpack(hb_s[...]), NT, preferred_element_type=f32)
                for b in range(2):
                    qT_s[b] = _pack(qf[:, QB * b:QB * b + QB] * QSCALE)
                vf = lax.dot_general(_unpack(wvT_s[...]), _unpack(hi_s[...]), NT, preferred_element_type=f32)
                for b in range(2):
                    vstore(vf[:, QB * b:QB * b + QB], g0 + b)
                an = [z[r:r + 8, 128 * b:128 * b + 128] for z in (qf, vf) for b in range(2)
                      for r in range(0, 576, 96)]
                for c in range(NCH):
                    anchor_x1(an[c])
                    ln23_chunk(c)
            a1 = stage1(0, 0)
            if second:
                wo_stage(0, T)
            pend = {}
            done23 = 0 if second else NCH
            for u in range(NU):
                if u == NU - 2:
                    if second:
                        wait("x2", "b1", "b2", "w1")
                    nxt = jnp.minimum(step + 1, NS - 1)
                    t1 = [ln1_chunk(c, nxt) for c in range(NCH)]
                    w1_stage(0, T, t1 if second else t1[0:12])
                    w1_rem()
                if done23 < NCH and u >= 3:
                    anchor_x1(a1)
                    hi23 = min(NCH, -(-NCH * (u - 2) // 10))
                    pend[u + 3] = [ln23_chunk(c) for c in range(done23, hi23)]
                    done23 = hi23
                if u + 1 < NU:
                    a1 = stage1(u + 1, (u + 1) % 2, pend.pop(u + 1, ()))
                elif second:
                    wait("wm3", "w2")
                    mod_vpu(range(25, 30), 8)
                    w2_stage(0, [wt_cols(wqT_s, 0, t) for t in range(5)])
                else:
                    w2_stage(0, t1[12:])
                stage2(u)
            w2_stage(1, [wt_cols(wvT_s, 2 * D, t) for t in range(5)] if second else ())
            if second:
                wait("xr")
        else:
            wo_stage(0, QB)
            for c in range(NCH // 2):
                ln23_chunk(c)
            wo_stage(QB, QB)

            def ln23_b(raw):
                toks = {}
                for i in range(NCH // 2):
                    anchor_x1(raw[0:8, 128 * i:128 * i + 128])
                    toks[i + 5] = ln23_chunk(NCH // 2 + i)
                return toks

            w1_stage(0, QB, ln23_b)
            w1_stage(QB, QB)
            w1_rem()
            w2_stage(0)
            w2_stage(1, (), ((0, 512), (512, D)))
            pltpu.make_async_copy(o_v, o_h.at[0], osem.at[0]).wait()

    @pl.when(step == 0)
    def _():
        body("first")

    @pl.when(step == 1)
    def _():
        body("second")

    @pl.when((step > 1) & (step < NS))
    def _():
        body("mid")

    @pl.when(step == NS)
    def _():
        body("last")


@jax.jit
def pallas_adaLN_cond__sliding_block__mixer_channel_mlp__prompt_kernel(
    A_x: jax.Array,
    A_wqkv: jax.Array,
    A_wo: jax.Array,
    B_x: jax.Array,
    B_w1: jax.Array,
    B_b1: jax.Array,
    B_w2: jax.Array,
    B_b2: jax.Array,
    c: jax.Array,
    w_mod: jax.Array,
):
    del B_x
    anyspec = pl.BlockSpec(memory_space=pl.ANY)
    V = pltpu.VMEM
    return pl.pallas_call(
        _kernel,
        grid=(NS + 1,),
        in_specs=[anyspec] * 9,
        out_specs=anyspec,
        out_shape=jax.ShapeDtypeStruct((1, S, D), bf16),
        scratch_shapes=[
            V((S, D), bf16), V((1, D), bf16), V((F,), bf16), V((D,), bf16),
            V((D, 3 * D), bf16), V((D, D), bf16), V((F, D), bf16), V((F, D), bf16),
            V((D, 6 * D), bf16), V((S, D), bf16),
            pltpu.SemaphoreType.DMA((27,)), pltpu.SemaphoreType.DMA((1,)),
            V((8, 6 * D), f32), V((D, 128), f32),
            V((D // 2, D), u32), V((D // 2, D), u32), V((D // 2, D), u32), V((D // 2, D), u32),
            V((F // 2, D), u32), V((FM // 2 + 128, D), u32),
            V((NB, QB // 2, 128 * NG), u32), V((NB, 16 * H, QB), u32), V((4, D // 2, QB), u32),
            V((3, 256, 512), f32), V((3, D, QB), f32), V((QB // 2, D), u32), V((QB // 2, D), u32),
            V((T // 2, D), u32), V((T // 2, D), u32), V((T + 8, D), f32), V((T // 2, D), u32),
            V((T // 2, FM), u32), V((QB // 2, 128), u32),
            V((2 * T, D), f32), V((2 * T, 3 * D), f32),
        ],
        compiler_params=pltpu.CompilerParams(
            dimension_semantics=("arbitrary",),
            vmem_limit_bytes=100 * 1024 * 1024,
            disable_bounds_checks=True,
            disable_semaphore_checks=True,
        ),
    )(A_x, c, B_b1, B_b2, A_wqkv, A_wo, B_w1.T, B_w2, w_mod)
```

```python
import jax
import jax.numpy as jnp
from jax import lax
import jax.experimental.pallas as pl
import jax.experimental.pallas.tpu as pltpu

S, D, H, DH, F = 2048, 640, 32, 20, 1728
T = 256
QB = 128
NB = S // QB
NS = S // T
NG = 8
NU = 2 * NG
CH = 16
NCH = T // CH
FM = 1664
EPS = 1e-5
QSCALE = DH ** -0.5 * 1.4426950408889634
f32, bf16, u32 = jnp.float32, jnp.bfloat16, jnp.uint32
NT = (((1,), (1,)), ((), ()))


def _ln(x):
    m = jnp.sum(x, axis=-1, keepdims=True) * (1.0 / D)
    v = jnp.sum(x * x, axis=-1, keepdims=True) * (1.0 / D) - m * m
    return (x - m) * lax.rsqrt(jnp.maximum(v, 0.0) + EPS)


def _pack(x):
    return pltpu.bitcast(x.astype(bf16), u32)


def _unpack(x):
    return pltpu.bitcast(x, bf16)


def _rep(v, n):
    return jnp.concatenate([v] * (n // 8), axis=0)


def _gelu(x):
    c = 0.7978845608028654
    return 0.5 * x * (1.0 + jnp.tanh(x * (c + (c * 0.044715) * (x * x))))


def _kernel(x_h, c_h, b1_h, b2_h, wqkv_h, wo_h, w1t_h, w2_h, wmod_h, o_h,
            x_v, c_v, b1_v, b2_v, wqkv_v, wo_v, w1t_v, w2_v, wmod_v, o_v, sems, osem,
            mod_s, col_s, wqT_s, wvT_s, wk_p, wo_p, w1_p, w2_p,
            k_s, vT_s, qT_s, s_s, oT_s, oa_s, ob_s, hb_s, x1_s, y_s, hh_s, hr_s,
            n_s, acc_s):
    step = pl.program_id(0)
    dyn0 = step >> 10

    def xrows(lo, hi):
        return x_h.at[0, lo:hi], x_v.at[lo:hi]

    def wmcols(lo, hi):
        return wmod_h.at[:, lo:hi], wmod_v.at[:, lo:hi]

    def wrows(lo, hi):
        return wqkv_h.at[lo:hi], wqkv_v.at[lo:hi]

    pairs = dict(c=(c_h, c_v), x0=xrows(0, T))
    for k in range(5):
        pairs["sa%d" % k] = wmcols(128 * k, 128 * k + 128)
        pairs["ca%d" % k] = wmcols(D + 128 * k, D + 128 * k + 128)
        pairs["r%d" % k] = wrows(128 * k, 128 * k + 128)
        if k == 0:
            pairs["x1"] = xrows(T, 2 * T)
    pairs.update(
        wm2=wmcols(2 * D, 5 * D), wo=(wo_h, wo_v), x2=xrows(2 * T, 3 * T),
        b1=(b1_h, b1_v), b2=(b2_h, b2_v), w1=(w1t_h, w1t_v),
        wm3=wmcols(5 * D, 6 * D), w2=(w2_h, w2_v), xr=xrows(3 * T, S),
    )
    names = list(pairs)

    def cp(n):
        s, d = pairs[n]
        return pltpu.make_async_copy(s, d, sems.at[names.index(n)])

    def wait(*ns):
        for n in ns:
            cp(n).wait()

    def silu_c():
        c = c_v[...].astype(f32)
        return (c * jax.nn.sigmoid(c)).astype(bf16)

    def modv(i, n):
        return _rep(mod_s[:, i * D:(i + 1) * D], n)

    def mod_put(t, v):
        mod_s[:, 128 * t:128 * t + 128] = v + 1.0 if t // 5 in (1, 4) else v

    def mod_mxu(tiles):
        w = jnp.concatenate([wmod_v[:, 128 * t:128 * t + 128] for t in tiles], axis=1)
        r = jnp.dot(jnp.broadcast_to(silu_c(), (16, D)), w, preferred_element_type=f32)[0:8]
        for i, t in enumerate(tiles):
            mod_put(t, r[:, 128 * i:128 * i + 128])

    def mod_vpu(tiles, mw):
        acc = jnp.zeros((mw, 128), f32)
        for t in tiles:
            acc = jnp.where(dyn0 == 1, acc, 0.0)
            for r in range(D // mw):
                rows = slice(mw * r, mw * r + mw)
                acc = acc + wmod_v[rows, 128 * t:128 * t + 128].astype(f32) * col_s[rows, :]
            mod_put(t, jnp.broadcast_to(jnp.sum(acc, axis=0, keepdims=True), (8, 128)))

    def token(v):
        return jnp.where(dyn0 == 1, v[0:8, 0:128], jnp.where(dyn0 == 2, v[8:16, 0:128], 0.0))

    def body(variant):
        first = variant == "first"
        second = variant == "second"
        g0 = step * (T // QB)
        q0 = 2 if second else 0
        lo4 = lax.broadcasted_iota(jnp.int32, (8, QB), 0) < 4
        st = {}

        def weight(w_v, w_p, fresh, lo=0, hi=None):
            hi = w_v.shape[0] if hi is None else hi
            if fresh:
                w = w_v[lo:hi, :]
                w_p[lo // 2:hi // 2, :] = pltpu.bitcast(w, u32)
                return w
            return _unpack(w_p[lo // 2:hi // 2, :])

        def anchor_x1(v):
            x1_s[pl.ds(pl.multiple_of(T + 8 * dyn0, 8), 8), 0:128] = v

        def ln1_chunk(c, blk):
            x = x_v[pl.ds(pl.multiple_of(blk * T + CH * c, CH), CH), :].astype(f32)
            h = _ln(x) * modv(1, CH) + modv(0, CH)
            hb_s[CH // 2 * c:CH // 2 * (c + 1), :] = _pack(h)
            return token(h)

        def kstore(kb, blk):
            lane = lax.broadcasted_iota(jnp.int32, (QB, 128), 1)
            tiles = []
            for g in range(NG):
                t0, t1 = (80 * g) // 128, (80 * g + 79) // 128
                if t0 == t1:
                    tiles.append(kb[:, 128 * t0:128 * t0 + 128])
                else:
                    tiles.append(jnp.where(lane >= 64, kb[:, 128 * t0:128 * t0 + 128],
                                           kb[:, 128 * t1:128 * t1 + 128]))
            k_s[blk] = _pack(jnp.concatenate(tiles, axis=1))

        def vstore(src, blk):
            fl = jnp.ones((8, QB), f32)
            out = []
            for hh in range(H):
                a = (DH * hh) // 16
                off = DH * hh - 16 * a
                v = [src[16 * a + 8 * i:16 * a + 8 * i + 8] for i in range(4)]
                if off == 0:
                    out += [v[0], v[1], jnp.where(lo4, v[2], fl), fl]
                elif off == 4:
                    out += [jnp.where(lo4, fl, v[0]), v[1], v[2], fl]
                elif off == 8:
                    out += [fl, v[1], v[2], jnp.where(lo4, v[3], fl)]
                else:
                    out += [fl, jnp.where(lo4, fl, v[1]), v[2], v[3]]
            vT_s[blk] = _pack(jnp.concatenate(out, axis=0))

        dd = (lax.broadcasted_iota(jnp.int32, (16, 128), 1)
              - lax.broadcasted_iota(jnp.int32, (16, 128), 0))
        old = jnp.concatenate([dd < 16 * i for i in range(8)], axis=0)
        z8 = jnp.zeros((8, 128), u32)
        lane16 = lax.broadcasted_iota(jnp.int32, (16, 128), 1)
        g_lo = (lane16 & 32) != 0
        g_hi = lane16 >= 64
        r40 = lax.broadcasted_iota(jnp.int32, (40, 128), 0)
        hrow = (r40 >= 10).astype(jnp.int32) + (r40 >= 20).astype(jnp.int32) + (r40 >= 30).astype(jnp.int32)
        hx = hrow ^ (lax.broadcasted_iota(jnp.int32, (40, 128), 1) >> 5)

        def nkeys(b):
            return min(b + 1, 3) if first else 3

        def place(g, vs, tok=None):
            parts = [z8] * 8
            if tok is not None:
                parts[(5 * g + 6) % 8] = pltpu.bitcast(tok, u32)
            for i, v in vs.items():
                parts[(5 * g + i) % 8] = v
            return jnp.concatenate(parts, axis=0)

        def stage1(u, slot, toks=()):
            b, g = divmod(u, NG)
            nk = nkeys(b)
            gb_ = g0 + b
            q5 = qT_s[q0 + b, 40 * g:40 * g + 40, :]
            ws = []
            for j in range(4):
                qm = jnp.where(hrow[8 * j:8 * j + 16] == j, q5[8 * j:8 * j + 16], jnp.uint32(0))
                ws.append(place(g, {j: qm[0:8], j + 1: qm[8:16]}))
            w = _unpack(jnp.concatenate(ws, axis=1))
            ln = slice(128 * g, 128 * g + 128)
            mx = [None]

            def emit(r0, sm):
                s_s[slot, r0:r0 + 16, :] = sm
                mx[0] = sm if mx[0] is None else jnp.maximum(mx[0], sm)

            if nk < 3:
                rows = [k_s[gb_, :, ln]]
                if nk == 2:
                    rows.append(k_s[gb_ - 1, :, ln])
                s = jnp.dot(_unpack(jnp.concatenate(rows, axis=0)), w, preferred_element_type=f32)
                for i in range(8):
                    old4 = jnp.concatenate([dd < 16 * i] * 4, axis=1)
                    emit(16 * i, jnp.where(old4, -1e30, s[16 * i:16 * i + 16]))
                for i in range(8, 8 * nk):
                    emit(16 * i, s[16 * i:16 * i + 16])
            else:
                def kb(B):
                    return k_s[gb_ - 2 + B // 4, 16 * (B % 4):16 * (B % 4) + 16, ln]
                fl = (lane16 - (80 * g) % 128) & 127
                h_hi = fl >= 40
                h_lo = ((fl >= 20) & (fl < 40)) | (fl >= 60)
                x = [kb(0), kb(1), kb(2), kb(11)]
                t = [jnp.where(h_lo, x[v ^ 1], x[v]) for v in range(4)]
                e_l = [jnp.where(h_hi, t[v ^ 2], t[v]) for v in range(4)]
                k9, k10 = kb(9), kb(10)
                j2_l = [jnp.where(h_hi, k10, x[2]), jnp.where(h_hi, x[2], k10)]
                sm = []
                for v in range(4):
                    j1_l = jnp.where((fl >= 20 * v) & (fl < 20 * v + 20), x[1], k9)
                    lhs = jnp.concatenate([e_l[v][0:8], j1_l[0:8], j2_l[v // 2][0:8],
                                           e_l[v][8:16], j1_l[8:16], j2_l[v // 2][8:16]], axis=0)
                    qm = jnp.where(hx == v, q5, jnp.uint32(0))
                    wv = place(g, {i: qm[8 * i:8 * i + 8] for i in range(5)}, toks[v] if v < len(toks) else None)
                    sm.append(jnp.dot(_unpack(lhs), _unpack(wv), preferred_element_type=f32))
                for c in range(2):
                    for J in (1, 2):
                        msk = (dd < 32 * J + 16 * c) & (lane16 >= 32 * J)
                        uu = [jnp.where(msk, sm[v][48 * c:48 * c + 16], sm[v][48 * c + 16 * J:48 * c + 16 * J + 16])
                              for v in range(4)]
                        t = [jnp.where(g_lo, uu[v ^ 1], uu[v]) for v in range(4)]
                        emit(32 * J + 16 * c,
                             jnp.concatenate([jnp.where(g_hi, t[v ^ 2], t[v]) for v in range(4)], axis=1))
                k8, k3 = kb(8), kb(3)
                lhs = jnp.concatenate([k8[0:8], k3[0:8], k8[8:16], k3[8:16], k_s[gb_ - 1, :, ln]], axis=0)
                s = jnp.dot(_unpack(lhs), w, preferred_element_type=f32)
                for c in range(2):
                    e0 = jnp.concatenate([sm[v][48 * c:48 * c + 16] for v in range(4)], axis=1)
                    e3 = jnp.concatenate([sm[v ^ 3][48 * c:48 * c + 16] for v in range(4)], axis=1)
                    old4 = jnp.concatenate([dd < 16 * c] * 4, axis=1)
                    emit(16 * c, jnp.where(old4, e0, s[32 * c:32 * c + 16]))
                    old4 = jnp.concatenate([dd < 96 + 16 * c] * 4, axis=1)
                    emit(96 + 16 * c, jnp.where(old4, s[32 * c + 16:32 * c + 32], e3))
                for i in range(8):
                    emit(128 + 16 * i, s[64 + 16 * i:64 + 16 * i + 16])
            st["m", u] = (jnp.max(mx[0], axis=0, keepdims=True), slot)
            return mx[0][0:8, 0:128]

        def stage2(u):
            b, g = divmod(u, NG)
            m, slot = st.pop(("m", u))
            nk = nkeys(b)
            gb_ = g0 + b
            res = []
            for j in range(4):
                hh = 4 * g + j
                off = DH * hh - 16 * ((DH * hh) // 16)
                ln = slice(128 * j, 128 * j + 128)
                mj = m[:, ln]

                e = jnp.exp2(s_s[slot, 0:128 * min(nk, 2), ln] - mj)
                if nk == 3:
                    eo = jnp.where(old, e[0:128], 0.0)
                    e = jnp.concatenate([eo, e[0:128] - eo, e[128:256]], axis=0)
                blks = [[gb_], [gb_, gb_ - 1], [gb_ - 2, gb_, gb_ - 1]][nk - 1]
                vw = _unpack(jnp.concatenate([vT_s[bb, 16 * hh:16 * hh + 16, :] for bb in blks], axis=1))
                o = jnp.dot(vw, e.astype(bf16), preferred_element_type=f32)
                if off < 8:
                    l, o3 = o[24:32], o[0:24]
                else:
                    l, o3 = o[0:8], o[8:32]
                r = pl.reciprocal(l, approx=True)
                r = r * (2.0 - l * r)
                res.append([o3[8 * i:8 * i + 8] * r for i in range(3)])
            out = []
            for j in (0, 2):
                a_, b_ = res[j], res[j + 1]
                out += [a_[0], a_[1], jnp.where(lo4, a_[2], b_[0]), b_[1], b_[2]]
            ot = 2 if (first and b == 0) else b
            oT_s[ot, 80 * g:80 * g + 80, :] = jnp.concatenate(out, axis=0)
            if u == NG - 1 and not first:
                oa_s[...] = _pack(oT_s[0].T)

        def wo_stage(r0, n):
            if second:
                oa_s[...] = _pack(oT_s[2].T)
            if r0 + n > QB:
                ob_s[...] = _pack(oT_s[1].T)
            ob = jnp.concatenate([r[...] for r in (oa_s, ob_s)[r0 // QB:(r0 + n) // QB]], axis=0)
            y = jnp.dot(_unpack(ob), weight(wo_v, wo_p, second), preferred_element_type=f32)
            x = x_v[pl.ds(pl.multiple_of((step - 1) * T + r0, QB), n), :].astype(f32)
            x1_s[r0:r0 + n, :] = x + modv(2, n) * y

        def ln23_chunk(c):
            y = _ln(_ln(x1_s[CH * c:CH * (c + 1), :]) * modv(4, CH) + modv(3, CH))
            y_s[CH // 2 * c:CH // 2 * (c + 1), :] = _pack(y)
            return token(y)

        def bias(b, n, toks):
            nt = b.shape[1] // 128
            b8 = jnp.broadcast_to(b, (8, b.shape[1]))
            tiles = [b8[:, 128 * j:128 * j + 128] for j in range(nt)]
            if isinstance(toks, dict):
                toks = list(toks.items())
            else:
                toks = [(i * nt // len(toks), t) for i, t in enumerate(toks)]
            for j, t in toks:
                tiles[j] = tiles[j] + t
            return _rep(jnp.concatenate(tiles, axis=1), n)

        def w1_stage(r0, n, toks=()):
            b1 = b1_v[...].astype(f32).reshape(1, F)
            raw = lax.dot_general(_unpack(y_s[r0 // 2:(r0 + n) // 2, :]), weight(w1t_v, w1_p, second, 0, FM),
                                  NT, preferred_element_type=f32)
            if callable(toks):
                toks = toks(raw)
            hh_s[r0 // 2:(r0 + n) // 2, :] = _pack(_gelu(raw + bias(b1[:, 0:FM], n, toks)))

        def w1_rem():
            b1 = b1_v[...].astype(f32).reshape(1, F)[:, FM:F]
            rt = lax.dot_general(weight(w1t_v, w1_p, second, FM, F), _unpack(y_s[...]), NT,
                                 preferred_element_type=f32)
            r = jnp.concatenate([rt[:, 0:QB], rt[:, QB:T]], axis=0).T
            hr_s[...] = _pack(_gelu(r + jnp.concatenate([b1, b1], axis=1)))

        def w2_stage(b, toks=(), strips=((0, D),)):
            r0 = QB * b
            b2 = bias(b2_v[...].astype(f32).reshape(1, D), QB, toks)
            if second and b == 0:
                wr = pltpu.bitcast(w2_v[FM:F, :], u32)
                zz = jnp.zeros_like(wr)
                w2_p[FM // 2:FM // 2 + 128, :] = jnp.concatenate([wr, zz, zz, wr], axis=0)
            wm = weight(w2_v, w2_p, second and b == 0, 0, FM)
            wr = _unpack(w2_p[FM // 2 + 64 * b:FM // 2 + 64 * b + 64, :])
            lhs = jnp.concatenate([hh_s[r0 // 2:(r0 + QB) // 2, :], hr_s[...]], axis=1)
            mo = jnp.dot(_unpack(lhs), jnp.concatenate([wm, wr], axis=0), preferred_element_type=f32) + b2
            rows = pl.ds(pl.multiple_of((step - 1) * T + r0, QB), QB)
            res = (x1_s[r0:r0 + QB, :] + modv(5, QB) * mo).astype(bf16)
            for c0, c1 in strips:
                o_v[rows, c0:c1] = res[:, c0:c1]
                pltpu.make_async_copy(o_v.at[rows, c0:c1], o_h.at[0, rows, c0:c1], osem.at[0]).start()

        def wt_cols(dst, c0, t):
            w = wqkv_v[128 * t:128 * t + 128, c0:c0 + D].astype(f32).T
            dst[:, 128 * t:128 * t + 128] = _pack(w)
            return token(w[D - 16:D])

        if first:
            def seg(k, c0, c1, r0, r1):
                lo, hi = 128 * k, 128 * k + 128
                h = n_s[r0:r1, lo:hi] * _rep(mod_s[:, D + lo:D + hi], r1 - r0) + _rep(mod_s[:, lo:hi], r1 - r0)
                lhs = h.astype(bf16)
                w = wqkv_v[lo:hi, c0:c1]
                if r0 == 0 and c1 == 2 * D:
                    wk_p[lo // 2:hi // 2, :] = pltpu.bitcast(w[:, c1 - c0 - D:], u32)
                r = jnp.dot(lhs, w, preferred_element_type=f32)
                return r if k == 0 else r + acc_s[r0:r1, c0:c1]

            def segment(k, blocks):
                for b in blocks:
                    r0, r1 = QB * b, QB * b + QB
                    acc_s[r0:r1, 0:2 * D] = seg(k, 0, 2 * D, r0, r1)
                    acc_s[r0:r1, 2 * D:3 * D] = seg(k, 2 * D, 3 * D, r0, r1)

            def norm(c0, c1):
                for c in range(c0, c1):
                    n_s[CH * c:CH * (c + 1), :] = _ln(x_v[CH * c:CH * (c + 1), :].astype(f32))

            def fin(which, b0, b1):
                r = seg(4, which * D, (which + 1) * D, QB * b0, QB * b1)
                for b in range(b0, b1):
                    rb = r[QB * (b - b0):QB * (b - b0 + 1)]
                    if which == 0:
                        qT_s[b] = _pack((rb * QSCALE).T)
                    elif which == 1:
                        kstore(rb, b)
                    else:
                        vstore(rb.T, b)

            for n in names:
                cp(n).start()
            wait("c", "x0")
            norm(0, NCH)
            wait("sa0", "ca0")
            col_s[...] = jnp.broadcast_to(silu_c().astype(f32), (128, D)).T
            mod_mxu([0, 5])
            wait("r0")
            segment(0, [0])
            wait("x1")
            norm(NCH, 2 * NCH)
            segment(0, [1, 2])
            wait("sa1", "ca1")
            mod_vpu([1, 6], 16)
            segment(0, [3])
            wait("r1")
            segment(1, [0, 1, 2])
            for k in (2, 3):
                wait("sa%d" % k, "ca%d" % k, "r%d" % k)
                mod_vpu([k, k + 5], 16)
                segment(k - 1, [3])
                segment(k, [0, 1, 2])
            wait("sa4", "ca4", "r4")
            mod_vpu([4, 9], 16)
            segment(3, [3])
            fin(2, 0, 2)
            fin(0, 0, 2)
            fin(1, 0, 2)
            fin(2, 2, 4)
            order = [u for g in range(NG) for u in (NG + g, g)]
            stage1(order[0], 0)
            stage1(order[1], 1)
            for i, u in enumerate(order):
                if i + 2 < NU:
                    stage1(order[i + 2], (i + 2) % 3)
                if i == 6:
                    fin(0, 2, 4)
                if i == NU - 2:
                    fin(1, 2, 3)
                stage2(u)
            fin(1, 3, 4)
            wait("wm2", "wo")
        elif variant in ("second", "mid"):
            if second:
                mod_vpu([15, 20, 10, 16, 21, 17, 11, 22, 18, 23, 12, 19, 24, 14, 13], 16)
            else:
                kf = jnp.dot(_unpack(hb_s[...]), _unpack(wk_p[...]), preferred_element_type=f32)
                for b in range(2):
                    kstore(kf[QB * b:QB * b + QB], g0 + b)
                wo_stage(0, T)
                qf = lax.dot_general(_unpack(wqT_s[...]), _unpack(hb_s[...]), NT, preferred_element_type=f32)
                for b in range(2):
                    qT_s[b] = _pack(qf[:, QB * b:QB * b + QB] * QSCALE)
                vf = lax.dot_general(_unpack(wvT_s[...]), _unpack(hb_s[...]), NT, preferred_element_type=f32)
                for b in range(2):
                    vstore(vf[:, QB * b:QB * b + QB], g0 + b)
                an = [z[r:r + 8, 128 * b:128 * b + 128] for z in (qf, vf) for b in range(2)
                      for r in range(0, 576, 96)]
                for c in range(NCH):
                    anchor_x1(an[c])
                    ln23_chunk(c)
            a1 = stage1(0, 0)
            if second:
                wo_stage(0, T)
            pend = {}
            done23 = 0 if second else NCH
            for u in range(NU):
                if u == NU - 2:
                    if second:
                        wait("x2", "b1", "b2", "w1")
                    nxt = jnp.minimum(step + 1, NS - 1)
                    t1 = [ln1_chunk(c, nxt) for c in range(NCH)]
                    w1_stage(0, T, t1 if second else t1[0:12])
                    w1_rem()
                if done23 < NCH and u >= 3:
                    anchor_x1(a1)
                    hi23 = min(NCH, -(-NCH * (u - 2) // 10))
                    pend[u + 3] = [ln23_chunk(c) for c in range(done23, hi23)]
                    done23 = hi23
                if u + 1 < NU:
                    a1 = stage1(u + 1, (u + 1) % 2, pend.pop(u + 1, ()))
                elif second:
                    wait("wm3", "w2")
                    mod_vpu(range(25, 30), 8)
                    w2_stage(0, [wt_cols(wqT_s, 0, t) for t in range(5)])
                else:
                    w2_stage(0, t1[12:])
                stage2(u)
            w2_stage(1, [wt_cols(wvT_s, 2 * D, t) for t in range(5)] if second else ())
            if second:
                wait("xr")
        else:
            wo_stage(0, QB)
            for c in range(NCH // 2):
                ln23_chunk(c)
            wo_stage(QB, QB)

            def ln23_b(raw):
                toks = {}
                for i in range(NCH // 2):
                    anchor_x1(raw[0:8, 128 * i:128 * i + 128])
                    toks[i + 5] = ln23_chunk(NCH // 2 + i)
                return toks

            w1_stage(0, QB, ln23_b)
            w1_stage(QB, QB)
            w1_rem()
            w2_stage(0)
            w2_stage(1, (), ((0, 512), (512, D)))
            pltpu.make_async_copy(o_v, o_h.at[0], osem.at[0]).wait()

    @pl.when(step == 0)
    def _():
        body("first")

    @pl.when(step == 1)
    def _():
        body("second")

    @pl.when((step > 1) & (step < NS))
    def _():
        body("mid")

    @pl.when(step == NS)
    def _():
        body("last")


@jax.jit
def pallas_adaLN_cond__sliding_block__mixer_channel_mlp__prompt_kernel(
    A_x: jax.Array,
    A_wqkv: jax.Array,
    A_wo: jax.Array,
    B_x: jax.Array,
    B_w1: jax.Array,
    B_b1: jax.Array,
    B_w2: jax.Array,
    B_b2: jax.Array,
    c: jax.Array,
    w_mod: jax.Array,
):
    del B_x
    anyspec = pl.BlockSpec(memory_space=pl.ANY)
    V = pltpu.VMEM
    return pl.pallas_call(
        _kernel,
        grid=(NS + 1,),
        in_specs=[anyspec] * 9,
        out_specs=anyspec,
        out_shape=jax.ShapeDtypeStruct((1, S, D), bf16),
        scratch_shapes=[
            V((S, D), bf16), V((1, D), bf16), V((F,), bf16), V((D,), bf16),
            V((D, 3 * D), bf16), V((D, D), bf16), V((F, D), bf16), V((F, D), bf16),
            V((D, 6 * D), bf16), V((S, D), bf16),
            pltpu.SemaphoreType.DMA((27,)), pltpu.SemaphoreType.DMA((1,)),
            V((8, 6 * D), f32), V((D, 128), f32),
            V((D // 2, D), u32), V((D // 2, D), u32), V((D // 2, D), u32), V((D // 2, D), u32),
            V((F // 2, D), u32), V((FM // 2 + 128, D), u32),
            V((NB, QB // 2, 128 * NG), u32), V((NB, 16 * H, QB), u32), V((4, D // 2, QB), u32),
            V((3, 256, 512), f32), V((3, D, QB), f32), V((QB // 2, D), u32), V((QB // 2, D), u32),
            V((T // 2, D), u32), V((T + 8, D), f32), V((T // 2, D), u32),
            V((T // 2, FM), u32), V((QB // 2, 128), u32),
            V((2 * T, D), f32), V((2 * T, 3 * D), f32),
        ],
        compiler_params=pltpu.CompilerParams(
            dimension_semantics=("arbitrary",),
            vmem_limit_bytes=100 * 1024 * 1024,
            disable_bounds_checks=True,
            disable_semaphore_checks=True,
        ),
    )(A_x, c, B_b1, B_b2, A_wqkv, A_wo, B_w1.T, B_w2, w_mod)
```

```python
import jax
import jax.numpy as jnp
from jax import lax
import jax.experimental.pallas as pl
import jax.experimental.pallas.tpu as pltpu

S, D, H, DH, F = 2048, 640, 32, 20, 1728
T = 256
QB = 128
NB = S // QB
NS = S // T
NG = 8
NU = 2 * NG
CH = 16
NCH = T // CH
FM = 1664
EPS = 1e-5
QSCALE = DH ** -0.5 * 1.4426950408889634
f32, bf16, u32 = jnp.float32, jnp.bfloat16, jnp.uint32
NT = (((1,), (1,)), ((), ()))


def _ln(x):
    m = jnp.sum(x, axis=-1, keepdims=True) * (1.0 / D)
    v = jnp.sum(x * x, axis=-1, keepdims=True) * (1.0 / D) - m * m
    return (x - m) * lax.rsqrt(jnp.maximum(v, 0.0) + EPS)


def _pack(x):
    return pltpu.bitcast(x.astype(bf16), u32)


def _unpack(x):
    return pltpu.bitcast(x, bf16)


def _rep(v, n):
    return jnp.concatenate([v] * (n // 8), axis=0)


def _gelu(x):
    c = 0.7978845608028654
    return 0.5 * x * (1.0 + jnp.tanh(x * (c + (c * 0.044715) * (x * x))))


def _kernel(x_h, c_h, b1_h, b2_h, wqkv_h, wo_h, w1t_h, w2_h, wmod_h, o_h,
            x_v, c_v, b1_v, b2_v, wqkv_v, wo_v, w1t_v, w2_v, wmod_v, o_v, sems, osem,
            mod_s, col_s, wqT_s, wvT_s, wk_p, wo_p, w1_p, w2_p,
            k_s, vT_s, qT_s, s_s, oT_s, oa_s, ob_s, hb_s, x1_s, y_s, hh_s, hr_s,
            n_s, acc_s):
    step = pl.program_id(0)
    dyn0 = step >> 10

    def xrows(lo, hi):
        return x_h.at[0, lo:hi], x_v.at[lo:hi]

    def wmcols(lo, hi):
        return wmod_h.at[:, lo:hi], wmod_v.at[:, lo:hi]

    def wrows(lo, hi):
        return wqkv_h.at[lo:hi], wqkv_v.at[lo:hi]

    pairs = dict(c=(c_h, c_v), x0=xrows(0, T))
    for k in range(5):
        pairs["sa%d" % k] = wmcols(128 * k, 128 * k + 128)
        pairs["ca%d" % k] = wmcols(D + 128 * k, D + 128 * k + 128)
        pairs["r%d" % k] = wrows(128 * k, 128 * k + 128)
        if k == 0:
            pairs["x1"] = xrows(T, 2 * T)
    pairs.update(
        wm2=wmcols(2 * D, 5 * D), wo=(wo_h, wo_v), x2=xrows(2 * T, 3 * T),
        b1=(b1_h, b1_v), b2=(b2_h, b2_v), w1=(w1t_h, w1t_v),
        wm3=wmcols(5 * D, 6 * D), w2=(w2_h, w2_v), xr=xrows(3 * T, S),
    )
    names = list(pairs)

    def cp(n):
        s, d = pairs[n]
        return pltpu.make_async_copy(s, d, sems.at[names.index(n)])

    def wait(*ns):
        for n in ns:
            cp(n).wait()

    def silu_c():
        c = c_v[...].astype(f32)
        return (c * jax.nn.sigmoid(c)).astype(bf16)

    def modv(i, n):
        return _rep(mod_s[:, i * D:(i + 1) * D], n)

    def mod_put(t, v):
        mod_s[:, 128 * t:128 * t + 128] = v + 1.0 if t // 5 in (1, 4) else v

    def mod_mxu(tiles):
        w = jnp.concatenate([wmod_v[:, 128 * t:128 * t + 128] for t in tiles], axis=1)
        r = jnp.dot(jnp.broadcast_to(silu_c(), (16, D)), w, preferred_element_type=f32)[0:8]
        for i, t in enumerate(tiles):
            mod_put(t, r[:, 128 * i:128 * i + 128])

    def mod_vpu(tiles, mw):
        acc = jnp.zeros((mw, 128), f32)
        for t in tiles:
            acc = jnp.where(dyn0 == 1, acc, 0.0)
            for r in range(D // mw):
                rows = slice(mw * r, mw * r + mw)
                acc = acc + wmod_v[rows, 128 * t:128 * t + 128].astype(f32) * col_s[rows, :]
            mod_put(t, jnp.broadcast_to(jnp.sum(acc, axis=0, keepdims=True), (8, 128)))

    def token(v):
        return jnp.where(dyn0 == 1, v[0:8, 0:128], jnp.where(dyn0 == 2, v[8:16, 0:128], 0.0))

    def body(variant):
        first = variant == "first"
        second = variant == "second"
        g0 = step * (T // QB)
        q0 = 2 if second else 0
        lo4 = lax.broadcasted_iota(jnp.int32, (8, QB), 0) < 4
        st = {}

        def weight(w_v, w_p, fresh, lo=0, hi=None):
            hi = w_v.shape[0] if hi is None else hi
            if fresh:
                w = w_v[lo:hi, :]
                w_p[lo // 2:hi // 2, :] = pltpu.bitcast(w, u32)
                return w
            return _unpack(w_p[lo // 2:hi // 2, :])

        def anchor_x1(v):
            x1_s[pl.ds(pl.multiple_of(T + 8 * dyn0, 8), 8), 0:128] = v

        def ln1_chunk(c, blk):
            x = x_v[pl.ds(pl.multiple_of(blk * T + CH * c, CH), CH), :].astype(f32)
            h = _ln(x) * modv(1, CH) + modv(0, CH)
            hb_s[CH // 2 * c:CH // 2 * (c + 1), :] = _pack(h)
            return token(h)

        def kstore(kb, blk):
            lane = lax.broadcasted_iota(jnp.int32, (QB, 128), 1)
            tiles = []
            for g in range(NG):
                t0, t1 = (80 * g) // 128, (80 * g + 79) // 128
                if t0 == t1:
                    tiles.append(kb[:, 128 * t0:128 * t0 + 128])
                else:
                    tiles.append(jnp.where(lane >= 64, kb[:, 128 * t0:128 * t0 + 128],
                                           kb[:, 128 * t1:128 * t1 + 128]))
            k_s[blk] = _pack(jnp.concatenate(tiles, axis=1))

        def vstore(src, blk):
            fl = jnp.ones((8, QB), f32)
            out = []
            for hh in range(H):
                a = (DH * hh) // 16
                off = DH * hh - 16 * a
                v = [src[16 * a + 8 * i:16 * a + 8 * i + 8] for i in range(4)]
                if off == 0:
                    out += [v[0], v[1], jnp.where(lo4, v[2], fl), fl]
                elif off == 4:
                    out += [jnp.where(lo4, fl, v[0]), v[1], v[2], fl]
                elif off == 8:
                    out += [fl, v[1], v[2], jnp.where(lo4, v[3], fl)]
                else:
                    out += [fl, jnp.where(lo4, fl, v[1]), v[2], v[3]]
            vT_s[blk] = _pack(jnp.concatenate(out, axis=0))

        dd = (lax.broadcasted_iota(jnp.int32, (16, 128), 1)
              - lax.broadcasted_iota(jnp.int32, (16, 128), 0))
        old = jnp.concatenate([dd < 16 * i for i in range(8)], axis=0)
        z8 = jnp.zeros((8, 128), u32)
        lane16 = lax.broadcasted_iota(jnp.int32, (16, 128), 1)
        g_lo = (lane16 & 32) != 0
        g_hi = lane16 >= 64
        r40 = lax.broadcasted_iota(jnp.int32, (40, 128), 0)
        hrow = (r40 >= 10).astype(jnp.int32) + (r40 >= 20).astype(jnp.int32) + (r40 >= 30).astype(jnp.int32)
        hx = hrow ^ (lax.broadcasted_iota(jnp.int32, (40, 128), 1) >> 5)

        def nkeys(b):
            return min(b + 1, 3) if first else 3

        def place(g, vs, tok=None):
            parts = [z8] * 8
            if tok is not None:
                parts[(5 * g + 6) % 8] = pltpu.bitcast(tok, u32)
            for i, v in vs.items():
                parts[(5 * g + i) % 8] = v
            return jnp.concatenate(parts, axis=0)

        def stage1(u, slot, toks=()):
            b, g = divmod(u, NG)
            nk = nkeys(b)
            gb_ = g0 + b
            q5 = qT_s[q0 + b, 40 * g:40 * g + 40, :]
            ws = []
            for j in range(4):
                qm = jnp.where(hrow[8 * j:8 * j + 16] == j, q5[8 * j:8 * j + 16], jnp.uint32(0))
                ws.append(place(g, {j: qm[0:8], j + 1: qm[8:16]}))
            w = _unpack(jnp.concatenate(ws, axis=1))
            ln = slice(128 * g, 128 * g + 128)
            mx = [None]

            def emit(r0, sm):
                s_s[slot, r0:r0 + 16, :] = sm
                mx[0] = sm if mx[0] is None else jnp.maximum(mx[0], sm)

            if nk < 3:
                rows = [k_s[gb_, :, ln]]
                if nk == 2:
                    rows.append(k_s[gb_ - 1, :, ln])
                s = jnp.dot(_unpack(jnp.concatenate(rows, axis=0)), w, preferred_element_type=f32)
                for i in range(8):
                    old4 = jnp.concatenate([dd < 16 * i] * 4, axis=1)
                    emit(16 * i, jnp.where(old4, -1e30, s[16 * i:16 * i + 16]))
                for i in range(8, 8 * nk):
                    emit(16 * i, s[16 * i:16 * i + 16])
            else:
                def kb(B):
                    return k_s[gb_ - 2 + B // 4, 16 * (B % 4):16 * (B % 4) + 16, ln]
                fl = (lane16 - (80 * g) % 128) & 127
                h_hi = fl >= 40
                h_lo = ((fl >= 20) & (fl < 40)) | (fl >= 60)
                x = [kb(0), kb(1), kb(2), kb(11)]
                t = [jnp.where(h_lo, x[v ^ 1], x[v]) for v in range(4)]
                e_l = [jnp.where(h_hi, t[v ^ 2], t[v]) for v in range(4)]
                k9, k10 = kb(9), kb(10)
                j2_l = [jnp.where(h_hi, k10, x[2]), jnp.where(h_hi, x[2], k10)]
                sm = []
                for v in range(4):
                    j1_l = jnp.where((fl >= 20 * v) & (fl < 20 * v + 20), x[1], k9)
                    lhs = jnp.concatenate([e_l[v][0:8], j1_l[0:8], j2_l[v // 2][0:8],
                                           e_l[v][8:16], j1_l[8:16], j2_l[v // 2][8:16]], axis=0)
                    qm = jnp.where(hx == v, q5, jnp.uint32(0))
                    wv = place(g, {i: qm[8 * i:8 * i + 8] for i in range(5)}, toks[v] if v < len(toks) else None)
                    sm.append(jnp.dot(_unpack(lhs), _unpack(wv), preferred_element_type=f32))
                for c in range(2):
                    for J in (1, 2):
                        msk = (dd < 32 * J + 16 * c) & (lane16 >= 32 * J)
                        uu = [jnp.where(msk, sm[v][48 * c:48 * c + 16], sm[v][48 * c + 16 * J:48 * c + 16 * J + 16])
                              for v in range(4)]
                        t = [jnp.where(g_lo, uu[v ^ 1], uu[v]) for v in range(4)]
                        emit(32 * J + 16 * c,
                             jnp.concatenate([jnp.where(g_hi, t[v ^ 2], t[v]) for v in range(4)], axis=1))
                k8, k3 = kb(8), kb(3)
                lhs = jnp.concatenate([k8[0:8], k3[0:8], k8[8:16], k3[8:16], k_s[gb_ - 1, :, ln]], axis=0)
                s = jnp.dot(_unpack(lhs), w, preferred_element_type=f32)
                for c in range(2):
                    e0 = jnp.concatenate([sm[v][48 * c:48 * c + 16] for v in range(4)], axis=1)
                    e3 = jnp.concatenate([sm[v ^ 3][48 * c:48 * c + 16] for v in range(4)], axis=1)
                    old4 = jnp.concatenate([dd < 16 * c] * 4, axis=1)
                    emit(16 * c, jnp.where(old4, e0, s[32 * c:32 * c + 16]))
                    old4 = jnp.concatenate([dd < 96 + 16 * c] * 4, axis=1)
                    emit(96 + 16 * c, jnp.where(old4, s[32 * c + 16:32 * c + 32], e3))
                for i in range(8):
                    emit(128 + 16 * i, s[64 + 16 * i:64 + 16 * i + 16])
            st["m", u] = (jnp.max(mx[0], axis=0, keepdims=True), slot)
            return mx[0][0:8, 0:128]

        def stage2(u):
            b, g = divmod(u, NG)
            m, slot = st.pop(("m", u))
            nk = nkeys(b)
            gb_ = g0 + b
            res = []
            for j in range(4):
                hh = 4 * g + j
                off = DH * hh - 16 * ((DH * hh) // 16)
                ln = slice(128 * j, 128 * j + 128)
                e = jnp.exp2(s_s[slot, 0:128 * min(nk, 2), ln] - m[:, ln])
                if nk == 3:
                    eo = jnp.where(old, e[0:128], 0.0)
                    e = jnp.concatenate([eo, e[0:128] - eo, e[128:256]], axis=0)
                blks = [[gb_], [gb_, gb_ - 1], [gb_ - 2, gb_, gb_ - 1]][nk - 1]
                vw = _unpack(jnp.concatenate([vT_s[bb, 16 * hh:16 * hh + 16, :] for bb in blks], axis=1))
                o = jnp.dot(vw, e.astype(bf16), preferred_element_type=f32)
                if off < 8:
                    l, o3 = o[24:32], o[0:24]
                else:
                    l, o3 = o[0:8], o[8:32]
                r = pl.reciprocal(l, approx=True)
                r = r * (2.0 - l * r)
                res.append([o3[8 * i:8 * i + 8] * r for i in range(3)])
            out = []
            for j in (0, 2):
                a_, b_ = res[j], res[j + 1]
                out += [a_[0], a_[1], jnp.where(lo4, a_[2], b_[0]), b_[1], b_[2]]
            ot = 2 if (first and b == 0) else b
            oT_s[ot, 80 * g:80 * g + 80, :] = jnp.concatenate(out, axis=0)
            if u == NG - 1 and not first:
                oa_s[...] = _pack(oT_s[0].T)

        def wo_stage(r0, n):
            if second:
                oa_s[...] = _pack(oT_s[2].T)
            if r0 + n > QB:
                ob_s[...] = _pack(oT_s[1].T)
            ob = jnp.concatenate([r[...] for r in (oa_s, ob_s)[r0 // QB:(r0 + n) // QB]], axis=0)
            y = jnp.dot(_unpack(ob), weight(wo_v, wo_p, second), preferred_element_type=f32)
            x = x_v[pl.ds(pl.multiple_of((step - 1) * T + r0, QB), n), :].astype(f32)
            x1_s[r0:r0 + n, :] = x + modv(2, n) * y

        def ln23_chunk(c):
            y = _ln(_ln(x1_s[CH * c:CH * (c + 1), :]) * modv(4, CH) + modv(3, CH))
            y_s[CH // 2 * c:CH // 2 * (c + 1), :] = _pack(y)
            return token(y)

        def bias(b, n, toks):
            nt = b.shape[1] // 128
            b8 = jnp.broadcast_to(b, (8, b.shape[1]))
            tiles = [b8[:, 128 * j:128 * j + 128] for j in range(nt)]
            if isinstance(toks, dict):
                toks = list(toks.items())
            else:
                toks = [(i * nt // len(toks), t) for i, t in enumerate(toks)]
            for j, t in toks:
                tiles[j] = tiles[j] + t
            return _rep(jnp.concatenate(tiles, axis=1), n)

        def w1_stage(r0, n, toks=()):
            b1 = b1_v[...].astype(f32).reshape(1, F)
            raw = lax.dot_general(_unpack(y_s[r0 // 2:(r0 + n) // 2, :]), weight(w1t_v, w1_p, second, 0, FM),
                                  NT, preferred_element_type=f32)
            if callable(toks):
                toks = toks(raw)
            hh_s[r0 // 2:(r0 + n) // 2, :] = _pack(_gelu(raw + bias(b1[:, 0:FM], n, toks)))

        def w1_rem():
            b1 = b1_v[...].astype(f32).reshape(1, F)[:, FM:F]
            rt = lax.dot_general(weight(w1t_v, w1_p, second, FM, F), _unpack(y_s[...]), NT,
                                 preferred_element_type=f32)
            r = jnp.concatenate([rt[:, 0:QB], rt[:, QB:T]], axis=0).T
            hr_s[...] = _pack(_gelu(r + jnp.concatenate([b1, b1], axis=1)))

        def w2_stage(b, toks=(), strips=((0, D),)):
            r0 = QB * b
            b2 = bias(b2_v[...].astype(f32).reshape(1, D), QB, toks)
            if second and b == 0:
                wr = pltpu.bitcast(w2_v[FM:F, :], u32)
                zz = jnp.zeros_like(wr)
                w2_p[FM // 2:FM // 2 + 128, :] = jnp.concatenate([wr, zz, zz, wr], axis=0)
            wm = weight(w2_v, w2_p, second and b == 0, 0, FM)
            wr = _unpack(w2_p[FM // 2 + 64 * b:FM // 2 + 64 * b + 64, :])
            lhs = jnp.concatenate([hh_s[r0 // 2:(r0 + QB) // 2, :], hr_s[...]], axis=1)
            mo = jnp.dot(_unpack(lhs), jnp.concatenate([wm, wr], axis=0), preferred_element_type=f32) + b2
            rows = pl.ds(pl.multiple_of((step - 1) * T + r0, QB), QB)
            res = (x1_s[r0:r0 + QB, :] + modv(5, QB) * mo).astype(bf16)
            for c0, c1 in strips:
                o_v[rows, c0:c1] = res[:, c0:c1]
                pltpu.make_async_copy(o_v.at[rows, c0:c1], o_h.at[0, rows, c0:c1], osem.at[0]).start()

        def wt_cols(dst, c0, t):
            w = wqkv_v[128 * t:128 * t + 128, c0:c0 + D].astype(f32).T
            dst[:, 128 * t:128 * t + 128] = _pack(w)
            return token(w[D - 16:D])

        def seg(k, c0, c1, r0, r1):
            lo, hi = 128 * k, 128 * k + 128
            h = n_s[r0:r1, lo:hi] * _rep(mod_s[:, D + lo:D + hi], r1 - r0) + _rep(mod_s[:, lo:hi], r1 - r0)
            w = wqkv_v[lo:hi, c0:c1]
            if r0 == 0 and c0 <= D and c1 >= 2 * D:
                wk_p[lo // 2:hi // 2, :] = pltpu.bitcast(w[:, D - c0:2 * D - c0], u32)
            r = jnp.dot(h.astype(bf16), w, preferred_element_type=f32)
            return r if k == 0 else r + acc_s[r0:r1, c0:c1]

        def fin(which, b0, b1):
            r = seg(4, which * D, (which + 1) * D, QB * b0, QB * b1)
            for b in range(b0, b1):
                rb = r[QB * (b - b0):QB * (b - b0 + 1)]
                if which == 0:
                    qT_s[b] = _pack((rb * QSCALE).T)
                elif which == 1:
                    kstore(rb, b)
                else:
                    vstore(rb.T, b)

        if first:
            st["job"] = 0

            def jobs(n):
                j0, j1 = st["job"], st["job"] + n
                st["job"] = j1
                while j0 < j1:
                    kb_, t0 = divmod(j0, 15)
                    t1 = min(15, t0 + j1 - j0)
                    k, b = divmod(kb_, 4)
                    acc_s[QB * b:QB * b + QB, 128 * t0:128 * t1] = seg(k, 128 * t0, 128 * t1, QB * b, QB * b + QB)
                    j0 += t1 - t0

            def norm(c0, c1):
                for c in range(c0, c1):
                    n_s[CH * c:CH * (c + 1), :] = _ln(x_v[CH * c:CH * (c + 1), :].astype(f32))

            for n in names:
                cp(n).start()
            wait("c", "x0")
            norm(0, NCH)
            wait("sa0", "ca0")
            col_s[...] = jnp.broadcast_to(silu_c().astype(f32), (128, D)).T
            mod_mxu([0, 5])
            wait("r0")
            jobs(16)
            wait("x1")
            norm(NCH, 2 * NCH)
            jobs(28)
            wait("sa1", "ca1")
            mod_vpu([1, 6], 16)
            jobs(16)
            wait("r1")
            jobs(44)
            for k in (2, 3):
                wait("sa%d" % k, "ca%d" % k, "r%d" % k)
                mod_vpu([k, k + 5], 16)
                jobs(60 if k == 2 else 48)
            wait("sa4", "ca4", "r4")
            mod_vpu([4, 9], 16)
            jobs(13)
            fin(2, 0, 2)
            fin(0, 0, 2)
            fin(1, 0, 3)
            fin(2, 2, 3)
            fin(0, 2, 3)
            order = [u for g in range(NG) for u in (NG + g, g)]
            stage1(order[0], 0)
            stage1(order[1], 1)
            for i, u in enumerate(order):
                if i + 2 < NU:
                    stage1(order[i + 2], (i + 2) % 3)
                if i == NU - 2:
                    jobs(8)
                stage2(u)
            jobs(7)
            wait("wm2", "wo")
        elif variant in ("second", "mid"):
            if second:
                mod_vpu([15, 20, 10, 16, 21, 17, 11, 22, 18, 23, 12, 19, 24, 14, 13], 16)
            else:
                kf = jnp.dot(_unpack(hb_s[...]), _unpack(wk_p[...]), preferred_element_type=f32)
                for b in range(2):
                    kstore(kf[QB * b:QB * b + QB], g0 + b)
                wo_stage(0, T)
                qf = lax.dot_general(_unpack(wqT_s[...]), _unpack(hb_s[...]), NT, preferred_element_type=f32)
                for b in range(2):
                    qT_s[b] = _pack(qf[:, QB * b:QB * b + QB] * QSCALE)
                vf = lax.dot_general(_unpack(wvT_s[...]), _unpack(hb_s[...]), NT, preferred_element_type=f32)
                for b in range(2):
                    vstore(vf[:, QB * b:QB * b + QB], g0 + b)
                an = [z[r:r + 8, 128 * b:128 * b + 128] for z in (qf, vf) for b in range(2)
                      for r in range(0, 576, 96)]
                for c in range(NCH):
                    anchor_x1(an[c])
                    ln23_chunk(c)
            if second:
                for which in (1, 2, 0):
                    fin(which, 3, 4)
            a1 = stage1(0, 0)
            if second:
                wo_stage(0, T)
            pend = {}
            done23 = 0 if second else NCH
            for u in range(NU):
                if u == NU - 2:
                    if second:
                        wait("x2", "b1", "b2", "w1")
                    nxt = jnp.minimum(step + 1, NS - 1)
                    t1 = [ln1_chunk(c, nxt) for c in range(NCH)]
                    w1_stage(0, T, t1 if second else t1[0:12])
                    w1_rem()
                if done23 < NCH and u >= 3:
                    anchor_x1(a1)
                    hi23 = min(NCH, -(-NCH * (u - 2) // 10))
                    pend[u + 3] = [ln23_chunk(c) for c in range(done23, hi23)]
                    done23 = hi23
                if u + 1 < NU:
                    a1 = stage1(u + 1, (u + 1) % 2, pend.pop(u + 1, ()))
                elif second:
                    wait("wm3", "w2")
                    mod_vpu(range(25, 30), 8)
                    w2_stage(0, [wt_cols(wqT_s, 0, t) for t in range(5)])
                else:
                    w2_stage(0, t1[12:])
                stage2(u)
            w2_stage(1, [wt_cols(wvT_s, 2 * D, t) for t in range(5)] if second else ())
            if second:
                wait("xr")
        else:
            wo_stage(0, QB)
            for c in range(NCH // 2):
                ln23_chunk(c)
            wo_stage(QB, QB)

            def ln23_b(raw):
                toks = {}
                for i in range(NCH // 2):
                    anchor_x1(raw[0:8, 128 * i:128 * i + 128])
                    toks[i + 5] = ln23_chunk(NCH // 2 + i)
                return toks

            w1_stage(0, QB, ln23_b)
            w1_stage(QB, QB)
            w1_rem()
            w2_stage(0)
            w2_stage(1, (), ((0, 512), (512, D)))
            pltpu.make_async_copy(o_v, o_h.at[0], osem.at[0]).wait()

    @pl.when(step == 0)
    def _():
        body("first")

    @pl.when(step == 1)
    def _():
        body("second")

    @pl.when((step > 1) & (step < NS))
    def _():
        body("mid")

    @pl.when(step == NS)
    def _():
        body("last")


@jax.jit
def pallas_adaLN_cond__sliding_block__mixer_channel_mlp__prompt_kernel(
    A_x: jax.Array,
    A_wqkv: jax.Array,
    A_wo: jax.Array,
    B_x: jax.Array,
    B_w1: jax.Array,
    B_b1: jax.Array,
    B_w2: jax.Array,
    B_b2: jax.Array,
    c: jax.Array,
    w_mod: jax.Array,
):
    del B_x
    anyspec = pl.BlockSpec(memory_space=pl.ANY)
    V = pltpu.VMEM
    return pl.pallas_call(
        _kernel,
        grid=(NS + 1,),
        in_specs=[anyspec] * 9,
        out_specs=anyspec,
        out_shape=jax.ShapeDtypeStruct((1, S, D), bf16),
        scratch_shapes=[
            V((S, D), bf16), V((1, D), bf16), V((F,), bf16), V((D,), bf16),
            V((D, 3 * D), bf16), V((D, D), bf16), V((F, D), bf16), V((F, D), bf16),
            V((D, 6 * D), bf16), V((S, D), bf16),
            pltpu.SemaphoreType.DMA((27,)), pltpu.SemaphoreType.DMA((1,)),
            V((8, 6 * D), f32), V((D, 128), f32),
            V((D // 2, D), u32), V((D // 2, D), u32), V((D // 2, D), u32), V((D // 2, D), u32),
            V((F // 2, D), u32), V((FM // 2 + 128, D), u32),
            V((NB, QB // 2, 128 * NG), u32), V((NB, 16 * H, QB), u32), V((4, D // 2, QB), u32),
            V((3, 256, 512), f32), V((3, D, QB), f32), V((QB // 2, D), u32), V((QB // 2, D), u32),
            V((T // 2, D), u32), V((T + 8, D), f32), V((T // 2, D), u32),
            V((T // 2, FM), u32), V((QB // 2, 128), u32),
            V((2 * T, D), f32), V((2 * T, 3 * D), f32),
        ],
        compiler_params=pltpu.CompilerParams(
            dimension_semantics=("arbitrary",),
            vmem_limit_bytes=100 * 1024 * 1024,
            disable_bounds_checks=True,
            disable_semaphore_checks=True,
        ),
    )(A_x, c, B_b1, B_b2, A_wqkv, A_wo, B_w1.T, B_w2, w_mod)
```

```python
import jax
import jax.numpy as jnp
from jax import lax
import jax.experimental.pallas as pl
import jax.experimental.pallas.tpu as pltpu

S, D, H, DH, F = 2048, 640, 32, 20, 1728
T = 256
QB = 128
NB = S // QB
NS = S // T
NG = 8
NU = 2 * NG
CH = 16
NCH = T // CH
FM = 1664
EPS = 1e-5
QSCALE = DH ** -0.5 * 1.4426950408889634
f32, bf16, u32 = jnp.float32, jnp.bfloat16, jnp.uint32
NT = (((1,), (1,)), ((), ()))


def _ln(x):
    xc = x - jnp.sum(x, axis=-1, keepdims=True) * (1.0 / D)
    v = jnp.sum(xc * xc, axis=-1, keepdims=True) * (1.0 / D)
    return xc * lax.rsqrt(v + EPS)


def _pack(x):
    return pltpu.bitcast(x.astype(bf16), u32)


def _unpack(x):
    return pltpu.bitcast(x, bf16)


def _rep(v, n):
    return jnp.concatenate([v] * (n // 8), axis=0)


def _gelu(x):
    c = 0.7978845608028654
    return 0.5 * x * (1.0 + jnp.tanh(x * (c + (c * 0.044715) * (x * x))))


def _kernel(x_h, c_h, b1_h, b2_h, wqkv_h, wo_h, w1t_h, w2_h, wmod_h, o_h,
            x_v, c_v, b1_v, b2_v, wqkv_v, wo_v, w1t_v, w2_v, wmod_v, o_v, sems, osem,
            mod_s, col_s, wqT_s, wvT_s, wk_p, wo_p, w1_p, w2_p,
            k_s, vT_s, qT_s, s_s, oT_s, oa_s, ob_s, hb_s, x1_s, y_s, hh_s, hr_s,
            n_s, acc_s):
    step = pl.program_id(0)
    dyn0 = step >> 10

    def xrows(lo, hi):
        return x_h.at[0, lo:hi], x_v.at[lo:hi]

    def wmcols(lo, hi):
        return wmod_h.at[:, lo:hi], wmod_v.at[:, lo:hi]

    def wrows(lo, hi):
        return wqkv_h.at[lo:hi], wqkv_v.at[lo:hi]

    pairs = dict(c=(c_h, c_v), x0=xrows(0, T))
    for k in range(5):
        pairs["sa%d" % k] = wmcols(128 * k, 128 * k + 128)
        pairs["ca%d" % k] = wmcols(D + 128 * k, D + 128 * k + 128)
        pairs["r%d" % k] = wrows(128 * k, 128 * k + 128)
        if k == 0:
            pairs["x1"] = xrows(T, 2 * T)
    pairs.update(
        wm2=wmcols(2 * D, 5 * D), wo=(wo_h, wo_v), x2=xrows(2 * T, 3 * T),
        b1=(b1_h, b1_v), b2=(b2_h, b2_v), w1=(w1t_h, w1t_v),
        wm3=wmcols(5 * D, 6 * D), w2=(w2_h, w2_v), xr=xrows(3 * T, S),
    )
    names = list(pairs)

    def cp(n):
        s, d = pairs[n]
        return pltpu.make_async_copy(s, d, sems.at[names.index(n)])

    def wait(*ns):
        for n in ns:
            cp(n).wait()

    def silu_c():
        c = c_v[...].astype(f32)
        return (c * jax.nn.sigmoid(c)).astype(bf16)

    def modv(i, n):
        return _rep(mod_s[:, i * D:(i + 1) * D], n)

    def mod_put(t, v):
        mod_s[:, 128 * t:128 * t + 128] = v + 1.0 if t // 5 in (1, 4) else v

    def mod_mxu(tiles):
        w = jnp.concatenate([wmod_v[:, 128 * t:128 * t + 128] for t in tiles], axis=1)
        r = jnp.dot(jnp.broadcast_to(silu_c(), (16, D)), w, preferred_element_type=f32)[0:8]
        for i, t in enumerate(tiles):
            mod_put(t, r[:, 128 * i:128 * i + 128])

    def mod_vpu(tiles, mw):
        acc = jnp.zeros((mw, 128), f32)
        for t in tiles:
            acc = jnp.where(dyn0 == 1, acc, 0.0)
            for r in range(D // mw):
                rows = slice(mw * r, mw * r + mw)
                acc = acc + wmod_v[rows, 128 * t:128 * t + 128].astype(f32) * col_s[rows, :]
            mod_put(t, jnp.broadcast_to(jnp.sum(acc, axis=0, keepdims=True), (8, 128)))

    def token(v):
        return jnp.where(dyn0 == 1, v[0:8, 0:128], jnp.where(dyn0 == 2, v[8:16, 0:128], 0.0))

    def body(variant):
        first = variant == "first"
        second = variant == "second"
        g0 = step * (T // QB)
        q0 = 2 if second else 0
        lo4 = lax.broadcasted_iota(jnp.int32, (8, QB), 0) < 4
        st = {}

        def weight(w_v, w_p, fresh, lo=0, hi=None):
            hi = w_v.shape[0] if hi is None else hi
            if fresh:
                w = w_v[lo:hi, :]
                w_p[lo // 2:hi // 2, :] = pltpu.bitcast(w, u32)
                return w
            return _unpack(w_p[lo // 2:hi // 2, :])

        def anchor_x1(v):
            x1_s[pl.ds(pl.multiple_of(T + 8 * dyn0, 8), 8), 0:128] = v

        def ln1_chunk(c, blk):
            x = x_v[pl.ds(pl.multiple_of(blk * T + CH * c, CH), CH), :].astype(f32)
            h = _ln(x) * modv(1, CH) + modv(0, CH)
            hb_s[CH // 2 * c:CH // 2 * (c + 1), :] = _pack(h)
            return token(h)

        def kstore(kb, blk):
            lane = lax.broadcasted_iota(jnp.int32, (QB, 128), 1)
            tiles = []
            for g in range(NG):
                t0, t1 = (80 * g) // 128, (80 * g + 79) // 128
                if t0 == t1:
                    tiles.append(kb[:, 128 * t0:128 * t0 + 128])
                else:
                    tiles.append(jnp.where(lane >= 64, kb[:, 128 * t0:128 * t0 + 128],
                                           kb[:, 128 * t1:128 * t1 + 128]))
            k_s[blk] = _pack(jnp.concatenate(tiles, axis=1))

        def vstore(src, blk):
            fl = jnp.ones((8, QB), f32)
            out = []
            for hh in range(H):
                a = (DH * hh) // 16
                off = DH * hh - 16 * a
                v = [src[16 * a + 8 * i:16 * a + 8 * i + 8] for i in range(4)]
                if off == 0:
                    out += [v[0], v[1], jnp.where(lo4, v[2], fl), fl]
                elif off == 4:
                    out += [jnp.where(lo4, fl, v[0]), v[1], v[2], fl]
                elif off == 8:
                    out += [fl, v[1], v[2], jnp.where(lo4, v[3], fl)]
                else:
                    out += [fl, jnp.where(lo4, fl, v[1]), v[2], v[3]]
            vT_s[blk] = _pack(jnp.concatenate(out, axis=0))

        dd = (lax.broadcasted_iota(jnp.int32, (16, 128), 1)
              - lax.broadcasted_iota(jnp.int32, (16, 128), 0))
        old = jnp.concatenate([dd < 16 * i for i in range(8)], axis=0)
        z8 = jnp.zeros((8, 128), u32)
        lane16 = lax.broadcasted_iota(jnp.int32, (16, 128), 1)
        g_lo = (lane16 & 32) != 0
        g_hi = lane16 >= 64
        r40 = lax.broadcasted_iota(jnp.int32, (40, 128), 0)
        hrow = (r40 >= 10).astype(jnp.int32) + (r40 >= 20).astype(jnp.int32) + (r40 >= 30).astype(jnp.int32)
        hx = hrow ^ (lax.broadcasted_iota(jnp.int32, (40, 128), 1) >> 5)

        def nkeys(b):
            return min(b + 1, 3) if first else 3

        def place(g, vs, tok=None):
            parts = [z8] * 8
            if tok is not None:
                parts[(5 * g + 6) % 8] = pltpu.bitcast(tok, u32)
            for i, v in vs.items():
                parts[(5 * g + i) % 8] = v
            return jnp.concatenate(parts, axis=0)

        def stage1(u, slot, toks=()):
            b, g = divmod(u, NG)
            nk = nkeys(b)
            gb_ = g0 + b
            q5 = qT_s[q0 + b, 40 * g:40 * g + 40, :]
            ws = []
            for j in range(4):
                qm = jnp.where(hrow[8 * j:8 * j + 16] == j, q5[8 * j:8 * j + 16], jnp.uint32(0))
                ws.append(place(g, {j: qm[0:8], j + 1: qm[8:16]}))
            w = _unpack(jnp.concatenate(ws, axis=1))
            ln = slice(128 * g, 128 * g + 128)
            mx = [None]

            def emit(r0, sm):
                s_s[slot, r0:r0 + 16, :] = sm
                mx[0] = sm if mx[0] is None else jnp.maximum(mx[0], sm)

            if nk < 3:
                rows = [k_s[gb_, :, ln]]
                if nk == 2:
                    rows.append(k_s[gb_ - 1, :, ln])
                s = jnp.dot(_unpack(jnp.concatenate(rows, axis=0)), w, preferred_element_type=f32)
                for i in range(8):
                    old4 = jnp.concatenate([dd < 16 * i] * 4, axis=1)
                    emit(16 * i, jnp.where(old4, -1e30, s[16 * i:16 * i + 16]))
                for i in range(8, 8 * nk):
                    emit(16 * i, s[16 * i:16 * i + 16])
            else:
                def kb(B):
                    return k_s[gb_ - 2 + B // 4, 16 * (B % 4):16 * (B % 4) + 16, ln]
                fl = (lane16 - (80 * g) % 128) & 127
                h_hi = fl >= 40
                h_lo = ((fl >= 20) & (fl < 40)) | (fl >= 60)
                x = [kb(0), kb(1), kb(2), kb(11)]
                t = [jnp.where(h_lo, x[v ^ 1], x[v]) for v in range(4)]
                e_l = [jnp.where(h_hi, t[v ^ 2], t[v]) for v in range(4)]
                k9, k10 = kb(9), kb(10)
                j2_l = [jnp.where(h_hi, k10, x[2]), jnp.where(h_hi, x[2], k10)]
                sm = []
                for v in range(4):
                    j1_l = jnp.where((fl >= 20 * v) & (fl < 20 * v + 20), x[1], k9)
                    lhs = jnp.concatenate([e_l[v][0:8], j1_l[0:8], j2_l[v // 2][0:8],
                                           e_l[v][8:16], j1_l[8:16], j2_l[v // 2][8:16]], axis=0)
                    qm = jnp.where(hx == v, q5, jnp.uint32(0))
                    wv = place(g, {i: qm[8 * i:8 * i + 8] for i in range(5)}, toks[v] if v < len(toks) else None)
                    sm.append(jnp.dot(_unpack(lhs), _unpack(wv), preferred_element_type=f32))
                for c in range(2):
                    for J in (1, 2):
                        msk = (dd < 32 * J + 16 * c) & (lane16 >= 32 * J)
                        uu = [jnp.where(msk, sm[v][48 * c:48 * c + 16], sm[v][48 * c + 16 * J:48 * c + 16 * J + 16])
                              for v in range(4)]
                        t = [jnp.where(g_lo, uu[v ^ 1], uu[v]) for v in range(4)]
                        emit(32 * J + 16 * c,
                             jnp.concatenate([jnp.where(g_hi, t[v ^ 2], t[v]) for v in range(4)], axis=1))
                k8, k3 = kb(8), kb(3)
                lhs = jnp.concatenate([k8[0:8], k3[0:8], k8[8:16], k3[8:16], k_s[gb_ - 1, :, ln]], axis=0)
                s = jnp.dot(_unpack(lhs), w, preferred_element_type=f32)
                for c in range(2):
                    e0 = jnp.concatenate([sm[v][48 * c:48 * c + 16] for v in range(4)], axis=1)
                    e3 = jnp.concatenate([sm[v ^ 3][48 * c:48 * c + 16] for v in range(4)], axis=1)
                    old4 = jnp.concatenate([dd < 16 * c] * 4, axis=1)
                    emit(16 * c, jnp.where(old4, e0, s[32 * c:32 * c + 16]))
                    old4 = jnp.concatenate([dd < 96 + 16 * c] * 4, axis=1)
                    emit(96 + 16 * c, jnp.where(old4, s[32 * c + 16:32 * c + 32], e3))
                for i in range(8):
                    emit(128 + 16 * i, s[64 + 16 * i:64 + 16 * i + 16])
            st["m", u] = (jnp.max(mx[0], axis=0, keepdims=True), slot)
            return mx[0][0:8, 0:128]

        def stage2(u):
            b, g = divmod(u, NG)
            m, slot = st.pop(("m", u))
            nk = nkeys(b)
            gb_ = g0 + b
            res = []
            for j in range(4):
                hh = 4 * g + j
                off = DH * hh - 16 * ((DH * hh) // 16)
                ln = slice(128 * j, 128 * j + 128)
                e = jnp.exp2(s_s[slot, 0:128 * min(nk, 2), ln] - m[:, ln])
                if nk == 3:
                    eo = jnp.where(old, e[0:128], 0.0)
                    e = jnp.concatenate([eo, e[0:128] - eo, e[128:256]], axis=0)
                blks = [[gb_], [gb_, gb_ - 1], [gb_ - 2, gb_, gb_ - 1]][nk - 1]
                vw = _unpack(jnp.concatenate([vT_s[bb, 16 * hh:16 * hh + 16, :] for bb in blks], axis=1))
                o = jnp.dot(vw, e.astype(bf16), preferred_element_type=f32)
                if off < 8:
                    l, o3 = o[24:32], o[0:24]
                else:
                    l, o3 = o[0:8], o[8:32]
                r = pl.reciprocal(l, approx=True)
                r = r * (2.0 - l * r)
                res.append([o3[8 * i:8 * i + 8] * r for i in range(3)])
            out = []
            for j in (0, 2):
                a_, b_ = res[j], res[j + 1]
                out += [a_[0], a_[1], jnp.where(lo4, a_[2], b_[0]), b_[1], b_[2]]
            ot = 2 if (first and b == 0) else b
            oT_s[ot, 80 * g:80 * g + 80, :] = jnp.concatenate(out, axis=0)
            if u == NG - 1 and not first:
                oa_s[...] = _pack(oT_s[0].T)

        def wo_stage(r0, n):
            if second:
                oa_s[...] = _pack(oT_s[2].T)
            if r0 + n > QB:
                ob_s[...] = _pack(oT_s[1].T)
            ob = jnp.concatenate([r[...] for r in (oa_s, ob_s)[r0 // QB:(r0 + n) // QB]], axis=0)
            y = jnp.dot(_unpack(ob), weight(wo_v, wo_p, second), preferred_element_type=f32)
            x = x_v[pl.ds(pl.multiple_of((step - 1) * T + r0, QB), n), :].astype(f32)
            x1_s[r0:r0 + n, :] = x + modv(2, n) * y

        def ln23_chunk(c):
            y = _ln(_ln(x1_s[CH * c:CH * (c + 1), :]) * modv(4, CH) + modv(3, CH))
            y_s[CH // 2 * c:CH // 2 * (c + 1), :] = _pack(y)
            return token(y)

        def bias(b, n, toks):
            nt = b.shape[1] // 128
            b8 = jnp.broadcast_to(b, (8, b.shape[1]))
            tiles = [b8[:, 128 * j:128 * j + 128] for j in range(nt)]
            if isinstance(toks, dict):
                toks = list(toks.items())
            else:
                toks = [(i * nt // len(toks), t) for i, t in enumerate(toks)]
            for j, t in toks:
                tiles[j] = tiles[j] + t
            return _rep(jnp.concatenate(tiles, axis=1), n)

        def w1_stage(r0, n, toks=()):
            b1 = b1_v[...].astype(f32).reshape(1, F)
            raw = lax.dot_general(_unpack(y_s[r0 // 2:(r0 + n) // 2, :]), weight(w1t_v, w1_p, second, 0, FM),
                                  NT, preferred_element_type=f32)
            if callable(toks):
                toks = toks(raw)
            hh_s[r0 // 2:(r0 + n) // 2, :] = _pack(_gelu(raw + bias(b1[:, 0:FM], n, toks)))

        def w1_rem():
            b1 = b1_v[...].astype(f32).reshape(1, F)[:, FM:F]
            rt = lax.dot_general(weight(w1t_v, w1_p, second, FM, F), _unpack(y_s[...]), NT,
                                 preferred_element_type=f32)
            r = jnp.concatenate([rt[:, 0:QB], rt[:, QB:T]], axis=0).T
            hr_s[...] = _pack(_gelu(r + jnp.concatenate([b1, b1], axis=1)))

        def w2_stage(b, toks=(), strips=((0, D),)):
            r0 = QB * b
            b2 = bias(b2_v[...].astype(f32).reshape(1, D), QB, toks)
            if second and b == 0:
                wr = pltpu.bitcast(w2_v[FM:F, :], u32)
                zz = jnp.zeros_like(wr)
                w2_p[FM // 2:FM // 2 + 128, :] = jnp.concatenate([wr, zz, zz, wr], axis=0)
            wm = weight(w2_v, w2_p, second and b == 0, 0, FM)
            wr = _unpack(w2_p[FM // 2 + 64 * b:FM // 2 + 64 * b + 64, :])
            lhs = jnp.concatenate([hh_s[r0 // 2:(r0 + QB) // 2, :], hr_s[...]], axis=1)
            mo = jnp.dot(_unpack(lhs), jnp.concatenate([wm, wr], axis=0), preferred_element_type=f32) + b2
            rows = pl.ds(pl.multiple_of((step - 1) * T + r0, QB), QB)
            res = (x1_s[r0:r0 + QB, :] + modv(5, QB) * mo).astype(bf16)
            for c0, c1 in strips:
                o_v[rows, c0:c1] = res[:, c0:c1]
                pltpu.make_async_copy(o_v.at[rows, c0:c1], o_h.at[0, rows, c0:c1], osem.at[0]).start()

        def wt_cols(dst, c0, t):
            w = wqkv_v[128 * t:128 * t + 128, c0:c0 + D].astype(f32).T
            dst[:, 128 * t:128 * t + 128] = _pack(w)
            return token(w[D - 16:D])

        def seg(k, c0, c1, r0, r1):
            lo, hi = 128 * k, 128 * k + 128
            h = n_s[r0:r1, lo:hi] * _rep(mod_s[:, D + lo:D + hi], r1 - r0) + _rep(mod_s[:, lo:hi], r1 - r0)
            w = wqkv_v[lo:hi, c0:c1]
            if r0 == 0 and c0 <= D and c1 >= 2 * D:
                wk_p[lo // 2:hi // 2, :] = pltpu.bitcast(w[:, D - c0:2 * D - c0], u32)
            r = jnp.dot(h.astype(bf16), w, preferred_element_type=f32)
            return r if k == 0 else r + acc_s[r0:r1, c0:c1]

        def fin(which, b0, b1):
            r = seg(4, which * D, (which + 1) * D, QB * b0, QB * b1)
            for b in range(b0, b1):
                rb = r[QB * (b - b0):QB * (b - b0 + 1)]
                if which == 0:
                    qT_s[b] = _pack((rb * QSCALE).T)
                elif which == 1:
                    kstore(rb, b)
                else:
                    vstore(rb.T, b)

        if first:
            st["job"] = 0

            def jobs(n):
                j0, j1 = st["job"], st["job"] + n
                st["job"] = j1
                while j0 < j1:
                    kb_, t0 = divmod(j0, 15)
                    t1 = min(15, t0 + j1 - j0)
                    k, b = divmod(kb_, 4)
                    acc_s[QB * b:QB * b + QB, 128 * t0:128 * t1] = seg(k, 128 * t0, 128 * t1, QB * b, QB * b + QB)
                    j0 += t1 - t0

            def norm(c0, c1):
                for c in range(c0, c1):
                    n_s[CH * c:CH * (c + 1), :] = _ln(x_v[CH * c:CH * (c + 1), :].astype(f32))

            for n in names:
                cp(n).start()
            wait("c", "x0")
            norm(0, NCH)
            wait("sa0", "ca0")
            col_s[...] = jnp.broadcast_to(silu_c().astype(f32), (128, D)).T
            mod_mxu([0, 5])
            wait("r0")
            jobs(16)
            wait("x1")
            norm(NCH, 2 * NCH)
            jobs(28)
            wait("sa1", "ca1")
            mod_vpu([1, 6], 16)
            jobs(16)
            wait("r1")
            jobs(44)
            for k in (2, 3):
                wait("sa%d" % k, "ca%d" % k, "r%d" % k)
                mod_vpu([k, k + 5], 16)
                jobs(60 if k == 2 else 48)
            wait("sa4", "ca4", "r4")
            mod_vpu([4, 9], 16)
            jobs(13)
            fin(2, 0, 2)
            fin(0, 0, 2)
            fin(1, 0, 3)
            fin(2, 2, 3)
            fin(0, 2, 3)
            order = [u for g in range(NG) for u in (NG + g, g)]
            stage1(order[0], 0)
            stage1(order[1], 1)
            for i, u in enumerate(order):
                if i + 2 < NU:
                    stage1(order[i + 2], (i + 2) % 3)
                if i == NU - 2:
                    jobs(8)
                stage2(u)
            jobs(7)
            wait("wm2", "wo")
        elif variant in ("second", "mid"):
            if second:
                mod_vpu([15, 20, 10, 16, 21, 17, 11, 22, 18, 23, 12, 19, 24, 14, 13], 16)
            else:
                kf = jnp.dot(_unpack(hb_s[...]), _unpack(wk_p[...]), preferred_element_type=f32)
                for b in range(2):
                    kstore(kf[QB * b:QB * b + QB], g0 + b)
                wo_stage(0, T)
                qf = lax.dot_general(_unpack(wqT_s[...]), _unpack(hb_s[...]), NT, preferred_element_type=f32)
                for b in range(2):
                    qT_s[b] = _pack(qf[:, QB * b:QB * b + QB] * QSCALE)
                vf = lax.dot_general(_unpack(wvT_s[...]), _unpack(hb_s[...]), NT, preferred_element_type=f32)
                for b in range(2):
                    vstore(vf[:, QB * b:QB * b + QB], g0 + b)
                an = [z[r:r + 8, 128 * b:128 * b + 128] for z in (qf, vf) for b in range(2)
                      for r in range(0, 576, 96)]
                for c in range(NCH):
                    anchor_x1(an[c])
                    ln23_chunk(c)
            if second:
                for which in (1, 2, 0):
                    fin(which, 3, 4)
            a1 = stage1(0, 0)
            if second:
                wo_stage(0, T)
            pend = {}
            done23 = 0 if second else NCH
            for u in range(NU):
                if u == NU - 2:
                    if second:
                        wait("x2", "b1", "b2", "w1")
                    nxt = jnp.minimum(step + 1, NS - 1)
                    t1 = [ln1_chunk(c, nxt) for c in range(NCH)]
                    w1_stage(0, T, t1 if second else t1[0:8])
                    w1_rem()
                if done23 < NCH and u >= 2:
                    anchor_x1(a1)
                    hi23 = min(NCH, -(-NCH * (u - 1) // 10))
                    pend[u + 3] = [ln23_chunk(c) for c in range(done23, hi23)]
                    done23 = hi23
                if u + 1 < NU:
                    a1 = stage1(u + 1, (u + 1) % 2, pend.pop(u + 1, ()))
                elif second:
                    wait("wm3", "w2")
                    mod_vpu(range(25, 30), 8)
                    w2_stage(0, [wt_cols(wqT_s, 0, t) for t in range(5)])
                else:
                    w2_stage(0, t1[8:13])
                stage2(u)
            w2_stage(1, [wt_cols(wvT_s, 2 * D, t) for t in range(5)] if second else dict(enumerate(t1[13:])))
            if second:
                wait("xr")
        else:
            wo_stage(0, QB)
            for c in range(NCH // 2):
                ln23_chunk(c)
            wo_stage(QB, QB)

            def ln23_b(raw):
                toks = {}
                for i in range(NCH // 2):
                    anchor_x1(raw[0:8, 128 * i:128 * i + 128])
                    toks[i + 5] = ln23_chunk(NCH // 2 + i)
                return toks

            w1_stage(0, QB, ln23_b)
            w1_stage(QB, QB)
            w1_rem()
            w2_stage(0)
            w2_stage(1, (), ((0, 512), (512, D)))
            pltpu.make_async_copy(o_v, o_h.at[0], osem.at[0]).wait()

    @pl.when(step == 0)
    def _():
        body("first")

    @pl.when(step == 1)
    def _():
        body("second")

    @pl.when((step > 1) & (step < NS))
    def _():
        body("mid")

    @pl.when(step == NS)
    def _():
        body("last")


@jax.jit
def pallas_adaLN_cond__sliding_block__mixer_channel_mlp__prompt_kernel(
    A_x: jax.Array,
    A_wqkv: jax.Array,
    A_wo: jax.Array,
    B_x: jax.Array,
    B_w1: jax.Array,
    B_b1: jax.Array,
    B_w2: jax.Array,
    B_b2: jax.Array,
    c: jax.Array,
    w_mod: jax.Array,
):
    del B_x
    anyspec = pl.BlockSpec(memory_space=pl.ANY)
    V = pltpu.VMEM
    return pl.pallas_call(
        _kernel,
        grid=(NS + 1,),
        in_specs=[anyspec] * 9,
        out_specs=anyspec,
        out_shape=jax.ShapeDtypeStruct((1, S, D), bf16),
        scratch_shapes=[
            V((S, D), bf16), V((1, D), bf16), V((F,), bf16), V((D,), bf16),
            V((D, 3 * D), bf16), V((D, D), bf16), V((F, D), bf16), V((F, D), bf16),
            V((D, 6 * D), bf16), V((S, D), bf16),
            pltpu.SemaphoreType.DMA((27,)), pltpu.SemaphoreType.DMA((1,)),
            V((8, 6 * D), f32), V((D, 128), f32),
            V((D // 2, D), u32), V((D // 2, D), u32), V((D // 2, D), u32), V((D // 2, D), u32),
            V((F // 2, D), u32), V((FM // 2 + 128, D), u32),
            V((NB, QB // 2, 128 * NG), u32), V((NB, 16 * H, QB), u32), V((4, D // 2, QB), u32),
            V((3, 256, 512), f32), V((3, D, QB), f32), V((QB // 2, D), u32), V((QB // 2, D), u32),
            V((T // 2, D), u32), V((T + 8, D), f32), V((T // 2, D), u32),
            V((T // 2, FM), u32), V((QB // 2, 128), u32),
            V((2 * T, D), f32), V((2 * T, 3 * D), f32),
        ],
        compiler_params=pltpu.CompilerParams(
            dimension_semantics=("arbitrary",),
            vmem_limit_bytes=100 * 1024 * 1024,
            disable_bounds_checks=True,
            disable_semaphore_checks=True,
        ),
    )(A_x, c, B_b1, B_b2, A_wqkv, A_wo, B_w1.T, B_w2, w_mod)
```

```python
import jax
import jax.numpy as jnp
from jax import lax
import jax.experimental.pallas as pl
import jax.experimental.pallas.tpu as pltpu

S, D, H, DH, F = 2048, 640, 32, 20, 1728
T = 256
QB = 128
NB = S // QB
NS = S // T
NG = 8
NU = 2 * NG
CH = 16
NCH = T // CH
FM = 1664
EPS = 1e-5
QSCALE = DH ** -0.5 * 1.4426950408889634
f32, bf16, u32 = jnp.float32, jnp.bfloat16, jnp.uint32
NT = (((1,), (1,)), ((), ()))
NN = (((1,), (0,)), ((), ()))


def _ln(x):
    xc = x - jnp.sum(x, axis=-1, keepdims=True) * (1.0 / D)
    v = jnp.sum(xc * xc, axis=-1, keepdims=True) * (1.0 / D)
    return xc * lax.rsqrt(v + EPS)


def _pack(x):
    return pltpu.bitcast(x.astype(bf16), u32)


def _unpack(x):
    return pltpu.bitcast(x, bf16)


def _rep(v, n):
    return jnp.concatenate([v] * (n // 8), axis=0)


def _gelu(x):
    c = 0.7978845608028654
    return 0.5 * x * (1.0 + jnp.tanh(x * (c + (c * 0.044715) * (x * x))))


def _kernel(x_h, c_h, b1_h, b2_h, wqkv_h, wo_h, w1t_h, w2_h, wmod_h, o_h,
            x_v, c_v, b1_v, b2_v, wqkv_v, wo_v, w1t_v, w2_v, wmod_v, o_v, sems, osem,
            mod_s, col_s, wqT_s, wvT_s, wk_p, wo_p, w1_p, w2_p,
            k_s, vT_s, qT_s, s_s, oT_s, oa_s, ob_s, hb_s, x1_s, y_s, hh_s, hr_s,
            n_s, acc_s):
    step = pl.program_id(0)
    dyn0 = step >> 10

    def xrows(lo, hi):
        return x_h.at[0, lo:hi], x_v.at[lo:hi]

    def wmcols(lo, hi):
        return wmod_h.at[:, lo:hi], wmod_v.at[:, lo:hi]

    def wrows(lo, hi):
        return wqkv_h.at[lo:hi], wqkv_v.at[lo:hi]

    pairs = dict(c=(c_h, c_v), x0=xrows(0, T))
    for k in range(5):
        pairs["sa%d" % k] = wmcols(128 * k, 128 * k + 128)
        pairs["ca%d" % k] = wmcols(D + 128 * k, D + 128 * k + 128)
        pairs["r%d" % k] = wrows(128 * k, 128 * k + 128)
        if k == 0:
            pairs["x1"] = xrows(T, 2 * T)
    pairs.update(
        wm2=wmcols(2 * D, 5 * D), wo=(wo_h, wo_v), x2=xrows(2 * T, 3 * T),
        b1=(b1_h, b1_v), b2=(b2_h, b2_v), w1=(w1t_h, w1t_v),
        wm3=wmcols(5 * D, 6 * D), w2=(w2_h, w2_v), xr=xrows(3 * T, S),
    )
    names = list(pairs)

    def cp(n):
        s, d = pairs[n]
        return pltpu.make_async_copy(s, d, sems.at[names.index(n)])

    def wait(*ns):
        for n in ns:
            cp(n).wait()

    def silu_c():
        c = c_v[...].astype(f32)
        return (c * jax.nn.sigmoid(c)).astype(bf16)

    def modv(i, n):
        return _rep(mod_s[:, i * D:(i + 1) * D], n)

    def mod_put(t, v):
        mod_s[:, 128 * t:128 * t + 128] = v + 1.0 if t // 5 in (1, 4) else v

    def mod_mxu(tiles):
        w = jnp.concatenate([wmod_v[:, 128 * t:128 * t + 128] for t in tiles], axis=1)
        r = jnp.dot(jnp.broadcast_to(silu_c(), (16, D)), w, preferred_element_type=f32)[0:8]
        for i, t in enumerate(tiles):
            mod_put(t, r[:, 128 * i:128 * i + 128])

    def mod_vpu(tiles, mw):
        acc = jnp.zeros((mw, 128), f32)
        for t in tiles:
            acc = jnp.where(dyn0 == 1, acc, 0.0)
            for r in range(D // mw):
                rows = slice(mw * r, mw * r + mw)
                acc = acc + wmod_v[rows, 128 * t:128 * t + 128].astype(f32) * col_s[rows, :]
            mod_put(t, jnp.broadcast_to(jnp.sum(acc, axis=0, keepdims=True), (8, 128)))

    def token(v):
        return jnp.where(dyn0 == 1, v[0:8, 0:128], jnp.where(dyn0 == 2, v[8:16, 0:128], 0.0))

    def body(variant):
        first = variant == "first"
        second = variant == "second"
        g0 = step * (T // QB)
        q0 = 2 if second else 0
        lo4 = lax.broadcasted_iota(jnp.int32, (8, QB), 0) < 4
        st = {}

        def weight(w_v, w_p, fresh, lo=0, hi=None):
            hi = w_v.shape[0] if hi is None else hi
            if fresh:
                w = w_v[lo:hi, :]
                w_p[lo // 2:hi // 2, :] = pltpu.bitcast(w, u32)
                return w
            return _unpack(w_p[lo // 2:hi // 2, :])

        def anchor_x1(v):
            x1_s[pl.ds(pl.multiple_of(T + 8 * dyn0, 8), 8), 0:128] = v

        def ln1_chunk(c, blk):
            x = x_v[pl.ds(pl.multiple_of(blk * T + CH * c, CH), CH), :].astype(f32)
            h = _ln(x) * modv(1, CH) + modv(0, CH)
            hb_s[CH // 2 * c:CH // 2 * (c + 1), :] = _pack(h)
            return token(h)

        def kstore(kb, blk):
            lane = lax.broadcasted_iota(jnp.int32, (QB, 128), 1)
            tiles = []
            for g in range(NG):
                t0, t1 = (80 * g) // 128, (80 * g + 79) // 128
                if t0 == t1:
                    tiles.append(kb[:, 128 * t0:128 * t0 + 128])
                else:
                    tiles.append(jnp.where(lane >= 64, kb[:, 128 * t0:128 * t0 + 128],
                                           kb[:, 128 * t1:128 * t1 + 128]))
            k_s[blk] = _pack(jnp.concatenate(tiles, axis=1))

        def vstore(src, blk):
            out = []
            for hh in range(H):
                a = (DH * hh) // 8
                v = [src[8 * (a + i):8 * (a + i) + 8] for i in range(3)]
                if hh % 2 == 0:
                    out += [v[0], v[1], jnp.where(lo4, v[2], 1.0)]
                else:
                    out += [jnp.where(lo4, 1.0, v[0]), v[1], v[2]]
            vT_s[blk] = jnp.concatenate(out, axis=0)

        dd = (lax.broadcasted_iota(jnp.int32, (16, 128), 1)
              - lax.broadcasted_iota(jnp.int32, (16, 128), 0))
        old = jnp.concatenate([dd < 16 * i for i in range(8)], axis=0)
        z8 = jnp.zeros((8, 128), u32)
        lane16 = lax.broadcasted_iota(jnp.int32, (16, 128), 1)
        g_lo = (lane16 & 32) != 0
        g_hi = lane16 >= 64
        r40 = lax.broadcasted_iota(jnp.int32, (40, 128), 0)
        hrow = (r40 >= 10).astype(jnp.int32) + (r40 >= 20).astype(jnp.int32) + (r40 >= 30).astype(jnp.int32)
        hx = hrow ^ (lax.broadcasted_iota(jnp.int32, (40, 128), 1) >> 5)

        def nkeys(b):
            return min(b + 1, 3) if first else 3

        def place(g, vs):
            parts = [z8] * 8
            for i, v in vs.items():
                parts[(5 * g + i) % 8] = v
            return jnp.concatenate(parts, axis=0)

        def stage1(u, slot):
            b, g = divmod(u, NG)
            nk = nkeys(b)
            gb_ = g0 + b
            q5 = qT_s[q0 + b, 40 * g:40 * g + 40, :]
            ws = []
            for j in range(4):
                qm = jnp.where(hrow[8 * j:8 * j + 16] == j, q5[8 * j:8 * j + 16], jnp.uint32(0))
                ws.append(place(g, {j: qm[0:8], j + 1: qm[8:16]}))
            w = _unpack(jnp.concatenate(ws, axis=1))
            ln = slice(128 * g, 128 * g + 128)
            mx = [None]

            def emit(r0, sm):
                s_s[slot, r0:r0 + 16, :] = sm
                mx[0] = sm if mx[0] is None else jnp.maximum(mx[0], sm)

            if nk < 3:
                rows = [k_s[gb_, :, ln]]
                if nk == 2:
                    rows.append(k_s[gb_ - 1, :, ln])
                s = jnp.dot(_unpack(jnp.concatenate(rows, axis=0)), w, preferred_element_type=f32)
                for i in range(8):
                    old4 = jnp.concatenate([dd < 16 * i] * 4, axis=1)
                    emit(16 * i, jnp.where(old4, -1e30, s[16 * i:16 * i + 16]))
                for i in range(8, 8 * nk):
                    emit(16 * i, s[16 * i:16 * i + 16])
            else:
                def kb(B):
                    return k_s[gb_ - 2 + B // 4, 16 * (B % 4):16 * (B % 4) + 16, ln]
                fl = (lane16 - (80 * g) % 128) & 127
                h_hi = fl >= 40
                h_lo = ((fl >= 20) & (fl < 40)) | (fl >= 60)
                x = [kb(0), kb(1), kb(2), kb(11)]
                t = [jnp.where(h_lo, x[v ^ 1], x[v]) for v in range(4)]
                e_l = [jnp.where(h_hi, t[v ^ 2], t[v]) for v in range(4)]
                k9, k10 = kb(9), kb(10)
                j2_l = [jnp.where(h_hi, k10, x[2]), jnp.where(h_hi, x[2], k10)]
                sm = []
                for v in range(4):
                    j1_l = jnp.where((fl >= 20 * v) & (fl < 20 * v + 20), x[1], k9)
                    lhs = jnp.concatenate([e_l[v][0:8], j1_l[0:8], j2_l[v // 2][0:8],
                                           e_l[v][8:16], j1_l[8:16], j2_l[v // 2][8:16]], axis=0)
                    qm = jnp.where(hx == v, q5, jnp.uint32(0))
                    wv = place(g, {i: qm[8 * i:8 * i + 8] for i in range(5)})
                    sm.append(jnp.dot(_unpack(lhs), _unpack(wv), preferred_element_type=f32))
                for c in range(2):
                    for J in (1, 2):
                        msk = (dd < 32 * J + 16 * c) & (lane16 >= 32 * J)
                        uu = [jnp.where(msk, sm[v][48 * c:48 * c + 16], sm[v][48 * c + 16 * J:48 * c + 16 * J + 16])
                              for v in range(4)]
                        t = [jnp.where(g_lo, uu[v ^ 1], uu[v]) for v in range(4)]
                        emit(32 * J + 16 * c,
                             jnp.concatenate([jnp.where(g_hi, t[v ^ 2], t[v]) for v in range(4)], axis=1))
                k8, k3 = kb(8), kb(3)
                lhs = jnp.concatenate([k8[0:8], k3[0:8], k8[8:16], k3[8:16], k_s[gb_ - 1, :, ln]], axis=0)
                s = jnp.dot(_unpack(lhs), w, preferred_element_type=f32)
                for c in range(2):
                    e0 = jnp.concatenate([sm[v][48 * c:48 * c + 16] for v in range(4)], axis=1)
                    e3 = jnp.concatenate([sm[v ^ 3][48 * c:48 * c + 16] for v in range(4)], axis=1)
                    old4 = jnp.concatenate([dd < 16 * c] * 4, axis=1)
                    emit(16 * c, jnp.where(old4, e0, s[32 * c:32 * c + 16]))
                    old4 = jnp.concatenate([dd < 96 + 16 * c] * 4, axis=1)
                    emit(96 + 16 * c, jnp.where(old4, s[32 * c + 16:32 * c + 32], e3))
                for i in range(8):
                    emit(128 + 16 * i, s[64 + 16 * i:64 + 16 * i + 16])
            st["m", u] = (jnp.max(mx[0], axis=0, keepdims=True), slot)
            return mx[0][0:8, 0:128]

        def stage2(u):
            b, g = divmod(u, NG)
            m, slot = st.pop(("m", u))
            nk = nkeys(b)
            gb_ = g0 + b
            res = []
            for j in range(4):
                hh = 4 * g + j
                ln = slice(128 * j, 128 * j + 128)
                e = jnp.exp2(s_s[slot, 0:128 * min(nk, 2), ln] - m[:, ln])
                if nk == 3:
                    e = jnp.concatenate([jnp.where(old, e[0:128], 0.0), jnp.where(old, 0.0, e[0:128]),
                                         e[128:256]], axis=0)
                blks = [[gb_], [gb_, gb_ - 1], [gb_ - 2, gb_, gb_ - 1]][nk - 1]
                vw = jnp.concatenate([vT_s[bb, 24 * hh:24 * hh + 24, :] for bb in blks], axis=1)
                res.append(lax.dot_general(vw, e.astype(bf16), NN, preferred_element_type=f32))
            out = []
            for j in (0, 2):
                a_, b_ = res[j], res[j + 1]
                l = jnp.where(lo4, b_[0:8], a_[16:24])
                r = pl.reciprocal(l, approx=True)
                r = r * (2.0 - l * r)
                rr = pltpu.roll(r, 4, 0)
                ra, rb = jnp.where(lo4, rr, r), jnp.where(lo4, r, rr)
                out += [a_[0:8] * ra, a_[8:16] * ra, jnp.where(lo4, a_[16:24], b_[0:8]) * rr,
                        b_[8:16] * rb, b_[16:24] * rb]
            ot = 2 if (first and b == 0) else b
            oT_s[ot, 80 * g:80 * g + 80, :] = jnp.concatenate(out, axis=0)
            if u == NG - 1 and not first:
                oa_s[...] = _pack(oT_s[0].T)

        def wo_stage(r0, n):
            if second:
                oa_s[...] = _pack(oT_s[2].T)
            if r0 + n > QB:
                ob_s[...] = _pack(oT_s[1].T)
            ob = jnp.concatenate([r[...] for r in (oa_s, ob_s)[r0 // QB:(r0 + n) // QB]], axis=0)
            y = jnp.dot(_unpack(ob), weight(wo_v, wo_p, second), preferred_element_type=f32)
            x = x_v[pl.ds(pl.multiple_of((step - 1) * T + r0, QB), n), :].astype(f32)
            x1_s[r0:r0 + n, :] = x + modv(2, n) * y

        def ln23_chunk(c):
            y = _ln(_ln(x1_s[CH * c:CH * (c + 1), :]) * modv(4, CH) + modv(3, CH))
            y_s[CH // 2 * c:CH // 2 * (c + 1), :] = _pack(y)
            return token(y)

        def bias(b, n, toks):
            nt = b.shape[1] // 128
            b8 = jnp.broadcast_to(b, (8, b.shape[1]))
            tiles = [b8[:, 128 * j:128 * j + 128] for j in range(nt)]
            if isinstance(toks, dict):
                toks = list(toks.items())
            else:
                toks = [(i * nt // len(toks), t) for i, t in enumerate(toks)]
            for j, t in toks:
                tiles[j] = tiles[j] + t
            return _rep(jnp.concatenate(tiles, axis=1), n)

        def w1_stage(r0, n, toks=()):
            b1 = b1_v[...].astype(f32).reshape(1, F)
            raw = lax.dot_general(_unpack(y_s[r0 // 2:(r0 + n) // 2, :]), weight(w1t_v, w1_p, second, 0, FM),
                                  NT, preferred_element_type=f32)
            if callable(toks):
                toks = toks(raw)
            hh_s[r0 // 2:(r0 + n) // 2, :] = _pack(_gelu(raw + bias(b1[:, 0:FM], n, toks)))

        def w1_rem():
            b1 = b1_v[...].astype(f32).reshape(1, F)[:, FM:F]
            rt = lax.dot_general(weight(w1t_v, w1_p, second, FM, F), _unpack(y_s[...]), NT,
                                 preferred_element_type=f32)
            r = jnp.concatenate([rt[:, 0:QB], rt[:, QB:T]], axis=0).T
            hr_s[...] = _pack(_gelu(r + jnp.concatenate([b1, b1], axis=1)))

        def w2_stage(b, toks=(), strips=((0, D),)):
            r0 = QB * b
            b2 = bias(b2_v[...].astype(f32).reshape(1, D), QB, toks)
            if second and b == 0:
                wr = pltpu.bitcast(w2_v[FM:F, :], u32)
                zz = jnp.zeros_like(wr)
                w2_p[FM // 2:FM // 2 + 128, :] = jnp.concatenate([wr, zz, zz, wr], axis=0)
            wm = weight(w2_v, w2_p, second and b == 0, 0, FM)
            wr = _unpack(w2_p[FM // 2 + 64 * b:FM // 2 + 64 * b + 64, :])
            lhs = jnp.concatenate([hh_s[r0 // 2:(r0 + QB) // 2, :], hr_s[...]], axis=1)
            mo = jnp.dot(_unpack(lhs), jnp.concatenate([wm, wr], axis=0), preferred_element_type=f32) + b2
            rows = pl.ds(pl.multiple_of((step - 1) * T + r0, QB), QB)
            res = (x1_s[r0:r0 + QB, :] + modv(5, QB) * mo).astype(bf16)
            for c0, c1 in strips:
                o_v[rows, c0:c1] = res[:, c0:c1]
                pltpu.make_async_copy(o_v.at[rows, c0:c1], o_h.at[0, rows, c0:c1], osem.at[0]).start()

        def wt_cols(dst, c0, t):
            w = wqkv_v[128 * t:128 * t + 128, c0:c0 + D].astype(f32).T
            dst[:, 128 * t:128 * t + 128] = _pack(w)
            return token(w[D - 16:D])

        def seg(k, c0, c1, r0, r1):
            lo, hi = 128 * k, 128 * k + 128
            h = n_s[r0:r1, lo:hi] * _rep(mod_s[:, D + lo:D + hi], r1 - r0) + _rep(mod_s[:, lo:hi], r1 - r0)
            w = wqkv_v[lo:hi, c0:c1]
            if r0 == 0 and c0 <= D and c1 >= 2 * D:
                wk_p[lo // 2:hi // 2, :] = pltpu.bitcast(w[:, D - c0:2 * D - c0], u32)
            r = jnp.dot(h.astype(bf16), w, preferred_element_type=f32)
            return r if k == 0 else r + acc_s[r0:r1, c0:c1]

        def fin(which, b0, b1):
            r = seg(4, which * D, (which + 1) * D, QB * b0, QB * b1)
            for b in range(b0, b1):
                rb = r[QB * (b - b0):QB * (b - b0 + 1)]
                if which == 0:
                    qT_s[b] = _pack((rb * QSCALE).T)
                elif which == 1:
                    kstore(rb, b)
                else:
                    vstore(rb.T, b)

        if first:
            st["job"] = 0

            def jobs(n):
                j0, j1 = st["job"], st["job"] + n
                st["job"] = j1
                while j0 < j1:
                    kb_, t0 = divmod(j0, 15)
                    t1 = min(15, t0 + j1 - j0)
                    k, b = divmod(kb_, 4)
                    acc_s[QB * b:QB * b + QB, 128 * t0:128 * t1] = seg(k, 128 * t0, 128 * t1, QB * b, QB * b + QB)
                    j0 += t1 - t0

            def norm(c0, c1):
                for c in range(c0, c1):
                    n_s[CH * c:CH * (c + 1), :] = _ln(x_v[CH * c:CH * (c + 1), :].astype(f32))

            for n in names:
                cp(n).start()
            wait("c", "x0")
            norm(0, NCH)
            wait("sa0", "ca0")
            col_s[...] = jnp.broadcast_to(silu_c().astype(f32), (128, D)).T
            mod_mxu([0, 5])
            wait("r0")
            jobs(16)
            wait("x1")
            norm(NCH, 2 * NCH)
            jobs(28)
            wait("sa1", "ca1")
            mod_vpu([1, 6], 16)
            jobs(16)
            wait("r1")
            jobs(44)
            for k in (2, 3):
                wait("sa%d" % k, "ca%d" % k, "r%d" % k)
                mod_vpu([k, k + 5], 16)
                jobs(60 if k == 2 else 48)
            wait("sa4", "ca4", "r4")
            mod_vpu([4, 9], 16)
            jobs(13)
            fin(2, 0, 2)
            fin(0, 0, 2)
            fin(1, 0, 3)
            fin(2, 2, 3)
            fin(0, 2, 3)
            order = [u for g in range(NG) for u in (NG + g, g)]
            stage1(order[0], 0)
            stage1(order[1], 1)
            for i, u in enumerate(order):
                if i + 2 < NU:
                    stage1(order[i + 2], (i + 2) % 3)
                if i == NU - 2:
                    jobs(8)
                stage2(u)
            jobs(7)
            wait("wm2", "wo")
        elif variant in ("second", "mid"):
            if second:
                mod_vpu([15, 20, 10, 16, 21, 17, 11, 22, 18, 23, 12, 19, 24, 14, 13], 16)
            else:
                kf = jnp.dot(_unpack(hb_s[...]), _unpack(wk_p[...]), preferred_element_type=f32)
                for b in range(2):
                    kstore(kf[QB * b:QB * b + QB], g0 + b)
                wo_stage(0, T)
                qf = lax.dot_general(_unpack(wqT_s[...]), _unpack(hb_s[...]), NT, preferred_element_type=f32)
                for b in range(2):
                    qT_s[b] = _pack(qf[:, QB * b:QB * b + QB] * QSCALE)
                vf = lax.dot_general(_unpack(wvT_s[...]), _unpack(hb_s[...]), NT, preferred_element_type=f32)
                for b in range(2):
                    vstore(vf[:, QB * b:QB * b + QB], g0 + b)
                an = [z[r:r + 8, 128 * b:128 * b + 128] for z in (qf, vf) for b in range(2)
                      for r in range(0, 576, 96)]
                for c in range(NCH):
                    anchor_x1(an[c])
                    ln23_chunk(c)
            a1 = stage1(0, 0)
            if second:
                for which in (1, 2, 0):
                    fin(which, 3, 4)
                wo_stage(0, T)
            for u in range(NU):
                if u == NU - 2:
                    if second:
                        wait("x2", "b1", "b2", "w1")
                    nxt = jnp.minimum(step + 1, NS - 1)
                    t1 = [ln1_chunk(c, nxt) for c in range(NCH)]
                    w1_stage(0, T, t1 if second else t1[0:9])
                    w1_rem()
                if second and 1 <= u <= 10:
                    anchor_x1(a1)
                    for c in range(-(-NCH * (u - 1) // 10), -(-NCH * u // 10)):
                        ln23_chunk(c)
                if u + 1 < NU:
                    a1 = stage1(u + 1, (u + 1) % 3)
                elif second:
                    wait("wm3", "w2")
                    mod_vpu(range(25, 30), 8)
                    w2_stage(0, [wt_cols(wqT_s, 0, t) for t in range(5)])
                else:
                    w2_stage(0, t1[9:14])
                stage2(u)
            w2_stage(1, [wt_cols(wvT_s, 2 * D, t) for t in range(5)] if second else dict(enumerate(t1[14:])))
            if second:
                wait("xr")
        else:
            wo_stage(0, QB)
            for c in range(NCH // 2):
                ln23_chunk(c)
            wo_stage(QB, QB)

            def ln23_b(raw):
                toks = {}
                for i in range(NCH // 2):
                    anchor_x1(raw[0:8, 128 * i:128 * i + 128])
                    toks[i + 5] = ln23_chunk(NCH // 2 + i)
                return toks

            w1_stage(0, QB, ln23_b)
            w1_stage(QB, QB)
            w1_rem()
            w2_stage(0)
            w2_stage(1, (), ((0, 512), (512, D)))
            pltpu.make_async_copy(o_v, o_h.at[0], osem.at[0]).wait()

    @pl.when(step == 0)
    def _():
        body("first")

    @pl.when(step == 1)
    def _():
        body("second")

    @pl.when((step > 1) & (step < NS))
    def _():
        body("mid")

    @pl.when(step == NS)
    def _():
        body("last")


@jax.jit
def pallas_adaLN_cond__sliding_block__mixer_channel_mlp__prompt_kernel(
    A_x: jax.Array,
    A_wqkv: jax.Array,
    A_wo: jax.Array,
    B_x: jax.Array,
    B_w1: jax.Array,
    B_b1: jax.Array,
    B_w2: jax.Array,
    B_b2: jax.Array,
    c: jax.Array,
    w_mod: jax.Array,
):
    del B_x
    anyspec = pl.BlockSpec(memory_space=pl.ANY)
    V = pltpu.VMEM
    return pl.pallas_call(
        _kernel,
        grid=(NS + 1,),
        in_specs=[anyspec] * 9,
        out_specs=anyspec,
        out_shape=jax.ShapeDtypeStruct((1, S, D), bf16),
        scratch_shapes=[
            V((S, D), bf16), V((1, D), bf16), V((F,), bf16), V((D,), bf16),
            V((D, 3 * D), bf16), V((D, D), bf16), V((F, D), bf16), V((F, D), bf16),
            V((D, 6 * D), bf16), V((S, D), bf16),
            pltpu.SemaphoreType.DMA((27,)), pltpu.SemaphoreType.DMA((1,)),
            V((8, 6 * D), f32), V((D, 128), f32),
            V((D // 2, D), u32), V((D // 2, D), u32), V((D // 2, D), u32), V((D // 2, D), u32),
            V((F // 2, D), u32), V((FM // 2 + 128, D), u32),
            V((NB, QB // 2, 128 * NG), u32), V((NB, 24 * H, QB), f32), V((4, D // 2, QB), u32),
            V((3, 256, 512), f32), V((3, D, QB), f32), V((QB // 2, D), u32), V((QB // 2, D), u32),
            V((T // 2, D), u32), V((T + 8, D), f32), V((T // 2, D), u32),
            V((T // 2, FM), u32), V((QB // 2, 128), u32),
            V((2 * T, D), f32), V((2 * T, 3 * D), f32),
        ],
        compiler_params=pltpu.CompilerParams(
            dimension_semantics=("arbitrary",),
            vmem_limit_bytes=100 * 1024 * 1024,
            disable_bounds_checks=True,
            disable_semaphore_checks=True,
        ),
    )(A_x, c, B_b1, B_b2, A_wqkv, A_wo, B_w1.T, B_w2, w_mod)
```
